```python
import jax
import jax.numpy as jnp

def _softmax(x, axis=-1):
    return jax.nn.softmax(x, axis=axis)

def _gelu(x):
    return jax.nn.gelu(x, approximate=True)

def _silu(x):
    return jax.nn.silu(x)

def _sigmoid(x):
    return jax.nn.sigmoid(x)

def _layernorm(x, axis=-1, eps=1e-05):
    m = jnp.mean(x, axis=axis, keepdims=True)
    v = jnp.var(x, axis=axis, keepdims=True)
    return (x - m) / jnp.sqrt(v + eps)

def _scatter_add(tgt, idx, src, axis=0):
    return tgt.at[idx].add(src)

def _segment_sum(src, seg, n):
    return jax.ops.segment_sum(src, seg, n)

class _Rng:

    def __init__(self, key):
        self._k = key

    def _next(self):
        self._k, sub = jax.random.split(self._k)
        return sub

    def normal(self, shape):
        return jax.random.normal(self._next(), shape, dtype=jnp.bfloat16)

    def randint(self, lo, hi, shape):
        return jax.random.randint(self._next(), shape, lo, hi, dtype=jnp.int32)

    def uniform(self, shape, lo=0.0, hi=1.0):
        return jax.random.uniform(self._next(), shape, jnp.bfloat16, lo, hi)

    def permutation(self, n):
        return jax.random.permutation(self._next(), n)
kernel_name = 'adaLN_cond__linear_kernel_hedgehog__moe_arch_mod__prompt'

def setup_inputs():
    _rng = _Rng(jax.random.key(int.from_bytes(__import__("os").urandom(4), "little")))
    _w = lambda a: (lambda t: t.astype(jnp.bfloat16) if jnp.issubdtype(t.dtype, jnp.floating) else t)(jnp.asarray(a))

    def _A_setup():
        B, S, D, H = (1, 2048, 1024, 32)
        Dh = D // H
        return {'x': _w((lambda *s: _rng.normal(s) * 0.05)(B, S, D)), 'wqkv': _w((lambda *s: _rng.normal(s) * 0.05)(D, 3 * D)), 'w_phi': _w((lambda *s: _rng.normal(s) * 0.05)(H, Dh, Dh) * Dh ** (-0.5)), 'wo': _w((lambda *s: _rng.normal(s) * 0.05)(D, D))}
    _A_in = _A_setup()

    def _B_setup():
        B, S, D, F, C = (1, 2048, 1024, 3584, 2)
        return {'x': _w((lambda *s: _rng.normal(s) * 0.05)(B, S, D)), 'w_r': _w((lambda *s: _rng.normal(s) * 0.05)(D)), 'w_gate': _w((lambda *s: _rng.normal(s) * 0.05)(D, F)), 'w_up': _w((lambda *s: _rng.normal(s) * 0.05)(D, F)), 'w_down': _w((lambda *s: _rng.normal(s) * 0.05)(F, D))}
    _B_in = _B_setup()
    return {'A_x': _A_in['x'], 'A_wqkv': _A_in['wqkv'], 'A_w_phi': _A_in['w_phi'], 'A_wo': _A_in['wo'], 'B_x': _B_in['x'], 'B_w_r': _B_in['w_r'], 'B_w_gate': _B_in['w_gate'], 'B_w_up': _B_in['w_up'], 'B_w_down': _B_in['w_down'], 'c': _w((lambda *s: _rng.normal(s) * 0.05)(1, 1024)), 'w_mod': _w((lambda *s: _rng.normal(s) * 0.05)(1024, 6 * 1024) * 1024 ** (-0.5))}

def reference(A_x, A_wqkv, A_w_phi, A_wo, B_x, B_w_r, B_w_gate, B_w_up, B_w_down, c, w_mod):

    def _A_ref(x, wqkv, w_phi, wo):
        B, S, D = x.shape
        H = 32
        Dh = D // H
        qkv = (lambda x, *d: x.transpose(*d))((x @ wqkv).reshape(B, S, 3, H, Dh), 2, 0, 3, 1, 4)
        q, k, v = (qkv[0], qkv[1], qkv[2])
        pq = jnp.einsum('bhsd,hdf->bhsf', q, w_phi)
        pk = jnp.einsum('bhsd,hdf->bhsf', k, w_phi)
        phi_q = jnp.concatenate([_softmax(pq, axis=-1), _softmax(-pq, axis=-1)], axis=-1)
        phi_k = jnp.concatenate([_softmax(pk, axis=-1), _softmax(-pk, axis=-1)], axis=-1)
        kv = jnp.einsum('bhsf,bhsd->bhfd', phi_k, v)
        z = jnp.einsum('bhsf->bhf', phi_k)
        num = jnp.einsum('bhqf,bhfd->bhqd', phi_q, kv)
        den = jnp.einsum('bhqf,bhf->bhq', phi_q, z)[..., None] + 1e-06
        o = num / den
        return (lambda x, *d: x.transpose(*d))(o, 0, 2, 1, 3).reshape(B, S, D) @ wo

    def _B_ref(x, w_r, w_gate, w_up, w_down):
        B, S, D = x.shape
        C = 2
        r = x @ w_r
        idx = jnp.argsort(-r, axis=-1)[:, :C]
        idx_e = jnp.repeat(idx.reshape(B, C, 1), D, axis=2)
        x_sel = jnp.take_along_axis(x, idx_e, axis=1)
        g = _silu(x_sel @ w_gate)
        u = x_sel @ w_up
        y = g * u @ w_down
        r_sel = _sigmoid(jnp.take_along_axis(r, idx, axis=1))
        y = y * r_sel.reshape(B, C, 1)
        b_off = (jnp.arange(B) * S).reshape(B, 1)
        flat_idx = (idx + b_off).reshape(B * C)
        zero = (x * 0.0).reshape(B * S, D)
        upd = _scatter_add(zero, flat_idx, y.reshape(B * C, D), axis=0)
        return x + upd.reshape(B, S, D)
    x = A_x
    mod = (_silu(c) @ w_mod).reshape(c.shape[0], 6, 1, -1)
    sa, ca, ga, sb, cb, gb = (mod[:, 0].copy(), mod[:, 1].copy(), mod[:, 2].copy(), mod[:, 3].copy(), mod[:, 4].copy(), mod[:, 5].copy())
    h = _layernorm(x, axis=-1) * (1 + ca) + sa
    x = x + ga * _A_ref(h, A_wqkv, A_w_phi, A_wo)
    h = _layernorm(x, axis=-1) * (1 + cb) + sb
    x = x + gb * _B_ref(h, B_w_r, B_w_gate, B_w_up, B_w_down)
    return x
```

```python
import functools
import math

import jax
import jax.numpy as jnp
from jax import lax
import jax.experimental.pallas as pl
import jax.experimental.pallas.tpu as pltpu

S, D, H, DH, F = 2048, 1024, 32, 32, 3584
T = 256
NT = S // T
NPAIR = H // 2
PAD = 128
LOG2E = math.log2(math.e)
BF, F32, U32, I32 = jnp.bfloat16, jnp.float32, jnp.uint32, jnp.int32
NT_DIMS = (((1,), (1,)), ((), ()))


def _dot(a, b):
    return jnp.dot(a, b, preferred_element_type=F32)


def _dot_nt(a, b):
    return lax.dot_general(a, b, NT_DIMS, preferred_element_type=F32)


def _pack(v):
    return pltpu.bitcast(v.astype(BF), U32)


def _unpack(v):
    return pltpu.bitcast(v, BF)


def _normalize(v):
    m = jnp.mean(v, axis=-1, keepdims=True)
    vc = v - m
    var = jnp.mean(vc * vc, axis=-1, keepdims=True)
    return vc * lax.rsqrt(var + 1e-5)


def _hedgehog(p):
    parts = []
    for j in range(2):
        ph = p[j * DH:(j + 1) * DH]
        ep = jnp.exp2(ph - jnp.max(ph, axis=0, keepdims=True))
        en = jnp.exp2(jnp.min(ph, axis=0, keepdims=True) - ph)
        parts.append(ep * (1.0 / jnp.sum(ep, axis=0, keepdims=True)))
        parts.append(en * (1.0 / jnp.sum(en, axis=0, keepdims=True)))
    return jnp.concatenate(parts, axis=0).astype(BF)


def _kernel(x_hbm, wqkv_hbm, wphi_hbm, wo_hbm, wr_hbm, wg_hbm, wu_hbm, wd_hbm, c_hbm, wmod_hbm,
            out_hbm,
            x_v, wqkv_v, wphi_v, wo_v, wr_v, wg_v, wu_v, wd_v, c_v, wmod_v,
            wt_s, h_s, kv_s, kvm_s, mod_s, x1_s, out_s, p_s,
            sem_w, sem_x, sem_o, sem_p):
    def wcopy(i, src, dst):
        return pltpu.make_async_copy(src, dst, sem_w.at[i])

    cp_c = wcopy(0, c_hbm, c_v)
    cp_phi = wcopy(1, wphi_hbm, wphi_v)
    cp_wr = wcopy(2, wr_hbm, wr_v)
    cp_wq = wcopy(3, wqkv_hbm.at[:, 0:D], wqkv_v.at[0])
    cp_wk = wcopy(4, wqkv_hbm.at[:, D:2 * D], wqkv_v.at[1])
    cp_wv = wcopy(5, wqkv_hbm.at[:, 2 * D:3 * D], wqkv_v.at[2])
    cp_ma = wcopy(6, wmod_hbm.at[:, 0:2 * D], wmod_v.at[:, 0:2 * D])
    cp_mb = wcopy(7, wmod_hbm.at[:, 2 * D:6 * D], wmod_v.at[:, 2 * D:6 * D])
    cp_wo = wcopy(8, wo_hbm, wo_v)
    cp_wg = wcopy(9, wg_hbm, wg_v.at[:, 0:F])
    cp_wu = wcopy(10, wu_hbm, wu_v.at[:, 0:F])
    cp_wd = wcopy(11, wd_hbm, wd_v.at[:, 0:D])

    def x_copy(t):
        rows = pl.ds(pl.multiple_of(t * T, T), T)
        return pltpu.make_async_copy(x_hbm.at[rows], x_v.at[rows], sem_x.at[t])

    def out_copy(t):
        rows = pl.ds(pl.multiple_of(t * T, T), T)
        return pltpu.make_async_copy(out_s.at[rows], out_hbm.at[rows], sem_o.at[t])

    for cp in (cp_c, cp_phi, cp_wr, cp_wk, cp_ma):
        cp.start()
    x_copy(0).start()
    cp_wv.start()

    cp_phi.wait()
    rep = (lax.broadcasted_iota(I32, (128, DH), 0) % DH == lax.broadcasted_iota(I32, (128, DH), 1)).astype(BF)
    same_head = (lax.broadcasted_iota(I32, (128, 128), 0) // DH) == (lax.broadcasted_iota(I32, (128, 128), 1) // DH)
    for g in range(8):
        full = _dot_nt(rep, wphi_v[g * 128:(g + 1) * 128, :])
        p_s[g] = _pack(jnp.where(same_head, full, 0.0))

    def fold(which):
        for g in range(8):
            w = wqkv_v[which, :, g * 128:(g + 1) * 128]
            wt_s[which, g * 64:(g + 1) * 64, :] = _pack(_dot_nt(_unpack(p_s[g]), w) * LOG2E)

    cp_wk.wait()
    fold(1)

    cp_c.wait()
    cv = c_v[...].astype(F32)
    sc = jnp.broadcast_to(cv * jax.nn.sigmoid(cv), (16, D)).astype(BF)
    cp_ma.wait()
    mod_s[:, 0:2 * D] = _dot(sc, wmod_v[:, 0:2 * D])[0:8]

    for t in range(1, NT):
        x_copy(t).start()
    cp_wq.start()
    cp_mb.start()
    cp_wo.start()
    cp_wg.start()
    cp_wu.start()
    cp_wd.start()

    cp_wv.wait()
    for g in range(8):
        wt_s[2, g * 64:(g + 1) * 64, :] = pltpu.bitcast(wqkv_v[2, :, g * 128:(g + 1) * 128].T, U32)

    kv_s[...] = jnp.zeros(kv_s.shape, F32)

    def phase1(t, carry):
        x_copy(t).wait()
        rows = pl.ds(pl.multiple_of(t * T, T), T)
        xn = _normalize(x_v[rows, :].astype(F32))
        hb = (xn * (1.0 + mod_s[0:1, D:2 * D]) + mod_s[0:1, 0:D]).astype(BF)
        h_s[pl.ds(pl.multiple_of(t * (T // 2), T // 2), T // 2), :] = pltpu.bitcast(hb, U32)
        ones = jnp.ones((16, T), BF)
        for p in range(NPAIR):
            w = jnp.concatenate([_unpack(wt_s[1, p * 32:(p + 1) * 32, :]),
                                 _unpack(wt_s[2, p * 32:(p + 1) * 32, :])], axis=0)
            r = _dot_nt(w, hb)
            phi = _hedgehog(r[0:64])
            lhs = jnp.concatenate([r[64:128].astype(BF), ones], axis=0)
            kv_s[p] += _dot_nt(lhs, phi)
        return carry

    lax.fori_loop(0, NT, phase1, 0)

    cp_wq.wait()
    fold(0)
    cp_mb.wait()
    mod_s[:, 2 * D:6 * D] = _dot(sc, wmod_v[:, 2 * D:6 * D])[0:8]
    row = lax.broadcasted_iota(I32, (80, 128), 0)
    lane_head = lax.broadcasted_iota(I32, (80, 128), 1) // 64
    row_head = jnp.where(row < 64, row // 32, (row - 64) // 8)
    for p in range(NPAIR):
        kvm_s[p] = _pack(jnp.where(row_head == lane_head, kv_s[p], 0.0))
    cp_wr.wait()
    wr8 = wr_v[...].astype(F32)
    wr = jnp.concatenate([wr8[j:j + 1, :] for j in range(8)], axis=1)
    cp_wo.wait()

    def second_norm(x1):
        return _normalize(x1) * (1.0 + mod_s[0:1, 4 * D:5 * D]) + mod_s[0:1, 3 * D:4 * D]

    def phase2(t, carry):
        m1, i1, m2, i2 = carry
        rows = pl.ds(pl.multiple_of(t * T, T), T)
        hb = _unpack(h_s[pl.ds(pl.multiple_of(t * (T // 2), T // 2), T // 2), :])
        outs = []
        for g in range(8):
            r = _dot_nt(_unpack(wt_s[0, g * 64:(g + 1) * 64, :]), hb)
            for j in range(2):
                phi = _hedgehog(r[j * 64:(j + 1) * 64])
                nd = _dot(_unpack(kvm_s[2 * g + j]), phi)
                for k in range(2):
                    inv = 1.0 / (nd[64 + 8 * k:65 + 8 * k] + 1e-6)
                    outs.append((nd[k * 32:(k + 1) * 32] * inv).astype(BF))
        o = jnp.concatenate(outs, axis=0).T
        attn = _dot(o, wo_v[...])
        x1 = x_v[rows, :].astype(F32) + mod_s[0:1, 2 * D:3 * D] * attn
        x1_s[rows, :] = x1
        h2 = second_norm(x1)
        out_s[rows, :] = (x1 + mod_s[0:1, 5 * D:6 * D] * h2).astype(BF)
        out_copy(t).start()
        score = jnp.sum(h2 * wr, axis=-1, keepdims=True)
        sub = lax.broadcasted_iota(I32, (8, 1), 0)
        for j in range(T // 8):
            rj = score[j * 8:(j + 1) * 8]
            ij = sub + (t * T + j * 8)
            g1, g2 = rj > m1, rj > m2
            m2 = jnp.where(g1, m1, jnp.where(g2, rj, m2))
            i2 = jnp.where(g1, i1, jnp.where(g2, ij, i2))
            m1 = jnp.where(g1, rj, m1)
            i1 = jnp.where(g1, ij, i1)
        return m1, i1, m2, i2

    neg = jnp.full((8, 1), -jnp.inf, F32)
    zero = jnp.zeros((8, 1), I32)
    m1, i1, m2, i2 = lax.fori_loop(0, NT, phase2, (neg, zero, neg, zero))

    best = jnp.max(m1, axis=0, keepdims=True)
    ia = jnp.min(jnp.where(m1 == best, i1, S - 1), axis=0, keepdims=True)
    taken = i1 == ia
    mr = jnp.where(taken, m2, m1)
    ir = jnp.where(taken, i2, i1)
    second = jnp.max(mr, axis=0, keepdims=True)
    ib = jnp.min(jnp.where(mr == second, ir, S - 1), axis=0, keepdims=True)
    idx_a = jnp.clip(ia[0, 0], 0, S - 1)
    idx_b = jnp.clip(ib[0, 0], 0, S - 1)

    cp_wg.wait()
    cp_wu.wait()
    cp_wd.wait()
    r16 = lax.broadcasted_iota(I32, (16, D), 0)
    x1_sel = jnp.where(r16 == 0, x1_s[pl.ds(idx_a, 1), :], x1_s[pl.ds(idx_b, 1), :])
    h2_sel = second_norm(x1_sel)
    gate = jax.nn.sigmoid(jnp.sum(h2_sel * wr, axis=-1, keepdims=True))
    hs = h2_sel.astype(BF)
    y = jnp.zeros((16, D), F32)
    FC = 512
    for j in range(F // FC):
        gj = _dot(hs, wg_v[:, j * FC:(j + 1) * FC])
        uj = _dot(hs, wu_v[:, j * FC:(j + 1) * FC])
        a = (gj * jax.nn.sigmoid(gj) * uj).astype(BF)
        y = y + _dot(a, wd_v[j * FC:(j + 1) * FC, 0:D])
    new = x1_sel + mod_s[0:1, 5 * D:6 * D] * (h2_sel + y * gate)

    for t in range(NT):
        out_copy(t).wait()

    def patch(idx, k):
        base = pl.multiple_of((idx // 16) * 16, 16)
        blk = out_s[pl.ds(base, 16), :].astype(F32)
        out_s[pl.ds(base, 16), :] = jnp.where(r16 == idx - base, new[k:k + 1, :], blk).astype(BF)
        return pltpu.make_async_copy(out_s.at[pl.ds(base, 16)], out_hbm.at[pl.ds(base, 16)], sem_p.at[k])

    pa = patch(idx_a, 0)
    pb = patch(idx_b, 1)
    pa.start()

    @pl.when(idx_a // 16 != idx_b // 16)
    def _():
        pb.start()
        pb.wait()

    pa.wait()


@jax.jit
def pallas_adaLN_cond__linear_kernel_hedgehog__moe_arch_mod__prompt_kernel(
        A_x, A_wqkv, A_w_phi, A_wo, B_x, B_w_r, B_w_gate, B_w_up, B_w_down, c, w_mod):
    del B_x
    any_spec = pl.BlockSpec(memory_space=pl.ANY)
    out = pl.pallas_call(
        _kernel,
        out_shape=jax.ShapeDtypeStruct((S, D), BF),
        in_specs=[any_spec] * 10,
        out_specs=any_spec,
        scratch_shapes=[
            pltpu.VMEM((S, D), BF),
            pltpu.VMEM((3, D, D), BF),
            pltpu.VMEM((H * DH, DH), BF),
            pltpu.VMEM((D, D), BF),
            pltpu.VMEM((8, 128), BF),
            pltpu.VMEM((D, F + PAD), BF),
            pltpu.VMEM((D, F + PAD), BF),
            pltpu.VMEM((F, D + PAD), BF),
            pltpu.VMEM((1, D), BF),
            pltpu.VMEM((D, 6 * D + PAD), BF),
            pltpu.VMEM((3, D // 2, D), U32),
            pltpu.VMEM((S // 2, D), U32),
            pltpu.VMEM((NPAIR, 80, 128), F32),
            pltpu.VMEM((NPAIR, 40, 128), U32),
            pltpu.VMEM((8, 6 * D), F32),
            pltpu.VMEM((S, D), F32),
            pltpu.VMEM((S, D), BF),
            pltpu.VMEM((8, 64, 128), U32),
            pltpu.SemaphoreType.DMA((12,)),
            pltpu.SemaphoreType.DMA((NT,)),
            pltpu.SemaphoreType.DMA((NT,)),
            pltpu.SemaphoreType.DMA((2,)),
        ],
        compiler_params=pltpu.CompilerParams(vmem_limit_bytes=110 * 2**20),
        name="fused_block",
    )(A_x.reshape(S, D), A_wqkv, A_w_phi.reshape(H * DH, DH), A_wo, B_w_r.reshape(8, 128),
      B_w_gate, B_w_up, B_w_down, c, w_mod)
    return out.reshape(1, S, D)
```

```python
import math

import jax
import jax.numpy as jnp
from jax import lax
import jax.experimental.pallas as pl
import jax.experimental.pallas.tpu as pltpu

S, D, H, DH, F = 2048, 1024, 32, 32, 3584
U = 128
T = 2 * U
NT = S // T
KH = D // 2
NPAIR = H // 2
HROWS = 7 * U // 2
PAD = 128
FC = 512
LN_ROWS = 32
LOG2E = math.log2(math.e)
BF, F32, U32, I32 = jnp.bfloat16, jnp.float32, jnp.uint32, jnp.int32

SHIFT_A, SCALE_A, GATE_A, SHIFT_B, SCALE_B, GATE_B, ROUTER_SUMS = range(7)
COL_GATE_A, COL_ROUTER, COL_GAIN, COL_BIAS = range(4)

PLAN_FIRST = ("p p p p W s p p p", "W p N s p p p p p p", "W p N s p p p p p p",
              "X L p N p p p p p p", "p p p p p p p N")
PLAN_KV = ("p p N p p p p p",) * 4
PLAN_KV_LAST = ("p N p p p s p p p",) * 4
PLAN_Q_FIRST = ("s M N c c q q q q q q q",) * 4
PLAN_Q = ("w w w w w w w q N c c q q q q q q E",) * 4
PLAN_Q_SECOND = PLAN_Q[:3] + ("q q q q q q q w N c c w w w w w w",)
PLAN_Q_LAST = PLAN_Q[:3] + ("w w w w N c c w w w E",)
PLAN_DRAIN = ("w w w w w w w E E",) * 2 + ("w w w w w w w",) * 2


def _dot(a, b):
    return jnp.dot(a, b, preferred_element_type=F32)


def _dot_nt(a, b):
    return lax.dot_general(a, b, (((1,), (1,)), ((), ())), preferred_element_type=F32)


def _pack(v):
    return pltpu.bitcast(v.astype(BF), U32)


def _unpack(v):
    return pltpu.bitcast(v, BF)


def _recip(v):
    return pl.reciprocal(v, approx=False, full_range=False)


def _rows(start, size):
    return pl.ds(start if isinstance(start, int) else pl.multiple_of(start, 8), size)


def _normalize(v):
    centered = v - jnp.mean(v, axis=-1, keepdims=True)
    var = jnp.mean(centered * centered, axis=-1, keepdims=True)
    return centered * lax.rsqrt(var + 1e-5)


def _hedgehog(p):
    parts = []
    for j in range(2):
        ph = p[j * DH:(j + 1) * DH]
        pos = jnp.exp2(ph - jnp.max(ph, axis=0, keepdims=True))
        neg = jnp.exp2(jnp.min(ph, axis=0, keepdims=True) - ph)
        parts.append(pos * _recip(jnp.sum(pos, axis=0, keepdims=True)))
        parts.append(neg * _recip(jnp.sum(neg, axis=0, keepdims=True)))
    return jnp.concatenate(parts, axis=0).astype(BF)


def _fold8(v):
    parts = [v[i:i + 8] for i in range(0, v.shape[0], 8)]
    while len(parts) > 1:
        parts = [parts[i] + parts[i + 1] for i in range(0, len(parts), 2)]
    return parts[0]


def _left_terms(a11, a12, a21, a22):
    return a11 + a22, a21 + a22, a11, a22, a11 + a12, a21 - a11, a12 - a22


def _right_terms(b11, b12, b21, b22):
    return b11 + b22, b11, b12 - b22, b21 - b11, b22, b11 + b12, b21 + b22


class _Strassen:
    _SCHEDULE = ((0, ((0, 1), (3, 1))), (1, ((2, 1), (3, -1))), (2, ((1, 1), (3, 1))), (5, ((3, 1),)),
                 (3, ((0, 1), (2, 1))), (4, ((0, -1), (1, 1))), (6, ((0, 1),)))

    def __init__(self, product):
        self._product = product
        self._todo = list(self._SCHEDULE)
        self._c = [None] * 4

    @property
    def done(self):
        return not self._todo

    def step(self):
        i, uses = self._todo.pop(0)
        m = self._product(i)
        for k, sign in uses:
            if self._c[k] is None:
                self._c[k] = m
            else:
                self._c[k] = self._c[k] + m if sign > 0 else self._c[k] - m

    def result(self):
        assert self.done
        return jnp.concatenate(self._c[:2], axis=1), jnp.concatenate(self._c[2:], axis=1)


def _kernel(x_hbm, wqkv_hbm, wphi_hbm, wo_hbm, wr_hbm, wg_hbm, wu_hbm, wd_hbm, c_hbm, wmod_hbm,
            out_hbm,
            x_v, wqkv_v, wphi_v, wo_v, wr_v, wg_v, wu_v, wd_v, c_v, wmod_v,
            wkv_s, wq_s, wo_s, h_s, kv_s, mod_s, col_s, d_s, stat_s, out_s, fmap_s,
            oa_s, ob_s, vec_s, xn_s, carry_s,
            sem_w, sem_m, sem_k, sem_v, sem_x, sem_o, sem_p):
    def wcopy(i, src, dst):
        return pltpu.make_async_copy(src, dst, sem_w.at[i])

    cp_c = wcopy(0, c_hbm, c_v)
    cp_phi = wcopy(1, wphi_hbm, wphi_v)
    cp_wr = wcopy(2, wr_hbm, wr_v)
    cp_wq = wcopy(3, wqkv_hbm.at[:, 0:D], wqkv_v.at[:, 0:D])
    cp_mb = wcopy(4, wmod_hbm.at[:, 2 * D:4 * D], wmod_v.at[:, 2 * D:4 * D])
    cp_mc = wcopy(5, wmod_hbm.at[:, 4 * D:6 * D], wmod_v.at[:, 4 * D:6 * D])
    cp_wo = wcopy(6, wo_hbm, wo_v.at[:, 0:D])
    cp_wg = wcopy(7, wg_hbm, wg_v.at[:, 0:F])
    cp_wu = wcopy(8, wu_hbm, wu_v.at[:, 0:F])
    cp_wd = wcopy(9, wd_hbm, wd_v.at[:, 0:D])

    def mod_copy(j):
        cols = pl.ds(j * 512 if isinstance(j, int) else pl.multiple_of(j * 512, 512), 512)
        return pltpu.make_async_copy(wmod_hbm.at[:, cols], wmod_v.at[:, cols], sem_m.at[j])

    def kv_copies(o):
        ck, cv = pl.ds(D + o * 256, 256), pl.ds(2 * D + o * 256, 256)
        return (pltpu.make_async_copy(wqkv_hbm.at[:, ck], wqkv_v.at[:, ck], sem_k.at[o]),
                pltpu.make_async_copy(wqkv_hbm.at[:, cv], wqkv_v.at[:, cv], sem_v.at[o]))

    def x_copy(t):
        rows = _rows(t * T, T)
        return pltpu.make_async_copy(x_hbm.at[rows], x_v.at[rows], sem_x.at[t])

    def out_copy(t):
        rows = _rows(t * T, T)
        return pltpu.make_async_copy(out_s.at[rows], out_hbm.at[rows], sem_o.at[t])

    def start(*copies):
        for cp in copies:
            cp.start()

    def wait(*copies):
        for cp in copies:
            cp.wait()

    def fold(col0, g):
        return _dot_nt(_unpack(fmap_s[g * 64:(g + 1) * 64, :]),
                       wqkv_v[:, col0 + g * 128:col0 + (g + 1) * 128]) * LOG2E

    def stage_left(dst, o, upper, lower):
        n = upper.shape[0] // 2
        for i, a in enumerate(_left_terms(upper[:, :KH], upper[:, KH:], lower[:, :KH], lower[:, KH:])):
            dst[(i * 4 + o) * n:(i * 4 + o + 1) * n, :] = _pack(a)

    def stage_kv_weights(o):
        blocks = []
        for g in (2 * o, 2 * o + 1):
            fk = fold(D, g)
            fv = wqkv_v[:, 2 * D + g * 128:2 * D + (g + 1) * 128].T.astype(F32)
            blocks.append(jnp.concatenate([fk[:64], fv[:64], fk[64:], fv[64:]], axis=0))
        stage_left(wkv_s, o, *blocks)

    def stage_q_weights(o):
        stage_left(wq_s, o, fold(0, o), fold(0, o + 4))

    def stage_out_weights(o):
        stage_left(wo_s, o, wo_v[:, o * 128:(o + 1) * 128].T.astype(F32),
                   wo_v[:, KH + o * 128:KH + (o + 1) * 128].T.astype(F32))

    def param(k, n):
        return jnp.concatenate([mod_s[:, k * D:(k + 1) * D]] * (n // 8), axis=0)

    def modulation(col0, n):
        mod_s[:, col0:col0 + n] = _dot(_unpack(vec_s[...]), wmod_v[:, col0:col0 + n])[0:8]

    def first_norm(t, dst, base, normalized=None):
        for r0 in range(0, U, LN_ROWS):
            h = []
            for half in range(2):
                rows = _rows(t * T + half * U + r0, LN_ROWS)
                xn = _normalize(x_v[rows, :].astype(F32)) if normalized is None else normalized[rows, :]
                h.append(xn * param(SCALE_A, LN_ROWS) + param(SHIFT_A, LN_ROWS))
            for i, b in enumerate(_right_terms(h[0][:, :KH], h[1][:, :KH], h[0][:, KH:], h[1][:, KH:])):
                dst[base + i * 64 + r0 // 2:base + i * 64 + (r0 + LN_ROWS) // 2, :] = _pack(b)

    def kv_products(src, base, o):
        return _Strassen(lambda i: _dot_nt(_unpack(wkv_s[(i * 4 + o) * 128:(i * 4 + o + 1) * 128, :]),
                                           _unpack(src[base + i * 64:base + (i + 1) * 64, :])))

    def kv_operands(r):
        ops = []
        for j in range(4):
            rj = r[j // 2][(j % 2) * 128:(j % 2 + 1) * 128]
            ops.append((rj[64:].astype(BF), _hedgehog(rj[:64])))
        return ops

    def save_kv_operands(ops):
        for j, (v, phi) in enumerate(ops):
            carry_s[j * 64:(j + 1) * 64, :] = pltpu.bitcast(phi, U32)
            carry_s[256 + j * 32:256 + (j + 1) * 32, :] = pltpu.bitcast(v, U32)

    def load_kv_operands():
        return [(_unpack(carry_s[256 + j * 32:256 + (j + 1) * 32, :]), _unpack(carry_s[j * 64:(j + 1) * 64, :]))
                for j in range(4)]

    def accumulate_kv(ops, o, first=False, last=False):
        ones = jnp.ones((16, T), BF)
        for j, (v, phi) in enumerate(ops):
            acc = _dot_nt(jnp.concatenate([v, ones], axis=0), phi)
            if not first:
                acc = acc + kv_s[4 * o + j]
            if last:
                row = lax.broadcasted_iota(I32, (80, 128), 0)
                lane_head = lax.broadcasted_iota(I32, (80, 128), 1) // 64
                row_head = jnp.where(row < 64, row // 32, (row - 64) // 8)
                acc = jnp.where(row_head == lane_head, acc, 0.0)
            kv_s[4 * o + j] = acc

    start(cp_phi, cp_c, *kv_copies(0), x_copy(0))
    lax.fori_loop(0, 4, lambda j, _: mod_copy(j).start(), None)
    cp_c.wait()
    cv = c_v[...].astype(F32)
    vec_s[...] = _pack(jnp.broadcast_to(cv * jax.nn.sigmoid(cv), (16, D)))
    cp_phi.wait()
    start(*kv_copies(1))
    repeat = (lax.broadcasted_iota(I32, (128, DH), 0) % DH == lax.broadcasted_iota(I32, (128, DH), 1)).astype(BF)
    same_head = (lax.broadcasted_iota(I32, (128, 128), 0) // DH) == (lax.broadcasted_iota(I32, (128, 128), 1) // DH)
    for g in range(8):
        full = _dot_nt(repeat, wphi_v[g * 128:(g + 1) * 128, :])
        fmap_s[g * 64:(g + 1) * 64, :] = _pack(jnp.where(same_head, full, 0.0))
    wait(*kv_copies(0))
    stage_kv_weights(0)
    x_copy(0).wait()
    xn_s[...] = _normalize(x_v[0:T, :].astype(F32))
    for j in range(4):
        mod_copy(j).wait()
        if j == 0:
            start(*kv_copies(2))
        elif j == 2:
            start(*kv_copies(3))
        elif j == 3:
            x_copy(1).start()
        modulation(j * 512, 512)
    mod_s[:, SCALE_A * D:(SCALE_A + 1) * D] += 1.0
    first_norm(0, h_s, 0, normalized=xn_s)

    ops = None
    for o, plan in enumerate(PLAN_FIRST):
        products = kv_products(h_s, (o // 4) * HROWS, o % 4)
        for item in plan.split():
            if item == "p":
                products.step()
            elif item == "W":
                wait(*kv_copies(o + 1))
            elif item == "X":
                x_copy(1).wait()
                start(x_copy(2), x_copy(3), cp_wr)
            elif item == "s":
                stage_kv_weights(o + 1)
            elif item == "L":
                first_norm(1, h_s, HROWS)
            else:
                accumulate_kv(ops, o - 1, first=True)
        ops = kv_operands(products.result())
    save_kv_operands(ops)

    def kv_tile(t, ops, src, base, following=None):
        last = following is not None
        if not last:
            first_norm(t + 1, src, base + HROWS)
        for o, plan in enumerate(PLAN_KV_LAST if last else PLAN_KV):
            if o < 3:
                products = kv_products(src, base, o + 1)
            else:
                products = following if last else kv_products(src, base + HROWS, 0)
            for item in plan.split():
                if item == "p":
                    products.step()
                elif item == "s":
                    stage_q_weights(o)
                else:
                    accumulate_kv(ops, o, last=last)
            if o < 3:
                ops = kv_operands(products.result())
        return products.result()

    def pass1(i, remaining):
        t = 2 * i + 1
        wait(x_copy(t + 1), x_copy(t + 2))
        pl.when(i == 0)(lambda: start(*(x_copy(k) for k in range(4, NT)), cp_wq, cp_wo))
        pl.when(i == 1)(lambda: start(cp_mb, cp_mc, cp_wg))
        view = h_s.at[_rows(t * HROWS, 3 * HROWS)]
        r = kv_tile(t, load_kv_operands(), view, 0)
        save_kv_operands(kv_operands(kv_tile(t + 1, kv_operands(r), view, HROWS)))
        return remaining - 1

    first_tile = lax.fori_loop(0, 3, pass1, 3)

    def q_products(t, o):
        return _Strassen(lambda i: _dot_nt(_unpack(wq_s[(i * 4 + o) * 64:(i * 4 + o + 1) * 64, :]),
                                           _unpack(h_s[_rows(t * HROWS + i * 64, 64), :])))

    def derived_params():
        wr8 = wr_v[...].astype(F32)
        wr = jnp.broadcast_to(jnp.concatenate([wr8[j:j + 1, :] for j in range(8)], axis=1), (8, D))
        scale = 1.0 + param(SCALE_B, 8)
        mod_s[:, SCALE_B * D:(SCALE_B + 1) * D] = scale
        router = scale * wr
        tables = (param(GATE_A, 8), router, scale * param(GATE_B, 8), param(SHIFT_B, 8) * param(GATE_B, 8))
        for k, row in enumerate(tables):
            for g in range(8):
                tile = jnp.concatenate([row[:, g * 128:(g + 1) * 128]] * 16, axis=0)
                col_s[k * D + g * 128:k * D + (g + 1) * 128, :] = tile.T
        base = ROUTER_SUMS * D
        mod_s[:, base:base + T] = jnp.broadcast_to(jnp.sum(router, axis=-1, keepdims=True), (8, T))
        mod_s[:, base + T:base + 2 * T] = jnp.broadcast_to(
            jnp.sum(param(SHIFT_B, 8) * wr, axis=-1, keepdims=True), (8, T))

    def column(k, ch):
        v = col_s[k * D + ch:k * D + ch + 128, :]
        return jnp.concatenate([v, v], axis=1)

    def features(r):
        return [_hedgehog(r[j // 2][(j % 2) * 64:(j % 2 + 1) * 64]) for j in range(4)]

    def save_features(phis):
        for j, phi in enumerate(phis):
            carry_s[j * 64:(j + 1) * 64, :] = pltpu.bitcast(phi, U32)

    def load_features():
        return [_unpack(carry_s[j * 64:(j + 1) * 64, :]) for j in range(4)]

    def attend(phis, o):
        heads = {}
        for j in (0, 2, 1, 3):
            nd = _dot(kv_s[2 * o + 8 * (j // 2) + j % 2].astype(BF), phis[j])
            heads[j] = jnp.concatenate(
                [nd[k * 32:(k + 1) * 32] * _recip(nd[64 + 8 * k:65 + 8 * k] + 1e-6) for k in range(2)], axis=0)
        return heads

    def stage_heads(dst, o, j, lo, hi):
        base = o * 64 + j * 32
        terms = _right_terms(lo[:, :U], lo[:, U:], hi[:, :U], hi[:, U:])
        dst[base:base + 32, 0:6 * U] = _pack(jnp.concatenate(terms[:6], axis=1))
        dst[base:base + 16, 6 * U:8 * U] = _pack(jnp.concatenate([terms[6][:32], terms[6][32:]], axis=1))

    def out_products(src, o):
        def product(i):
            if i < 6:
                b = src[:, i * U:(i + 1) * U]
            else:
                b = jnp.concatenate([src[k * 32:k * 32 + 16, (6 + c) * U:(7 + c) * U]
                                     for k in range(8) for c in range(2)], axis=0)
            return _dot(_unpack(wo_s[(i * 4 + o) * 64:(i * 4 + o + 1) * 64, :]), _unpack(b))
        return _Strassen(product)

    def residual(t, o, attn, sums):
        ys = []
        for half, a in enumerate(attn):
            ch = half * KH + o * 128
            ys.append(x_v[_rows(t * T, T), ch:ch + 128].T.astype(F32) + column(COL_GATE_A, ch) * a)
        if sums is None:
            shift = jnp.sum(_fold8(ys[0]) + _fold8(ys[1]), axis=0, keepdims=True) * (1.0 / 256)
            sums = (shift, 0.0, 0.0, 0.0)
        shift, s1, s2, s3 = sums
        for half, y in enumerate(ys):
            ch = half * KH + o * 128
            d = y - shift
            for k in range(2):
                d_s[_rows((2 * t + k) * D + ch, 128), :] = d[:, k * U:(k + 1) * U]
            s1, s2, s3 = s1 + _fold8(d), s2 + _fold8(d * d), s3 + _fold8(d * column(COL_ROUTER, ch))
        return shift, s1, s2, s3

    def route(t, sums, top):
        m1, i1, m2, i2 = top
        shift = sums[0]
        s1, s2, s3 = (jnp.sum(s, axis=0, keepdims=True) for s in sums[1:])
        delta = s1 * (1.0 / D)
        rstd = lax.rsqrt(jnp.maximum(s2 * (1.0 / D) - delta * delta, 0.0) + 1e-5)
        score = (s3 - delta * mod_s[0:1, ROUTER_SUMS * D:ROUTER_SUMS * D + T]) * rstd
        for k, v in enumerate((shift, delta, rstd)):
            for half in range(2):
                stat_s[_rows(((2 * t + half) * 3 + k) * 8, 8), :] = jnp.broadcast_to(
                    v[:, half * U:(half + 1) * U], (8, U))
        idx = lax.broadcasted_iota(I32, (1, T), 1) + t * T
        g1, g2 = score > m1, score > m2
        return (jnp.where(g1, score, m1), jnp.where(g1, idx, i1),
                jnp.where(g1, m1, jnp.where(g2, score, m2)), jnp.where(g1, i1, jnp.where(g2, idx, i2)))

    def stat(block, k, n):
        return jnp.concatenate([stat_s[_rows((block * 3 + k) * 8, 8), :]] * (n // 8), axis=0)

    def emit(t, ch):
        n = 256
        for half in range(2):
            shift, delta, rstd = (stat(2 * t + half, k, n) for k in range(3))
            d = d_s[_rows((2 * t + half) * D + ch, n), :]
            gain = rstd * col_s[COL_GAIN * D + ch:COL_GAIN * D + ch + n, :]
            res = ((d + shift) + col_s[COL_BIAS * D + ch:COL_BIAS * D + ch + n, :]) + (d - delta) * gain
            out_s[_rows(t * T + half * U, U), ch:ch + n] = res.T.astype(BF)

    def q_tile(t, phis, top, plans, current, previous, more=True):
        sums, emitted = None, 0
        for o, plan in enumerate(plans):
            qs = None
            if phis is not None and (o < 3 or more):
                qs = q_products(t, o + 1) if o < 3 else q_products(t + 1, 0)
            ws = out_products(previous, o)
            heads, staged = None, 0
            for item in plan.split():
                if item == "q":
                    qs.step()
                elif item == "w":
                    ws.step()
                    if ws.done:
                        sums = residual(t - 1, o, ws.result(), sums)
                elif item == "N":
                    heads = attend(phis, o)
                elif item == "c":
                    stage_heads(current, o, staged, heads[staged], heads[staged + 2])
                    staged += 1
                elif item == "E" and plans is not PLAN_Q_SECOND:
                    emit(t - 2, emitted * 256)
                    emitted += 1
                elif item == "s":
                    stage_out_weights(o)
                elif item == "M":
                    modulation((GATE_A + o) * D, D)
            phis = None if qs is None else features(qs.result())
        if sums is not None:
            top = route(t - 1, sums, top)
        if emitted:
            out_copy(t - 2).start()
        return phis, top

    wait(cp_wq, cp_wo, cp_mb, cp_mc, cp_wr)
    cp_wu.start()
    r = kv_tile(NT - 1, load_kv_operands(), h_s, (NT - 1) * HROWS, following=q_products(first_tile, 0))
    lowest = jnp.full((1, T), -jnp.inf, F32)
    zero = jnp.zeros((1, T), I32)
    top = (lowest, zero, lowest, zero)
    phis, top = q_tile(first_tile, features(r), top, PLAN_Q_FIRST, oa_s, ob_s)
    derived_params()
    phis, top = q_tile(first_tile + 1, phis, top, PLAN_Q_SECOND, ob_s, oa_s)
    save_features(phis)

    def pass2(i, carry):
        top, tile = carry
        pl.when(i == 1)(cp_wd.start)
        phis, top = q_tile(2 * i, load_features(), top, PLAN_Q, oa_s, ob_s)
        phis, top = q_tile(2 * i + 1, phis, top, PLAN_Q, ob_s, oa_s)
        save_features(phis)
        return top, tile + 2

    top, tile = lax.fori_loop(1, 3, pass2, (top, 2))
    wait(cp_wg, cp_wu, cp_wd)
    phis, top = q_tile(tile, load_features(), top, PLAN_Q, oa_s, ob_s)
    _, top = q_tile(tile + 1, phis, top, PLAN_Q_LAST, ob_s, oa_s, more=False)
    _, top = q_tile(tile + 2, None, top, PLAN_DRAIN, oa_s, ob_s)

    m1, i1, m2, i2 = top
    best = jnp.max(m1, axis=1, keepdims=True)
    ia = jnp.min(jnp.where(m1 == best, i1, S - 1), axis=1, keepdims=True)
    taken = i1 == ia
    rest, rest_idx = jnp.where(taken, m2, m1), jnp.where(taken, i2, i1)
    second = jnp.max(rest, axis=1, keepdims=True)
    ib = jnp.min(jnp.where(rest == second, rest_idx, S - 1), axis=1, keepdims=True)
    idx = (jnp.clip(ia[0, 0], 0, S - 1), jnp.clip(ib[0, 0], 0, S - 1))

    row16 = lax.broadcasted_iota(I32, (16, U), 0)
    lane16 = lax.broadcasted_iota(I32, (16, U), 1)
    xn_sel = 0.0
    for k in range(2):
        block = idx[k] // U
        xn = (d_s[_rows(block * D, D), :] - stat(block, 1, D)) * stat(block, 2, D)
        pick = jnp.where((row16 == k) & (lane16 == idx[k] % U), 1.0, 0.0).astype(BF)
        xn_sel = xn_sel + _dot_nt(pick, xn.astype(BF))
    vec_s[...] = _pack(xn_sel * param(SCALE_B, 16) + param(SHIFT_B, 16))
    out_copy(0).wait()
    hs = _unpack(vec_s[...])
    score = jnp.where(row16[:, 0:1] == 0, best, second) + mod_s[0:1, ROUTER_SUMS * D + T:ROUTER_SUMS * D + T + 1]
    gate = jax.nn.sigmoid(score)

    for g in range(4):
        emit(NT - 1, g * 256)
    y = jnp.zeros((16, D), F32)
    for j in range(F // FC):
        if j == 2:
            out_copy(NT - 1).start()
            out_copy(1).wait()
        gj = _dot(hs, wg_v[:, j * FC:(j + 1) * FC])
        uj = _dot(hs, wu_v[:, j * FC:(j + 1) * FC])
        y = y + _dot((gj * jax.nn.sigmoid(gj) * uj).astype(BF), wd_v[j * FC:(j + 1) * FC, 0:D])
    update = param(GATE_B, 16) * (y * gate)

    wait(*(out_copy(t) for t in range(2, NT)))
    row = lax.broadcasted_iota(I32, (16, D), 0)

    def patch(k):
        base = pl.multiple_of((idx[k] // 16) * 16, 16)
        block = out_s[pl.ds(base, 16), :].astype(F32)
        out_s[pl.ds(base, 16), :] = jnp.where(row == idx[k] - base, block + update[k:k + 1, :], block).astype(BF)
        return pltpu.make_async_copy(out_s.at[pl.ds(base, 16)], out_hbm.at[pl.ds(base, 16)], sem_p.at[k])

    patch_a, patch_b = patch(0), patch(1)
    patch_a.start()

    @pl.when(idx[0] // 16 != idx[1] // 16)
    def _():
        patch_b.start()
        patch_b.wait()

    patch_a.wait()


@jax.jit
def pallas_adaLN_cond__linear_kernel_hedgehog__moe_arch_mod__prompt_kernel(
        A_x, A_wqkv, A_w_phi, A_wo, B_x, B_w_r, B_w_gate, B_w_up, B_w_down, c, w_mod):
    del B_x
    hbm = pl.BlockSpec(memory_space=pl.ANY)
    out = pl.pallas_call(
        _kernel,
        out_shape=jax.ShapeDtypeStruct((S, D), BF),
        in_specs=[hbm] * 10,
        out_specs=hbm,
        scratch_shapes=[
            pltpu.VMEM((S, D), BF),
            pltpu.VMEM((D, 3 * D + PAD), BF),
            pltpu.VMEM((H * DH, DH), BF),
            pltpu.VMEM((D, D + PAD), BF),
            pltpu.VMEM((8, 128), BF),
            pltpu.VMEM((D, F + PAD), BF),
            pltpu.VMEM((D, F + PAD), BF),
            pltpu.VMEM((F, D + PAD), BF),
            pltpu.VMEM((1, D), BF),
            pltpu.VMEM((D, 6 * D + PAD), BF),
            pltpu.VMEM((7 * 512, KH), U32),
            pltpu.VMEM((7 * 256, KH), U32),
            pltpu.VMEM((7 * 256, KH), U32),
            pltpu.VMEM((NT * HROWS, KH), U32),
            pltpu.VMEM((NPAIR, 80, 128), F32),
            pltpu.VMEM((8, 6 * D + 2 * T), F32),
            pltpu.VMEM((4 * D, 128), F32),
            pltpu.VMEM((2 * NT * D, U), F32),
            pltpu.VMEM((2 * NT * 3 * 8, U), F32),
            pltpu.VMEM((S, D), BF),
            pltpu.VMEM((8 * 64, 128), U32),
            pltpu.VMEM((KH // 2, 8 * U), U32),
            pltpu.VMEM((KH // 2, 8 * U), U32),
            pltpu.VMEM((8, D), U32),
            pltpu.VMEM((T, D), F32),
            pltpu.VMEM((384, T), U32),
            pltpu.SemaphoreType.DMA((10,)),
            pltpu.SemaphoreType.DMA((4,)),
            pltpu.SemaphoreType.DMA((4,)),
            pltpu.SemaphoreType.DMA((4,)),
            pltpu.SemaphoreType.DMA((NT,)),
            pltpu.SemaphoreType.DMA((NT,)),
            pltpu.SemaphoreType.DMA((2,)),
        ],
        compiler_params=pltpu.CompilerParams(
            vmem_limit_bytes=110 * 2**20,
            flags={"XLA_TPU_EVENLY_DISTRIBUTE_CRITICAL_NODES": True}),
        name="fused_block",
    )(A_x.reshape(S, D), A_wqkv, A_w_phi.reshape(H * DH, DH), A_wo, B_w_r.reshape(8, 128),
      B_w_gate, B_w_up, B_w_down, c, w_mod)
    return out.reshape(1, S, D)
```

```python
import math

import jax
import jax.numpy as jnp
from jax import lax
import jax.experimental.pallas as pl
import jax.experimental.pallas.tpu as pltpu

S, D, H, DH, F = 2048, 1024, 32, 32, 3584
U = 128
T = 2 * U
NT = S // T
KH = D // 2
NPAIR = H // 2
HROWS = 7 * U // 2
PAD = 128
FC = F // 2
LN_ROWS = 32
LOG2E = math.log2(math.e)
BF, F32, U32, I32 = jnp.bfloat16, jnp.float32, jnp.uint32, jnp.int32

SHIFT_A, SCALE_A, GATE_A, SHIFT_B, SCALE_B, GATE_B, ROUTER_SUMS = range(7)
COL_GATE_A, COL_ROUTER, COL_GAIN, COL_BIAS = range(4)

PLAN_FIRST = ("p p p W s p p p p", "W s p p p N p p p p", "p N W s p p p p p p",
              "X L p p N p p p p p", "p p p p p p p N")
PLAN_KV_A = ("p p p N p p p p",) * 4
PLAN_KV_B = ("p N p p p p p p",) * 2 + ("p p N p p p p p", "p p p N p p p p")
PLAN_KV_LAST = ("s p p N p p p p p o", "p N p p p p s p p o", "p s p p N p p p p o", "s p p p N p p p p o")
PLAN_Q_FIRST = ("q q N c c q M q q q q",) * 4
PLAN_Q_SECOND = ("w w w w w w w q N c c q q q q q q",) * 2 + (
    "w w w w w w w q q q N c c q q q q", "w w w w w w N c c w q q q q q q q")
PLAN_Q = ("w w w w w N c c w w q q q q q q q E",) * 4
PLAN_Q_LATE = PLAN_Q[:1] + ("w w w w w w w q q N c c q q q q q E",) * 3
PLAN_Q_LAST = PLAN_Q_LATE[1:] + ("w w w w w N c c w w E",)
PLAN_DRAIN = ("E w w w w w w w E", "w w w w w w w E", "w w w w w w w E", "w w w w w w w")


def _dot(a, b):
    return jnp.dot(a, b, preferred_element_type=F32)


def _dot_nt(a, b):
    return lax.dot_general(a, b, (((1,), (1,)), ((), ())), preferred_element_type=F32)


def _pack(v):
    return pltpu.bitcast(v.astype(BF), U32)


def _unpack(v):
    return pltpu.bitcast(v, BF)


def _recip(v):
    return pl.reciprocal(v, approx=False, full_range=False)


def _rows(start, size):
    return pl.ds(start if isinstance(start, int) else pl.multiple_of(start, 8), size)


def _normalize(v):
    centered = v - jnp.mean(v, axis=-1, keepdims=True)
    var = jnp.mean(centered * centered, axis=-1, keepdims=True)
    return centered * lax.rsqrt(var + 1e-5)


def _fold8(v, op=jnp.add):
    parts = [v[i:i + 8] for i in range(0, v.shape[0], 8)]
    while len(parts) > 1:
        parts = [op(parts[i], parts[i + 1]) for i in range(0, len(parts), 2)]
    return parts[0]


def _per_head(v, op):
    r = _fold8(v, op)
    r = op(r, pltpu.roll(r, 4, 0))
    return op(r, pltpu.roll(r, 2, 0))


def _hedgehog(p):
    def spread(v):
        return jnp.concatenate([v] * 8, axis=0)

    pos = jnp.exp2(p - spread(_per_head(p, jnp.maximum)))
    neg = jnp.exp2(spread(_per_head(p, jnp.minimum)) - p)
    pos = pos * spread(_recip(_per_head(pos, jnp.add)))
    neg = neg * spread(_recip(_per_head(neg, jnp.add)))
    return jnp.concatenate([pos, neg], axis=0)


def _left_terms(a11, a12, a21, a22):
    return a11 + a22, a21 + a22, a11, a22, a11 + a12, a21 - a11, a12 - a22


def _right_terms(b11, b12, b21, b22):
    return b11 + b22, b11, b12 - b22, b21 - b11, b22, b11 + b12, b21 + b22


class _Strassen:
    _SCHEDULE = ((0, ((0, 1), (3, 1))), (1, ((2, 1), (3, -1))), (2, ((1, 1), (3, 1))), (5, ((3, 1),)),
                 (3, ((0, 1), (2, 1))), (4, ((0, -1), (1, 1))), (6, ((0, 1),)))

    def __init__(self, product):
        self._product = product
        self._todo = list(self._SCHEDULE)
        self._c = [None] * 4

    @property
    def done(self):
        return not self._todo

    def step(self):
        i, uses = self._todo.pop(0)
        m = self._product(i)
        for k, sign in uses:
            if self._c[k] is None:
                self._c[k] = m
            else:
                self._c[k] = self._c[k] + m if sign > 0 else self._c[k] - m

    def result(self):
        assert self.done
        return jnp.concatenate(self._c[:2], axis=1), jnp.concatenate(self._c[2:], axis=1)


def _kernel(x_hbm, wqkv_hbm, wphi_hbm, wo_hbm, wr_hbm, wg_hbm, wu_hbm, wd_hbm, c_hbm, wmod_hbm,
            out_hbm,
            x_v, wqkv_v, wphi_v, wo_v, wr_v, wg_v, wu_v, wd_v, c_v, wmod_v,
            wkv_s, wq_s, wo_s, h_s, kv_s, mod_s, col_s, x1_s, stat_s, out_s, fmap_s,
            oa_s, ob_s, vec_s, xn_s, carry_s, raw_s, z_s,
            sem_w, sem_m, sem_k, sem_v, sem_x, sem_o, sem_p):
    def wcopy(i, src, dst):
        return pltpu.make_async_copy(src, dst, sem_w.at[i])

    cp_c = wcopy(0, c_hbm, c_v)
    cp_phi = wcopy(1, wphi_hbm, wphi_v)
    cp_wr = wcopy(2, wr_hbm, wr_v)
    cp_wq = wcopy(3, wqkv_hbm.at[:, 0:D], wqkv_v.at[:, 0:D])
    cp_mb = wcopy(4, wmod_hbm.at[:, 2 * D:4 * D], wmod_v.at[:, 2 * D:4 * D])
    cp_mc = wcopy(5, wmod_hbm.at[:, 4 * D:6 * D], wmod_v.at[:, 4 * D:6 * D])
    cp_wo = wcopy(6, wo_hbm, wo_v.at[:, 0:D])
    cp_wg = wcopy(7, wg_hbm, wg_v.at[:, 0:F])
    cp_wu = wcopy(8, wu_hbm, wu_v.at[:, 0:F])
    cp_wd = wcopy(9, wd_hbm, wd_v.at[:, 0:D])

    def mod_copy(j):
        cols = pl.ds(j * 512 if isinstance(j, int) else pl.multiple_of(j * 512, 512), 512)
        return pltpu.make_async_copy(wmod_hbm.at[:, cols], wmod_v.at[:, cols], sem_m.at[j])

    def kv_copies(o):
        ck, cv = pl.ds(D + o * 256, 256), pl.ds(2 * D + o * 256, 256)
        return (pltpu.make_async_copy(wqkv_hbm.at[:, ck], wqkv_v.at[:, ck], sem_k.at[o]),
                pltpu.make_async_copy(wqkv_hbm.at[:, cv], wqkv_v.at[:, cv], sem_v.at[o]))

    def x_copy(t):
        rows = _rows(t * T, T)
        return pltpu.make_async_copy(x_hbm.at[rows], x_v.at[rows], sem_x.at[t])

    def out_copy(t):
        rows = _rows(t * T, T)
        return pltpu.make_async_copy(out_s.at[rows], out_hbm.at[rows], sem_o.at[t])

    def start(*copies):
        for cp in copies:
            cp.start()

    def wait(*copies):
        for cp in copies:
            cp.wait()

    def fold(col0, g):
        return _dot_nt(_unpack(fmap_s[g * 64:(g + 1) * 64, :]),
                       wqkv_v[:, col0 + g * 128:col0 + (g + 1) * 128]) * LOG2E

    def stage_left(dst, o, upper, lower):
        n = upper.shape[0] // 2
        for i, a in enumerate(_left_terms(upper[:, :KH], upper[:, KH:], lower[:, :KH], lower[:, KH:])):
            dst[(i * 4 + o) * n:(i * 4 + o + 1) * n, :] = _pack(a)

    def stage_kv_weights(o):
        blocks = []
        for g in (2 * o, 2 * o + 1):
            fk = fold(D, g)
            fv = wqkv_v[:, 2 * D + g * 128:2 * D + (g + 1) * 128].T.astype(F32)
            blocks.append(jnp.concatenate([fk[:64], fv[:64], fk[64:], fv[64:]], axis=0))
        stage_left(wkv_s, o, *blocks)

    def stage_q_weights(o):
        stage_left(wq_s, o, fold(0, o), fold(0, o + 4))

    def stage_out_weights(o):
        stage_left(wo_s, o, wo_v[:, o * 128:(o + 1) * 128].T.astype(F32),
                   wo_v[:, KH + o * 128:KH + (o + 1) * 128].T.astype(F32))

    def param(k, n):
        return jnp.concatenate([mod_s[:, k * D:(k + 1) * D]] * (n // 8), axis=0)

    def modulation(col0, n):
        mod_s[:, col0:col0 + n] = _dot(_unpack(vec_s[...]), wmod_v[:, col0:col0 + n])[0:8]

    def first_norm(t, dst, base, normalized=None):
        for r0 in range(0, U, LN_ROWS):
            h = []
            for half in range(2):
                rows = _rows(t * T + half * U + r0, LN_ROWS)
                xn = _normalize(x_v[rows, :].astype(F32)) if normalized is None else normalized[rows, :]
                h.append(xn * param(SCALE_A, LN_ROWS) + param(SHIFT_A, LN_ROWS))
            for i, b in enumerate(_right_terms(h[0][:, :KH], h[1][:, :KH], h[0][:, KH:], h[1][:, KH:])):
                dst[base + i * 64 + r0 // 2:base + i * 64 + (r0 + LN_ROWS) // 2, :] = _pack(b)

    def kv_products(src, base, o):
        return _Strassen(lambda i: _dot_nt(_unpack(wkv_s[(i * 4 + o) * 128:(i * 4 + o + 1) * 128, :]),
                                           _unpack(src[base + i * 64:base + (i + 1) * 64, :])))

    def kv_pairs(block):
        return [(block[j * 128 + 64:(j + 1) * 128].astype(BF), _hedgehog(block[j * 128:j * 128 + 64]).astype(BF))
                for j in range(2)]

    def kv_operands(r):
        return kv_pairs(r[0]) + kv_pairs(r[1])

    def save_kv_operands(r):
        raw_s[...] = r[0]
        for j, (v, phi) in enumerate(kv_pairs(r[1])):
            carry_s[j * 64:(j + 1) * 64, :] = pltpu.bitcast(phi, U32)
            carry_s[128 + j * 32:128 + (j + 1) * 32, :] = pltpu.bitcast(v, U32)

    def load_kv_operands():
        done = [(_unpack(carry_s[128 + j * 32:128 + (j + 1) * 32, :]), _unpack(carry_s[j * 64:(j + 1) * 64, :]))
                for j in range(2)]
        return kv_pairs(raw_s[...]) + done

    def accumulate_kv(ops, o, first=False, last=False):
        ones = jnp.ones((16, T), BF)
        for j, (v, phi) in enumerate(ops):
            acc = _dot_nt(jnp.concatenate([v, ones], axis=0), phi)
            if not first:
                acc = acc + kv_s[4 * o + j]
            if last:
                z_s[4 * o + j] = jnp.concatenate([acc[64:72]] * 16, axis=0).T
                row_head = lax.broadcasted_iota(I32, (80, 128), 0) // DH
                lane_head = lax.broadcasted_iota(I32, (80, 128), 1) % 2
                acc = jnp.where(row_head == lane_head, acc, 0.0)
            kv_s[4 * o + j] = acc

    start(cp_phi, cp_c, *kv_copies(0), x_copy(0))
    lax.fori_loop(0, 4, lambda j, _: mod_copy(j).start(), None)
    cp_c.wait()
    cv = c_v[...].astype(F32)
    vec_s[...] = _pack(jnp.broadcast_to(cv * jax.nn.sigmoid(cv), (16, D)))
    cp_phi.wait()
    repeat = ((lax.broadcasted_iota(I32, (128, DH), 0) % 64) // 2
              == lax.broadcasted_iota(I32, (128, DH), 1)).astype(BF)
    block_row = lax.broadcasted_iota(I32, (128, 128), 0)
    same_head = 2 * (block_row // 64) + block_row % 2 == lax.broadcasted_iota(I32, (128, 128), 1) // DH
    for g in range(8):
        full = _dot_nt(repeat, wphi_v[g * 128:(g + 1) * 128, :])
        fmap_s[g * 64:(g + 1) * 64, :] = _pack(jnp.where(same_head, full, 0.0))
    wait(*kv_copies(0))
    stage_kv_weights(0)
    x_copy(0).wait()
    xn_s[...] = _normalize(x_v[0:T, :].astype(F32))
    for j in range(4):
        mod_copy(j).wait()
        if j == 2:
            start(*kv_copies(1), *kv_copies(2))
        elif j == 3:
            start(*kv_copies(3))
        modulation(j * 512, 512)
    mod_s[:, SCALE_A * D:(SCALE_A + 1) * D] += 1.0
    first_norm(0, h_s, 0, normalized=xn_s)

    ops = None
    for o, plan in enumerate(PLAN_FIRST):
        products = kv_products(h_s, (o // 4) * HROWS, o % 4)
        for item in plan.split():
            if item == "p":
                products.step()
            elif item == "W":
                wait(*kv_copies(o + 1))
                if o == 0:
                    x_copy(1).start()
            elif item == "X":
                x_copy(1).wait()
                start(x_copy(2), x_copy(3), cp_wr)
            elif item == "s":
                stage_kv_weights(o + 1)
            elif item == "L":
                first_norm(1, h_s, HROWS)
            else:
                accumulate_kv(ops, o - 1, first=True)
        if o < 4:
            ops = kv_operands(products.result())
    save_kv_operands(products.result())

    def kv_tile(t, ops, src, base, plans, following=None):
        last = following is not None
        if not last:
            first_norm(t + 1, src, base + HROWS)
        for o, plan in enumerate(plans):
            if o < 3:
                products = kv_products(src, base, o + 1)
            else:
                products = following if last else kv_products(src, base + HROWS, 0)
            for item in plan.split():
                if item == "p":
                    products.step()
                elif item == "s":
                    stage_q_weights(o)
                elif item == "o":
                    stage_out_weights(o)
                else:
                    accumulate_kv(ops, o, last=last)
            if o < 3:
                ops = kv_operands(products.result())
        return products.result()

    def pass1(i, remaining):
        t = 2 * i + 1
        wait(x_copy(t + 1), x_copy(t + 2))
        pl.when(i == 0)(lambda: start(*(x_copy(k) for k in range(4, NT)), cp_wq, cp_wo))
        pl.when(i == 1)(lambda: start(cp_mb, cp_mc, cp_wg))
        view = h_s.at[_rows(t * HROWS, 3 * HROWS)]
        r = kv_tile(t, load_kv_operands(), view, 0, PLAN_KV_A)
        save_kv_operands(kv_tile(t + 1, kv_operands(r), view, HROWS, PLAN_KV_B))
        return remaining - 1

    first_tile = lax.fori_loop(0, 3, pass1, 3)

    def q_products(t, o):
        return _Strassen(lambda i: _dot_nt(_unpack(wq_s[(i * 4 + o) * 64:(i * 4 + o + 1) * 64, :]),
                                           _unpack(h_s[_rows(t * HROWS + i * 64, 64), :])))

    def derived_params():
        wr8 = wr_v[...].astype(F32)
        wr = jnp.broadcast_to(jnp.concatenate([wr8[j:j + 1, :] for j in range(8)], axis=1), (8, D))
        scale = 1.0 + param(SCALE_B, 8)
        mod_s[:, SCALE_B * D:(SCALE_B + 1) * D] = scale
        router = scale * wr
        tables = (param(GATE_A, 8), router, scale * param(GATE_B, 8), param(SHIFT_B, 8) * param(GATE_B, 8))
        for k, row in enumerate(tables):
            for g in range(8):
                tile = jnp.concatenate([row[:, g * 128:(g + 1) * 128]] * 16, axis=0)
                col_s[k * D + g * 128:k * D + (g + 1) * 128, :] = tile.T
        base = ROUTER_SUMS * D
        mod_s[:, base:base + T] = jnp.broadcast_to(jnp.sum(router, axis=-1, keepdims=True), (8, T))
        mod_s[:, base + T:base + 2 * T] = jnp.broadcast_to(
            jnp.sum(param(SHIFT_B, 8) * wr, axis=-1, keepdims=True), (8, T))

    def column(k, ch):
        v = col_s[k * D + ch:k * D + ch + 128, :]
        return jnp.concatenate([v, v], axis=1)

    def feature_pairs(block, p0):
        out = []
        for j in range(2):
            phi = _hedgehog(block[j * 64:(j + 1) * 64])
            z = z_s[p0 + j]
            inv = _recip(_per_head(phi * jnp.concatenate([z, z], axis=1), jnp.add) + 1e-6)
            out.append((phi.astype(BF), inv))
        return out

    def features(r, o):
        return feature_pairs(r[0], 2 * o) + feature_pairs(r[1], 2 * o + 8)

    def save_features(r):
        raw_s[0:128, :] = r[0]
        for j, (phi, inv) in enumerate(feature_pairs(r[1], 8)):
            carry_s[j * 64:(j + 1) * 64, :] = pltpu.bitcast(phi, U32)
            raw_s[128 + 8 * j:136 + 8 * j, :] = inv

    def load_features():
        done = [(_unpack(carry_s[j * 64:(j + 1) * 64, :]), raw_s[128 + 8 * j:136 + 8 * j, :]) for j in range(2)]
        return feature_pairs(raw_s[0:128, :], 0) + done

    def attend(phis, o):
        heads = {}
        for j in (0, 2, 1, 3):
            phi, inv = phis[j]
            num = _dot(kv_s[2 * o + 8 * (j // 2) + j % 2, 0:64, :].astype(BF), phi)
            heads[j] = jnp.concatenate([num[k * DH:(k + 1) * DH] * inv[k:k + 1] for k in range(2)], axis=0)
        return heads

    def stage_heads(dst, o, j, lo, hi):
        base = o * 64 + j * 32
        terms = _right_terms(lo[:, :U], lo[:, U:], hi[:, :U], hi[:, U:])
        dst[base:base + 32, 0:6 * U] = _pack(jnp.concatenate(terms[:6], axis=1))
        dst[base:base + 16, 6 * U:8 * U] = _pack(jnp.concatenate([terms[6][:32], terms[6][32:]], axis=1))

    def out_products(src, o):
        def product(i):
            if i < 6:
                b = src[:, i * U:(i + 1) * U]
            else:
                b = jnp.concatenate([src[k * 32:k * 32 + 16, (6 + c) * U:(7 + c) * U]
                                     for k in range(8) for c in range(2)], axis=0)
            return _dot(_unpack(wo_s[(i * 4 + o) * 64:(i * 4 + o + 1) * 64, :]), _unpack(b))
        return _Strassen(product)

    def residual(t, o, attn, sums):
        ys = []
        for half, a in enumerate(attn):
            ch = half * KH + o * 128
            ys.append(x_v[_rows(t * T, T), ch:ch + 128].T.astype(F32) + column(COL_GATE_A, ch) * a)
        if sums is None:
            shift = jnp.sum(_fold8(ys[0]) + _fold8(ys[1]), axis=0, keepdims=True) * (1.0 / 256)
            sums = (shift, 0.0, 0.0, 0.0)
        shift, s1, s2, s3 = sums
        for half, y in enumerate(ys):
            ch = half * KH + o * 128
            d = y - shift
            for k in range(2):
                x1_s[_rows((2 * t + k) * D + ch, 128), :] = y[:, k * U:(k + 1) * U]
            s1, s2, s3 = s1 + _fold8(d), s2 + _fold8(d * d), s3 + _fold8(d * column(COL_ROUTER, ch))
        return shift, s1, s2, s3

    def route(t, sums, top):
        m1, i1, m2, i2 = top
        shift = sums[0]
        s1, s2, s3 = (jnp.sum(s, axis=0, keepdims=True) for s in sums[1:])
        delta = s1 * (1.0 / D)
        rstd = lax.rsqrt(jnp.maximum(s2 * (1.0 / D) - delta * delta, 0.0) + 1e-5)
        score = (s3 - delta * mod_s[0:1, ROUTER_SUMS * D:ROUTER_SUMS * D + T]) * rstd
        for k, v in enumerate((shift + delta, rstd)):
            for half in range(2):
                stat_s[_rows(((2 * t + half) * 2 + k) * 8, 8), :] = jnp.broadcast_to(
                    v[:, half * U:(half + 1) * U], (8, U))
        idx = lax.broadcasted_iota(I32, (1, T), 1) + t * T
        g1, g2 = score > m1, score > m2
        return (jnp.where(g1, score, m1), jnp.where(g1, idx, i1),
                jnp.where(g1, m1, jnp.where(g2, score, m2)), jnp.where(g1, i1, jnp.where(g2, idx, i2)))

    def stat(block, k, n):
        return jnp.concatenate([stat_s[_rows((block * 2 + k) * 8, 8), :]] * (n // 8), axis=0)

    def emit(t, ch):
        n = 256
        for half in range(2):
            mean, rstd = (stat(2 * t + half, k, n) for k in range(2))
            x1 = x1_s[_rows((2 * t + half) * D + ch, n), :]
            gain = rstd * col_s[COL_GAIN * D + ch:COL_GAIN * D + ch + n, :]
            res = (x1 + col_s[COL_BIAS * D + ch:COL_BIAS * D + ch + n, :]) + (x1 - mean) * gain
            out_s[_rows(t * T + half * U, U), ch:ch + n] = res.T.astype(BF)

    def q_tile(t, phis, top, plans, current, previous, more=True):
        sums, emitted = None, 0
        for o, plan in enumerate(plans):
            qs = None
            if phis is not None and (o < 3 or more):
                qs = q_products(t, o + 1) if o < 3 else q_products(t + 1, 0)
            ws = out_products(previous, o)
            heads, staged = None, 0
            for item in plan.split():
                if item == "q":
                    qs.step()
                elif item == "w":
                    ws.step()
                    if ws.done:
                        sums = residual(t - 1, o, ws.result(), sums)
                elif item == "N":
                    heads = attend(phis, o)
                elif item == "c":
                    stage_heads(current, o, staged, heads[staged], heads[staged + 2])
                    staged += 1
                elif item == "E":
                    emit(t - 2, emitted * 256)
                    emitted += 1
                elif item == "M":
                    modulation((GATE_A + o) * D, D)
            if qs is not None:
                phis = features(qs.result(), o + 1) if o < 3 else qs.result()
        if sums is not None:
            top = route(t - 1, sums, top)
        if emitted:
            out_copy(t - 2).start()
        return phis, top

    wait(cp_wq, cp_wo, cp_mb, cp_mc, cp_wr)
    cp_wu.start()
    r = kv_tile(NT - 1, load_kv_operands(), h_s, (NT - 1) * HROWS, PLAN_KV_LAST,
                following=q_products(first_tile, 0))
    lowest = jnp.full((1, T), -jnp.inf, F32)
    zero = jnp.zeros((1, T), I32)
    top = (lowest, zero, lowest, zero)
    r, top = q_tile(first_tile, features(r, 0), top, PLAN_Q_FIRST, oa_s, ob_s)
    derived_params()
    r, top = q_tile(first_tile + 1, features(r, 0), top, PLAN_Q_SECOND, ob_s, oa_s)
    save_features(r)

    def pass2(i, carry):
        top, tile = carry
        pl.when(i == 2)(cp_wd.start)
        r, top = q_tile(2 * i - 2, load_features(), top, PLAN_Q, oa_s, ob_s)
        r, top = q_tile(2 * i - 1, features(r, 0), top, PLAN_Q, ob_s, oa_s)
        save_features(r)
        return top, tile + 2

    top, tile = lax.fori_loop(2, 4, pass2, (top, 2))
    wait(cp_wg, cp_wu, cp_wd)
    r, top = q_tile(tile, load_features(), top, PLAN_Q_LATE, oa_s, ob_s)
    _, top = q_tile(tile + 1, features(r, 0), top, PLAN_Q_LAST, ob_s, oa_s, more=False)
    _, top = q_tile(tile + 2, None, top, PLAN_DRAIN, oa_s, ob_s)

    m1, i1, m2, i2 = top
    best = jnp.max(m1, axis=1, keepdims=True)
    ia = jnp.min(jnp.where(m1 == best, i1, S - 1), axis=1, keepdims=True)
    taken = i1 == ia
    rest, rest_idx = jnp.where(taken, m2, m1), jnp.where(taken, i2, i1)
    second = jnp.max(rest, axis=1, keepdims=True)
    ib = jnp.min(jnp.where(rest == second, rest_idx, S - 1), axis=1, keepdims=True)
    idx = (jnp.clip(ia[0, 0], 0, S - 1), jnp.clip(ib[0, 0], 0, S - 1))

    for g in range(4):
        emit(NT - 1, g * 256)
    out_copy(NT - 1).start()
    out_copy(0).wait()

    row16 = lax.broadcasted_iota(I32, (16, U), 0)
    lane16 = lax.broadcasted_iota(I32, (16, U), 1)
    xn_sel = 0.0
    for k in range(2):
        block = idx[k] // U
        xn = (x1_s[_rows(block * D, D), :] - stat(block, 0, D)) * stat(block, 1, D)
        pick = jnp.where((row16 == k) & (lane16 == idx[k] % U), 1.0, 0.0).astype(BF)
        xn_sel = xn_sel + _dot_nt(pick, xn.astype(BF))
    hs = (xn_sel * param(SCALE_B, 16) + param(SHIFT_B, 16)).astype(BF)
    score = jnp.where(row16[:, 0:1] == 0, best, second) + mod_s[0:1, ROUTER_SUMS * D + T:ROUTER_SUMS * D + T + 1]
    gate = jax.nn.sigmoid(score)

    y = jnp.zeros((16, D), F32)
    for j in range(F // FC):
        gj = _dot(hs, wg_v[:, j * FC:(j + 1) * FC])
        uj = _dot(hs, wu_v[:, j * FC:(j + 1) * FC])
        y = y + _dot((gj * jax.nn.sigmoid(gj) * uj).astype(BF), wd_v[j * FC:(j + 1) * FC, 0:D])
    update = param(GATE_B, 16) * (y * gate)

    wait(*(out_copy(t) for t in range(1, NT)))
    row = lax.broadcasted_iota(I32, (16, D), 0)

    def patch(k):
        base = pl.multiple_of((idx[k] // 16) * 16, 16)
        block = out_s[pl.ds(base, 16), :].astype(F32)
        out_s[pl.ds(base, 16), :] = jnp.where(row == idx[k] - base, block + update[k:k + 1, :], block).astype(BF)
        return pltpu.make_async_copy(out_s.at[pl.ds(base, 16)], out_hbm.at[pl.ds(base, 16)], sem_p.at[k])

    patch_a, patch_b = patch(0), patch(1)
    patch_a.start()

    @pl.when(idx[0] // 16 != idx[1] // 16)
    def _():
        patch_b.start()
        patch_b.wait()

    patch_a.wait()


@jax.jit
def pallas_adaLN_cond__linear_kernel_hedgehog__moe_arch_mod__prompt_kernel(
        A_x, A_wqkv, A_w_phi, A_wo, B_x, B_w_r, B_w_gate, B_w_up, B_w_down, c, w_mod):
    del B_x
    hbm = pl.BlockSpec(memory_space=pl.ANY)
    out = pl.pallas_call(
        _kernel,
        out_shape=jax.ShapeDtypeStruct((S, D), BF),
        in_specs=[hbm] * 10,
        out_specs=hbm,
        scratch_shapes=[
            pltpu.VMEM((S, D), BF),
            pltpu.VMEM((D, 3 * D + PAD), BF),
            pltpu.VMEM((H * DH, DH), BF),
            pltpu.VMEM((D, D + PAD), BF),
            pltpu.VMEM((8, 128), BF),
            pltpu.VMEM((D, F + PAD), BF),
            pltpu.VMEM((D, F + PAD), BF),
            pltpu.VMEM((F, D + PAD), BF),
            pltpu.VMEM((1, D), BF),
            pltpu.VMEM((D, 6 * D + PAD), BF),
            pltpu.VMEM((7 * 512, KH), U32),
            pltpu.VMEM((7 * 256, KH), U32),
            pltpu.VMEM((7 * 256, KH), U32),
            pltpu.VMEM((NT * HROWS, KH), U32),
            pltpu.VMEM((NPAIR, 80, 128), F32),
            pltpu.VMEM((8, 6 * D + 2 * T), F32),
            pltpu.VMEM((4 * D, 128), F32),
            pltpu.VMEM((2 * NT * D, U), F32),
            pltpu.VMEM((2 * NT * 2 * 8, U), F32),
            pltpu.VMEM((S, D), BF),
            pltpu.VMEM((8 * 64, 128), U32),
            pltpu.VMEM((KH // 2, 8 * U), U32),
            pltpu.VMEM((KH // 2, 8 * U), U32),
            pltpu.VMEM((8, D), U32),
            pltpu.VMEM((T, D), F32),
            pltpu.VMEM((192, T), U32),
            pltpu.VMEM((256, T), F32),
            pltpu.VMEM((NPAIR, 128, U), F32),
            pltpu.SemaphoreType.DMA((10,)),
            pltpu.SemaphoreType.DMA((4,)),
            pltpu.SemaphoreType.DMA((4,)),
            pltpu.SemaphoreType.DMA((4,)),
            pltpu.SemaphoreType.DMA((NT,)),
            pltpu.SemaphoreType.DMA((NT,)),
            pltpu.SemaphoreType.DMA((2,)),
        ],
        compiler_params=pltpu.CompilerParams(
            vmem_limit_bytes=110 * 2**20,
            flags={"XLA_TPU_EVENLY_DISTRIBUTE_CRITICAL_NODES": True}),
        name="fused_block",
    )(A_x.reshape(S, D), A_wqkv, A_w_phi.reshape(H * DH, DH), A_wo, B_w_r.reshape(8, 128),
      B_w_gate, B_w_up, B_w_down, c, w_mod)
    return out.reshape(1, S, D)
```

```python
import math

import jax
import jax.numpy as jnp
from jax import lax
import jax.experimental.pallas as pl
import jax.experimental.pallas.tpu as pltpu

S, D, H, DH, F = 2048, 1024, 32, 32, 3584
U = 128
T = 2 * U
NT = S // T
KH = D // 2
NPAIR = H // 2
HROWS = 7 * U // 2
PAD = 128
FC = F // 2
LN_ROWS = 32
LOG2E = math.log2(math.e)
BF, F32, U32, I32 = jnp.bfloat16, jnp.float32, jnp.uint32, jnp.int32

SHIFT_A, SCALE_A, GATE_A, SHIFT_B, SCALE_B, GATE_B, ROUTER_SUMS = range(7)
COL_GATE_A, COL_ROUTER, COL_GAIN, COL_BIAS = range(4)

PLAN_FIRST = ("p p p p W s p", "p p W s p N p p p p", "p N p W s p p p p p",
              "X L p p N p p p p p", "p p p p p p p N")
PLAN_KV_A = ("p p p N p p p p",) * 4
PLAN_KV_B = ("p N p p p p p p",) * 2 + ("p p N p p p p p", "p p p N p p p p")
PLAN_KV_LAST = ("s p p N p p p p p o", "p N p p p p s p p o", "p s p p N p p p p o", "s p p p N p p p p o")
PLAN_Q_FIRST = ("q q N c c q M q q q q",) * 4
PLAN_Q_SECOND = ("w w w w w w w q N c c q q q q q q",) * 2 + (
    "w w w w w w w q q q N c c q q q q", "w w w w w w N c c w q q q q q q q")
PLAN_Q = ("w w w w w N c c w w q q q q q q q E",) * 4
PLAN_Q_LATE = PLAN_Q[:1] + ("w w w w w w w q q N c c q q q q q E",) * 3
PLAN_Q_LAST = PLAN_Q_LATE[1:] + ("w w w w w N c c w w E",)
PLAN_DRAIN = ("E w w w w w w w E", "w w w w w w w E", "w w w w w w w E", "w w w w w w w")
ORDER_FIRST = (6, 2, 1, 3, 4, 5, 7)
ORDER_KV = (1, 2, 3, 6, 4, 5, 7)
ORDER_Q = (4, 3, 2, 5, 1, 6, 7)
ORDER_OUT = (4, 7, 3, 1, 5, 2, 6)


def _dot(a, b):
    return jnp.dot(a, b, preferred_element_type=F32)


def _dot_nt(a, b):
    return lax.dot_general(a, b, (((1,), (1,)), ((), ())), preferred_element_type=F32)


def _pack(v):
    return pltpu.bitcast(v.astype(BF), U32)


def _unpack(v):
    return pltpu.bitcast(v, BF)


def _recip(v):
    return pl.reciprocal(v, approx=False, full_range=False)


def _rows(start, size):
    return pl.ds(start if isinstance(start, int) else pl.multiple_of(start, 8), size)


def _normalize(v):
    centered = v - jnp.mean(v, axis=-1, keepdims=True)
    var = jnp.mean(centered * centered, axis=-1, keepdims=True)
    return centered * lax.rsqrt(var + 1e-5)


def _fold8(v, op=jnp.add):
    parts = [v[i:i + 8] for i in range(0, v.shape[0], 8)]
    while len(parts) > 1:
        parts = [op(parts[i], parts[i + 1]) for i in range(0, len(parts), 2)]
    return parts[0]


def _per_head(v, op):
    r = _fold8(v, op)
    r = op(r, pltpu.roll(r, 4, 0))
    return op(r, pltpu.roll(r, 2, 0))


def _hedgehog(p):
    def spread(v):
        return jnp.concatenate([v] * 8, axis=0)

    pos = jnp.exp2(p - spread(_per_head(p, jnp.maximum)))
    neg = jnp.exp2(spread(_per_head(p, jnp.minimum)) - p)
    pos = pos * spread(_recip(_per_head(pos, jnp.add)))
    neg = neg * spread(_recip(_per_head(neg, jnp.add)))
    return jnp.concatenate([pos, neg], axis=0)


def _left_terms(a11, a12, a21, a22):
    return a11 + a22, a21 + a22, a11, a22, a11 + a12, a21 - a11, a12 - a22


def _right_terms(b11, b12, b21, b22):
    return b11 + b22, b11, b12 - b22, b21 - b11, b22, b11 + b12, b21 + b22


class _Strassen:
    _USES = {1: ((0, 1), (3, 1)), 2: ((2, 1), (3, -1)), 3: ((1, 1), (3, 1)), 4: ((0, 1), (2, 1)),
             5: ((0, -1), (1, 1)), 6: ((3, 1),), 7: ((0, 1),)}

    def __init__(self, product, order):
        self._product = product
        self._todo = list(order)
        self._c = [None] * 4

    @property
    def done(self):
        return not self._todo

    def step(self):
        i = self._todo.pop(0)
        m = self._product(i - 1)
        for k, sign in self._USES[i]:
            if self._c[k] is None:
                assert sign > 0
                self._c[k] = m
            else:
                self._c[k] = self._c[k] + m if sign > 0 else self._c[k] - m

    def result(self):
        assert self.done
        return jnp.concatenate(self._c[:2], axis=1), jnp.concatenate(self._c[2:], axis=1)


def _kernel(x_hbm, wqkv_hbm, wphi_hbm, wo_hbm, wr_hbm, wg_hbm, wu_hbm, wd_hbm, c_hbm, wmod_hbm,
            out_hbm,
            x_v, wqkv_v, wphi_v, wo_v, wr_v, wg_v, wu_v, wd_v, c_v, wmod_v,
            wkv_s, wq_s, wo_s, h_s, kv_s, mod_s, col_s, x1_s, stat_s, out_s, fmap_s,
            oa_s, ob_s, vec_s, xn_s, carry_s, raw_s, z_s,
            sem_w, sem_m, sem_k, sem_v, sem_x, sem_o, sem_p):
    def wcopy(i, src, dst):
        return pltpu.make_async_copy(src, dst, sem_w.at[i])

    cp_c = wcopy(0, c_hbm, c_v)
    cp_phi = wcopy(1, wphi_hbm, wphi_v)
    cp_wr = wcopy(2, wr_hbm, wr_v)
    cp_wq = wcopy(3, wqkv_hbm.at[:, 0:D], wqkv_v.at[:, 0:D])
    cp_mb = wcopy(4, wmod_hbm.at[:, 2 * D:4 * D], wmod_v.at[:, 2 * D:4 * D])
    cp_mc = wcopy(5, wmod_hbm.at[:, 4 * D:6 * D], wmod_v.at[:, 4 * D:6 * D])
    cp_wo = wcopy(6, wo_hbm, wo_v.at[:, 0:D])
    cp_wg = wcopy(7, wg_hbm, wg_v.at[:, 0:F])
    cp_wu = wcopy(8, wu_hbm, wu_v.at[:, 0:F])
    cp_wd = wcopy(9, wd_hbm, wd_v.at[:, 0:D])

    def mod_copy(j):
        col0 = (j % 2) * D + (j // 2) * KH
        cols = pl.ds(col0 if isinstance(j, int) else pl.multiple_of(col0, KH), KH)
        return pltpu.make_async_copy(wmod_hbm.at[:, cols], wmod_v.at[:, cols], sem_m.at[j])

    def kv_copies(o):
        ck, cv = pl.ds(D + o * 256, 256), pl.ds(2 * D + o * 256, 256)
        return (pltpu.make_async_copy(wqkv_hbm.at[:, ck], wqkv_v.at[:, ck], sem_k.at[o]),
                pltpu.make_async_copy(wqkv_hbm.at[:, cv], wqkv_v.at[:, cv], sem_v.at[o]))

    def x_copy(t):
        rows = _rows(t * T, T)
        return pltpu.make_async_copy(x_hbm.at[rows], x_v.at[rows], sem_x.at[t])

    def out_copy(t):
        rows = _rows(t * T, T)
        return pltpu.make_async_copy(out_s.at[rows], out_hbm.at[rows], sem_o.at[t])

    def start(*copies):
        for cp in copies:
            cp.start()

    def wait(*copies):
        for cp in copies:
            cp.wait()

    def fold(col0, g):
        return _dot_nt(_unpack(fmap_s[g * 64:(g + 1) * 64, :]),
                       wqkv_v[:, col0 + g * 128:col0 + (g + 1) * 128]) * LOG2E

    def stage_left(dst, o, upper, lower):
        n = upper.shape[0] // 2
        for i, a in enumerate(_left_terms(upper[:, :KH], upper[:, KH:], lower[:, :KH], lower[:, KH:])):
            dst[(i * 4 + o) * n:(i * 4 + o + 1) * n, :] = _pack(a)

    def stage_kv_weights(o):
        blocks = []
        for g in (2 * o, 2 * o + 1):
            fk = fold(D, g)
            fv = wqkv_v[:, 2 * D + g * 128:2 * D + (g + 1) * 128].T.astype(F32)
            blocks.append(jnp.concatenate([fk[:64], fv[:64], fk[64:], fv[64:]], axis=0))
        stage_left(wkv_s, o, *blocks)

    def stage_q_weights(o):
        stage_left(wq_s, o, fold(0, o), fold(0, o + 4))

    def stage_out_weights(o):
        stage_left(wo_s, o, wo_v[:, o * 128:(o + 1) * 128].T.astype(F32),
                   wo_v[:, KH + o * 128:KH + (o + 1) * 128].T.astype(F32))

    def param(k, n):
        return jnp.concatenate([mod_s[:, k * D:(k + 1) * D]] * (n // 8), axis=0)

    def modulation(col0, n):
        mod_s[:, col0:col0 + n] = _dot(_unpack(vec_s[...]), wmod_v[:, col0:col0 + n])[0:8]

    def first_norm(t, dst, base, normalized=None):
        for r0 in range(0, U, LN_ROWS):
            h = []
            for half in range(2):
                rows = _rows(t * T + half * U + r0, LN_ROWS)
                xn = _normalize(x_v[rows, :].astype(F32)) if normalized is None else normalized[rows, :]
                h.append(xn * param(SCALE_A, LN_ROWS) + param(SHIFT_A, LN_ROWS))
            for i, b in enumerate(_right_terms(h[0][:, :KH], h[1][:, :KH], h[0][:, KH:], h[1][:, KH:])):
                dst[base + i * 64 + r0 // 2:base + i * 64 + (r0 + LN_ROWS) // 2, :] = _pack(b)

    def kv_products(src, base, o, order=ORDER_KV):
        return _Strassen(lambda i: _dot_nt(_unpack(wkv_s[(i * 4 + o) * 128:(i * 4 + o + 1) * 128, :]),
                                           _unpack(src[base + i * 64:base + (i + 1) * 64, :])), order)

    def kv_pairs(block):
        return [(block[j * 128 + 64:(j + 1) * 128].astype(BF), _hedgehog(block[j * 128:j * 128 + 64]).astype(BF))
                for j in range(2)]

    def kv_operands(r):
        return kv_pairs(r[0]) + kv_pairs(r[1])

    def save_kv_operands(r):
        raw_s[...] = r[0]
        for j, (v, phi) in enumerate(kv_pairs(r[1])):
            carry_s[j * 64:(j + 1) * 64, :] = pltpu.bitcast(phi, U32)
            carry_s[128 + j * 32:128 + (j + 1) * 32, :] = pltpu.bitcast(v, U32)

    def load_kv_operands():
        done = [(_unpack(carry_s[128 + j * 32:128 + (j + 1) * 32, :]), _unpack(carry_s[j * 64:(j + 1) * 64, :]))
                for j in range(2)]
        return kv_pairs(raw_s[...]) + done

    def accumulate_kv(ops, o, first=False, last=False):
        ones = jnp.ones((16, T), BF)
        for j, (v, phi) in enumerate(ops):
            acc = _dot_nt(jnp.concatenate([v, ones], axis=0), phi)
            if not first:
                acc = acc + kv_s[4 * o + j]
            if last:
                z_s[4 * o + j] = jnp.concatenate([acc[64:72]] * 16, axis=0).T
                row_head = lax.broadcasted_iota(I32, (80, 128), 0) // DH
                lane_head = lax.broadcasted_iota(I32, (80, 128), 1) % 2
                acc = jnp.where(row_head == lane_head, acc, 0.0)
            kv_s[4 * o + j] = acc

    start(cp_phi, cp_c, *kv_copies(0), x_copy(0))
    lax.fori_loop(0, 4, lambda j, _: mod_copy(j).start(), None)
    cp_c.wait()
    cv = c_v[...].astype(F32)
    vec_s[...] = _pack(jnp.broadcast_to(cv * jax.nn.sigmoid(cv), (16, D)))
    cp_phi.wait()
    repeat = ((lax.broadcasted_iota(I32, (128, DH), 0) % 64) // 2
              == lax.broadcasted_iota(I32, (128, DH), 1)).astype(BF)
    block_row = lax.broadcasted_iota(I32, (128, 128), 0)
    same_head = 2 * (block_row // 64) + block_row % 2 == lax.broadcasted_iota(I32, (128, 128), 1) // DH
    for g in range(8):
        full = _dot_nt(repeat, wphi_v[g * 128:(g + 1) * 128, :])
        fmap_s[g * 64:(g + 1) * 64, :] = _pack(jnp.where(same_head, full, 0.0))
    wait(*kv_copies(0))
    stage_kv_weights(0)
    x_copy(0).wait()
    xn_s[...] = _normalize(x_v[0:T, :].astype(F32))
    for j in range(4):
        mod_copy(j).wait()
        if j == 2:
            start(*kv_copies(1), *kv_copies(2))
        elif j == 3:
            start(*kv_copies(3))
        col0 = (j % 2) * D + (j // 2) * KH
        modulation(col0, KH)
        if j % 2:
            mod_s[:, col0:col0 + KH] += 1.0
        if j == 1:
            left = [xn_s[k * U:(k + 1) * U, 0:KH] * param(SCALE_A, U)[:, 0:KH] + param(SHIFT_A, U)[:, 0:KH]
                    for k in range(2)]
            h_s[64:128, :] = _pack(left[0])
            h_s[320:384, :] = _pack(left[0] + left[1])
            first_products = kv_products(h_s, 0, 0, ORDER_FIRST)
            first_products.step()
            first_products.step()
    first_norm(0, h_s, 0, normalized=xn_s)

    ops = None
    for o, plan in enumerate(PLAN_FIRST):
        products = kv_products(h_s, (o // 4) * HROWS, o % 4) if o else first_products
        for item in plan.split():
            if item == "p":
                products.step()
            elif item == "W":
                wait(*kv_copies(o + 1))
                if o == 0:
                    x_copy(1).start()
            elif item == "X":
                x_copy(1).wait()
                start(x_copy(2), x_copy(3), cp_wr)
            elif item == "s":
                stage_kv_weights(o + 1)
            elif item == "L":
                first_norm(1, h_s, HROWS)
            else:
                accumulate_kv(ops, o - 1, first=True)
        if o < 4:
            ops = kv_operands(products.result())
    save_kv_operands(products.result())

    def kv_tile(t, ops, src, base, plans, following=None):
        last = following is not None
        if not last:
            first_norm(t + 1, src, base + HROWS)
        for o, plan in enumerate(plans):
            if o < 3:
                products = kv_products(src, base, o + 1)
            else:
                products = following if last else kv_products(src, base + HROWS, 0)
            for item in plan.split():
                if item == "p":
                    products.step()
                elif item == "s":
                    stage_q_weights(o)
                elif item == "o":
                    stage_out_weights(o)
                else:
                    accumulate_kv(ops, o, last=last)
            if o < 3:
                ops = kv_operands(products.result())
        return products.result()

    def pass1(i, remaining):
        t = 2 * i + 1
        wait(x_copy(t + 1), x_copy(t + 2))
        pl.when(i == 0)(lambda: start(*(x_copy(k) for k in range(4, NT)), cp_wq, cp_wo))
        pl.when(i == 1)(lambda: start(cp_mb, cp_mc, cp_wg))
        view = h_s.at[_rows(t * HROWS, 3 * HROWS)]
        r = kv_tile(t, load_kv_operands(), view, 0, PLAN_KV_A)
        save_kv_operands(kv_tile(t + 1, kv_operands(r), view, HROWS, PLAN_KV_B))
        return remaining - 1

    first_tile = lax.fori_loop(0, 3, pass1, 3)

    def q_products(t, o):
        return _Strassen(lambda i: _dot_nt(_unpack(wq_s[(i * 4 + o) * 64:(i * 4 + o + 1) * 64, :]),
                                           _unpack(h_s[_rows(t * HROWS + i * 64, 64), :])), ORDER_Q)

    def derived_params():
        wr8 = wr_v[...].astype(F32)
        wr = jnp.broadcast_to(jnp.concatenate([wr8[j:j + 1, :] for j in range(8)], axis=1), (8, D))
        scale = 1.0 + param(SCALE_B, 8)
        mod_s[:, SCALE_B * D:(SCALE_B + 1) * D] = scale
        router = scale * wr
        tables = (param(GATE_A, 8), router, scale * param(GATE_B, 8), param(SHIFT_B, 8) * param(GATE_B, 8))
        for k, row in enumerate(tables):
            for g in range(8):
                tile = jnp.concatenate([row[:, g * 128:(g + 1) * 128]] * 16, axis=0)
                col_s[k * D + g * 128:k * D + (g + 1) * 128, :] = tile.T
        base = ROUTER_SUMS * D
        mod_s[:, base:base + T] = jnp.broadcast_to(jnp.sum(router, axis=-1, keepdims=True), (8, T))
        mod_s[:, base + T:base + 2 * T] = jnp.broadcast_to(
            jnp.sum(param(SHIFT_B, 8) * wr, axis=-1, keepdims=True), (8, T))

    def column(k, ch):
        v = col_s[k * D + ch:k * D + ch + 128, :]
        return jnp.concatenate([v, v], axis=1)

    def feature_pairs(block, p0):
        out = []
        for j in range(2):
            phi = _hedgehog(block[j * 64:(j + 1) * 64])
            z = z_s[p0 + j]
            inv = _recip(_per_head(phi * jnp.concatenate([z, z], axis=1), jnp.add) + 1e-6)
            out.append((phi.astype(BF), inv))
        return out

    def features(r, o):
        return feature_pairs(r[0], 2 * o) + feature_pairs(r[1], 2 * o + 8)

    def save_features(r):
        raw_s[0:128, :] = r[0]
        for j, (phi, inv) in enumerate(feature_pairs(r[1], 8)):
            carry_s[j * 64:(j + 1) * 64, :] = pltpu.bitcast(phi, U32)
            raw_s[128 + 8 * j:136 + 8 * j, :] = inv

    def load_features():
        done = [(_unpack(carry_s[j * 64:(j + 1) * 64, :]), raw_s[128 + 8 * j:136 + 8 * j, :]) for j in range(2)]
        return feature_pairs(raw_s[0:128, :], 0) + done

    def attend(phis, o):
        heads = {}
        for j in (0, 2, 1, 3):
            phi, inv = phis[j]
            num = _dot(kv_s[2 * o + 8 * (j // 2) + j % 2, 0:64, :].astype(BF), phi)
            heads[j] = jnp.concatenate([num[k * DH:(k + 1) * DH] * inv[k:k + 1] for k in range(2)], axis=0)
        return heads

    def stage_heads(dst, o, j, lo, hi):
        base = o * 64 + j * 32
        terms = _right_terms(lo[:, :U], lo[:, U:], hi[:, :U], hi[:, U:])
        dst[base:base + 32, 0:6 * U] = _pack(jnp.concatenate(terms[:6], axis=1))
        dst[base:base + 16, 6 * U:8 * U] = _pack(jnp.concatenate([terms[6][:32], terms[6][32:]], axis=1))

    def out_products(src, o):
        def product(i):
            if i < 6:
                b = src[:, i * U:(i + 1) * U]
            else:
                b = jnp.concatenate([src[k * 32:k * 32 + 16, (6 + c) * U:(7 + c) * U]
                                     for k in range(8) for c in range(2)], axis=0)
            return _dot(_unpack(wo_s[(i * 4 + o) * 64:(i * 4 + o + 1) * 64, :]), _unpack(b))
        return _Strassen(product, ORDER_OUT)

    def residual(t, o, attn, sums):
        ys = []
        for half, a in enumerate(attn):
            ch = half * KH + o * 128
            ys.append(x_v[_rows(t * T, T), ch:ch + 128].T.astype(F32) + column(COL_GATE_A, ch) * a)
        if sums is None:
            shift = jnp.sum(_fold8(ys[0]) + _fold8(ys[1]), axis=0, keepdims=True) * (1.0 / 256)
            sums = (shift, 0.0, 0.0, 0.0)
        shift, s1, s2, s3 = sums
        for half, y in enumerate(ys):
            ch = half * KH + o * 128
            d = y - shift
            for k in range(2):
                x1_s[_rows((2 * t + k) * D + ch, 128), :] = y[:, k * U:(k + 1) * U]
            s1, s2, s3 = s1 + _fold8(d), s2 + _fold8(d * d), s3 + _fold8(d * column(COL_ROUTER, ch))
        return shift, s1, s2, s3

    def route(t, sums, top):
        m1, i1, m2, i2 = top
        shift = sums[0]
        s1, s2, s3 = (jnp.sum(s, axis=0, keepdims=True) for s in sums[1:])
        delta = s1 * (1.0 / D)
        rstd = lax.rsqrt(jnp.maximum(s2 * (1.0 / D) - delta * delta, 0.0) + 1e-5)
        score = (s3 - delta * mod_s[0:1, ROUTER_SUMS * D:ROUTER_SUMS * D + T]) * rstd
        for k, v in enumerate((shift + delta, rstd)):
            for half in range(2):
                stat_s[_rows(((2 * t + half) * 2 + k) * 8, 8), :] = jnp.broadcast_to(
                    v[:, half * U:(half + 1) * U], (8, U))
        idx = lax.broadcasted_iota(I32, (1, T), 1) + t * T
        g1, g2 = score > m1, score > m2
        return (jnp.where(g1, score, m1), jnp.where(g1, idx, i1),
                jnp.where(g1, m1, jnp.where(g2, score, m2)), jnp.where(g1, i1, jnp.where(g2, idx, i2)))

    def stat(block, k, n):
        return jnp.concatenate([stat_s[_rows((block * 2 + k) * 8, 8), :]] * (n // 8), axis=0)

    def emit(t, ch):
        n = 256
        for half in range(2):
            mean, rstd = (stat(2 * t + half, k, n) for k in range(2))
            x1 = x1_s[_rows((2 * t + half) * D + ch, n), :]
            gain = rstd * col_s[COL_GAIN * D + ch:COL_GAIN * D + ch + n, :]
            res = (x1 + col_s[COL_BIAS * D + ch:COL_BIAS * D + ch + n, :]) + (x1 - mean) * gain
            out_s[_rows(t * T + half * U, U), ch:ch + n] = res.T.astype(BF)

    def q_tile(t, phis, top, plans, current, previous, more=True):
        sums, emitted = None, 0
        for o, plan in enumerate(plans):
            qs = None
            if phis is not None and (o < 3 or more):
                qs = q_products(t, o + 1) if o < 3 else q_products(t + 1, 0)
            ws = out_products(previous, o)
            heads, staged = None, 0
            for item in plan.split():
                if item == "q":
                    qs.step()
                elif item == "w":
                    ws.step()
                    if ws.done:
                        sums = residual(t - 1, o, ws.result(), sums)
                elif item == "N":
                    heads = attend(phis, o)
                elif item == "c":
                    stage_heads(current, o, staged, heads[staged], heads[staged + 2])
                    staged += 1
                elif item == "E":
                    emit(t - 2, emitted * 256)
                    emitted += 1
                elif item == "M":
                    modulation((GATE_A + o) * D, D)
            if qs is not None:
                phis = features(qs.result(), o + 1) if o < 3 else qs.result()
        if sums is not None:
            top = route(t - 1, sums, top)
        if emitted:
            out_copy(t - 2).start()
        return phis, top

    wait(cp_wq, cp_wo, cp_mb, cp_mc, cp_wr)
    cp_wu.start()
    r = kv_tile(NT - 1, load_kv_operands(), h_s, (NT - 1) * HROWS, PLAN_KV_LAST,
                following=q_products(first_tile, 0))
    lowest = jnp.full((1, T), -jnp.inf, F32)
    zero = jnp.zeros((1, T), I32)
    top = (lowest, zero, lowest, zero)
    r, top = q_tile(first_tile, features(r, 0), top, PLAN_Q_FIRST, oa_s, ob_s)
    derived_params()
    r, top = q_tile(first_tile + 1, features(r, 0), top, PLAN_Q_SECOND, ob_s, oa_s)
    save_features(r)

    def pass2(i, carry):
        top, tile = carry
        pl.when(i == 2)(cp_wd.start)
        r, top = q_tile(2 * i - 2, load_features(), top, PLAN_Q, oa_s, ob_s)
        r, top = q_tile(2 * i - 1, features(r, 0), top, PLAN_Q, ob_s, oa_s)
        save_features(r)
        return top, tile + 2

    top, tile = lax.fori_loop(2, 4, pass2, (top, 2))
    wait(cp_wg, cp_wu, cp_wd)
    r, top = q_tile(tile, load_features(), top, PLAN_Q_LATE, oa_s, ob_s)
    _, top = q_tile(tile + 1, features(r, 0), top, PLAN_Q_LAST, ob_s, oa_s, more=False)
    _, top = q_tile(tile + 2, None, top, PLAN_DRAIN, oa_s, ob_s)

    m1, i1, m2, i2 = top
    best = jnp.max(m1, axis=1, keepdims=True)
    ia = jnp.min(jnp.where(m1 == best, i1, S - 1), axis=1, keepdims=True)
    taken = i1 == ia
    rest, rest_idx = jnp.where(taken, m2, m1), jnp.where(taken, i2, i1)
    second = jnp.max(rest, axis=1, keepdims=True)
    ib = jnp.min(jnp.where(rest == second, rest_idx, S - 1), axis=1, keepdims=True)
    idx = (jnp.clip(ia[0, 0], 0, S - 1), jnp.clip(ib[0, 0], 0, S - 1))

    for g in range(4):
        emit(NT - 1, g * 256)
    out_copy(NT - 1).start()
    out_copy(0).wait()

    row16 = lax.broadcasted_iota(I32, (16, U), 0)
    lane16 = lax.broadcasted_iota(I32, (16, U), 1)
    xn_sel = 0.0
    for k in range(2):
        block = idx[k] // U
        xn = (x1_s[_rows(block * D, D), :] - stat(block, 0, D)) * stat(block, 1, D)
        pick = jnp.where((row16 == k) & (lane16 == idx[k] % U), 1.0, 0.0).astype(BF)
        xn_sel = xn_sel + _dot_nt(pick, xn.astype(BF))
    hs = (xn_sel * param(SCALE_B, 16) + param(SHIFT_B, 16)).astype(BF)
    score = jnp.where(row16[:, 0:1] == 0, best, second) + mod_s[0:1, ROUTER_SUMS * D + T:ROUTER_SUMS * D + T + 1]
    gate = jax.nn.sigmoid(score)

    y = jnp.zeros((16, D), F32)
    for j in range(F // FC):
        gj = _dot(hs, wg_v[:, j * FC:(j + 1) * FC])
        uj = _dot(hs, wu_v[:, j * FC:(j + 1) * FC])
        y = y + _dot((gj * jax.nn.sigmoid(gj) * uj).astype(BF), wd_v[j * FC:(j + 1) * FC, 0:D])
    update = param(GATE_B, 16) * (y * gate)

    wait(*(out_copy(t) for t in range(1, NT)))
    row = lax.broadcasted_iota(I32, (16, D), 0)

    def patch(k):
        base = pl.multiple_of((idx[k] // 16) * 16, 16)
        block = out_s[pl.ds(base, 16), :].astype(F32)
        out_s[pl.ds(base, 16), :] = jnp.where(row == idx[k] - base, block + update[k:k + 1, :], block).astype(BF)
        return pltpu.make_async_copy(out_s.at[pl.ds(base, 16)], out_hbm.at[pl.ds(base, 16)], sem_p.at[k])

    patch_a, patch_b = patch(0), patch(1)
    patch_a.start()

    @pl.when(idx[0] // 16 != idx[1] // 16)
    def _():
        patch_b.start()
        patch_b.wait()

    patch_a.wait()


@jax.jit
def pallas_adaLN_cond__linear_kernel_hedgehog__moe_arch_mod__prompt_kernel(
        A_x, A_wqkv, A_w_phi, A_wo, B_x, B_w_r, B_w_gate, B_w_up, B_w_down, c, w_mod):
    del B_x
    hbm = pl.BlockSpec(memory_space=pl.ANY)
    out = pl.pallas_call(
        _kernel,
        out_shape=jax.ShapeDtypeStruct((S, D), BF),
        in_specs=[hbm] * 10,
        out_specs=hbm,
        scratch_shapes=[
            pltpu.VMEM((S, D), BF),
            pltpu.VMEM((D, 3 * D + PAD), BF),
            pltpu.VMEM((H * DH, DH), BF),
            pltpu.VMEM((D, D + PAD), BF),
            pltpu.VMEM((8, 128), BF),
            pltpu.VMEM((D, F + PAD), BF),
            pltpu.VMEM((D, F + PAD), BF),
            pltpu.VMEM((F, D + PAD), BF),
            pltpu.VMEM((1, D), BF),
            pltpu.VMEM((D, 6 * D + PAD), BF),
            pltpu.VMEM((7 * 512, KH), U32),
            pltpu.VMEM((7 * 256, KH), U32),
            pltpu.VMEM((7 * 256, KH), U32),
            pltpu.VMEM((NT * HROWS, KH), U32),
            pltpu.VMEM((NPAIR, 80, 128), F32),
            pltpu.VMEM((8, 6 * D + 2 * T), F32),
            pltpu.VMEM((4 * D, 128), F32),
            pltpu.VMEM((2 * NT * D, U), F32),
            pltpu.VMEM((2 * NT * 2 * 8, U), F32),
            pltpu.VMEM((S, D), BF),
            pltpu.VMEM((8 * 64, 128), U32),
            pltpu.VMEM((KH // 2, 8 * U), U32),
            pltpu.VMEM((KH // 2, 8 * U), U32),
            pltpu.VMEM((8, D), U32),
            pltpu.VMEM((T, D), F32),
            pltpu.VMEM((192, T), U32),
            pltpu.VMEM((256, T), F32),
            pltpu.VMEM((NPAIR, 128, U), F32),
            pltpu.SemaphoreType.DMA((10,)),
            pltpu.SemaphoreType.DMA((4,)),
            pltpu.SemaphoreType.DMA((4,)),
            pltpu.SemaphoreType.DMA((4,)),
            pltpu.SemaphoreType.DMA((NT,)),
            pltpu.SemaphoreType.DMA((NT,)),
            pltpu.SemaphoreType.DMA((2,)),
        ],
        compiler_params=pltpu.CompilerParams(
            vmem_limit_bytes=110 * 2**20,
            flags={"XLA_TPU_EVENLY_DISTRIBUTE_CRITICAL_NODES": True}),
        name="fused_block",
    )(A_x.reshape(S, D), A_wqkv, A_w_phi.reshape(H * DH, DH), A_wo, B_w_r.reshape(8, 128),
      B_w_gate, B_w_up, B_w_down, c, w_mod)
    return out.reshape(1, S, D)
```

```python
import math

import jax
import jax.numpy as jnp
from jax import lax
import jax.experimental.pallas as pl
import jax.experimental.pallas.tpu as pltpu

S, D, H, DH, F = 2048, 1024, 32, 32, 3584
U = 128
T = 2 * U
NT = S // T
KH = D // 2
NPAIR = H // 2
HROWS = 7 * U // 2
PAD = 128
FC = F // 2
LN_ROWS = 32
LOG2E = math.log2(math.e)
BF, F32, U32, I32 = jnp.bfloat16, jnp.float32, jnp.uint32, jnp.int32

SHIFT_A, SCALE_A, GATE_A, SHIFT_B, SCALE_B, GATE_B, ROUTER_SUMS = range(7)
COL_GATE_A, COL_ROUTER, COL_GAIN, COL_BIAS = range(4)

PLAN_FIRST = (
    "p p p p W s p", "p p W s p N p p p p",
    "p N p W s p p p p p", "X N L p p p p p p p",
    "p p p p p p p N", "p p N p p p p p",
    "p p p p p p p N", "p p N p p p p p")
PLAN_KV = (
    "p p N p p p p p", "p N p p p p p p",
    "p p N p p p p p", "p p N p p p p p",
    "p p p N p p p p", "p N p p p p p p",
    "p p p N p p p p", "p p p N p p p p")
PLAN_KV_LAST = (
    "p p N p p p p p o", "p p p N p p p p o",
    "p p p N p p p p o", "p p N p p p p p o",
    "B p p p N s p p p p", "p N p s p p p p p",
    "p p s p N p p p p", "p p s p p p N p p",
    "p p p N p p p p")
PLAN_Q_FIRST = (
    "q q N c c q M q q q q", "q q N c c q M q q q q",
    "q q N c c M q q q q q", "q M N c c q q q q q q")
PLAN_Q_SECOND = (
    "w w w w w w w N c c q q q q q q q", "w w w w w w N c c w q q q q q q q",
    "w w w w w w w q q q q N c c q q q", "w w w w w w w q q N c c q q q q q")
PLAN_Q = (
    "w w w w w w N c c w q q q q q q q E", "w w w w w N c c w w q q q q q q E q",
    "w w w w w N c c w w q q q q q q E q", "w w w w w w w q N c c q q q q q q E")
PLAN_Q_LATE = (
    "w N c c w w w w w w q q q q q q q E", "w w w w w w w q q N c c q q q q q E",
    "w w w w w w w q q N c c q q q q q E", "w w w w w w w q q q q q q N c c q E")
PLAN_Q_LAST = (
    "w w w w w w w q q q q q N c c q q E", "w w w w w w w q q q N c c q q q E q",
    "w w w w w w w q q N c c q q q q q E", "w w w w w w N c c w E")
PLAN_DRAIN = (
    "w E w w w w w w E", "w w w w w E w w",
    "w w w w w w w E", "w w w w w w w")
ORDER_FIRST = (6, 2, 1, 3, 4, 5, 7)
ORDER_KV = (1, 2, 3, 6, 4, 5, 7)
ORDER_Q = (4, 3, 2, 5, 1, 6, 7)
ORDER_OUT = (4, 7, 3, 1, 5, 2, 6)


def _dot(a, b):
    return jnp.dot(a, b, preferred_element_type=F32)


def _dot_nt(a, b):
    return lax.dot_general(a, b, (((1,), (1,)), ((), ())), preferred_element_type=F32)


def _pack(v):
    return pltpu.bitcast(v.astype(BF), U32)


def _unpack(v):
    return pltpu.bitcast(v, BF)


def _recip(v):
    return pl.reciprocal(v, approx=False, full_range=False)


def _rows(start, size):
    return pl.ds(start if isinstance(start, int) else pl.multiple_of(start, 8), size)


def _normalize(v):
    centered = v - jnp.mean(v, axis=-1, keepdims=True)
    var = jnp.mean(centered * centered, axis=-1, keepdims=True)
    return centered * lax.rsqrt(var + 1e-5)


def _fold8(v, op=jnp.add):
    parts = [v[i:i + 8] for i in range(0, v.shape[0], 8)]
    while len(parts) > 1:
        parts = [op(parts[i], parts[i + 1]) for i in range(0, len(parts), 2)]
    return parts[0]


def _per_head(v, op):
    r = _fold8(v, op)
    r = op(r, pltpu.roll(r, 4, 0))
    return op(r, pltpu.roll(r, 2, 0))


def _hedgehog(p):
    def spread(v):
        return jnp.concatenate([v] * 8, axis=0)

    pos = jnp.exp2(p - spread(_per_head(p, jnp.maximum)))
    neg = jnp.exp2(spread(_per_head(p, jnp.minimum)) - p)
    pos = pos * spread(_recip(_per_head(pos, jnp.add)))
    neg = neg * spread(_recip(_per_head(neg, jnp.add)))
    return jnp.concatenate([pos, neg], axis=0)


def _left_terms(a11, a12, a21, a22):
    return a11 + a22, a21 + a22, a11, a22, a11 + a12, a21 - a11, a12 - a22


def _right_terms(b11, b12, b21, b22):
    return b11 + b22, b11, b12 - b22, b21 - b11, b22, b11 + b12, b21 + b22


class _Strassen:
    _USES = {1: ((0, 1), (3, 1)), 2: ((2, 1), (3, -1)), 3: ((1, 1), (3, 1)), 4: ((0, 1), (2, 1)),
             5: ((0, -1), (1, 1)), 6: ((3, 1),), 7: ((0, 1),)}

    def __init__(self, product, order):
        self._product = product
        self._todo = list(order)
        self._c = [None] * 4

    @property
    def done(self):
        return not self._todo

    def step(self):
        i = self._todo.pop(0)
        m = self._product(i - 1)
        for k, sign in self._USES[i]:
            if self._c[k] is None:
                assert sign > 0
                self._c[k] = m
            else:
                self._c[k] = self._c[k] + m if sign > 0 else self._c[k] - m

    def result(self):
        assert self.done
        return jnp.concatenate(self._c[:2], axis=1), jnp.concatenate(self._c[2:], axis=1)


def _kernel(x_hbm, wqkv_hbm, wphi_hbm, wo_hbm, wr_hbm, wg_hbm, wu_hbm, wd_hbm, c_hbm, wmod_hbm,
            out_hbm,
            x_v, wqkv_v, wphi_v, wo_v, wr_v, wg_v, wu_v, wd_v, c_v, wmod_v,
            wkv_s, wq_s, wo_s, h_s, kv_s, mod_s, col_s, x1_s, stat_s, out_s, fmap_s,
            oa_s, ob_s, vec_s, xn_s, carry_s, raw_s, z_s,
            sem_w, sem_m, sem_k, sem_v, sem_x, sem_o, sem_p):
    def wcopy(i, src, dst):
        return pltpu.make_async_copy(src, dst, sem_w.at[i])

    cp_c = wcopy(0, c_hbm, c_v)
    cp_phi = wcopy(1, wphi_hbm, wphi_v)
    cp_wr = wcopy(2, wr_hbm, wr_v)
    cp_wq = wcopy(3, wqkv_hbm.at[:, 0:D], wqkv_v.at[:, 0:D])
    cp_mb = wcopy(4, wmod_hbm.at[:, 2 * D:4 * D], wmod_v.at[:, 2 * D:4 * D])
    cp_mc = wcopy(5, wmod_hbm.at[:, 4 * D:6 * D], wmod_v.at[:, 4 * D:6 * D])
    cp_wo = wcopy(6, wo_hbm, wo_v.at[:, 0:D])
    cp_wg = wcopy(7, wg_hbm, wg_v.at[:, 0:F])
    cp_wu = wcopy(8, wu_hbm, wu_v.at[:, 0:F])
    cp_wd = wcopy(9, wd_hbm, wd_v.at[:, 0:D])

    def mod_copy(j):
        col0 = (j % 2) * D + (j // 2) * KH
        cols = pl.ds(col0 if isinstance(j, int) else pl.multiple_of(col0, KH), KH)
        return pltpu.make_async_copy(wmod_hbm.at[:, cols], wmod_v.at[:, cols], sem_m.at[j])

    def kv_copies(o):
        ck, cv = pl.ds(D + o * 256, 256), pl.ds(2 * D + o * 256, 256)
        return (pltpu.make_async_copy(wqkv_hbm.at[:, ck], wqkv_v.at[:, ck], sem_k.at[o]),
                pltpu.make_async_copy(wqkv_hbm.at[:, cv], wqkv_v.at[:, cv], sem_v.at[o]))

    def x_copy(t):
        rows = _rows(t * T, T)
        return pltpu.make_async_copy(x_hbm.at[rows], x_v.at[rows], sem_x.at[t])

    def out_copy(t):
        rows = _rows(t * T, T)
        return pltpu.make_async_copy(out_s.at[rows], out_hbm.at[rows], sem_o.at[t])

    def start(*copies):
        for cp in copies:
            cp.start()

    def wait(*copies):
        for cp in copies:
            cp.wait()

    def fold(col0, g):
        return _dot_nt(_unpack(fmap_s[g * 64:(g + 1) * 64, :]),
                       wqkv_v[:, col0 + g * 128:col0 + (g + 1) * 128]) * LOG2E

    def stage_left(dst, o, upper, lower):
        n = upper.shape[0] // 2
        for i, a in enumerate(_left_terms(upper[:, :KH], upper[:, KH:], lower[:, :KH], lower[:, KH:])):
            dst[(i * 4 + o) * n:(i * 4 + o + 1) * n, :] = _pack(a)

    def stage_kv_weights(o):
        blocks = []
        for g in (2 * o, 2 * o + 1):
            fk = fold(D, g)
            fv = wqkv_v[:, 2 * D + g * 128:2 * D + (g + 1) * 128].T.astype(F32)
            blocks.append(jnp.concatenate([fk[:64], fv[:64], fk[64:], fv[64:]], axis=0))
        stage_left(wkv_s, o, *blocks)

    def stage_q_weights(o):
        stage_left(wq_s, o, fold(0, o), fold(0, o + 4))

    def stage_out_weights(o):
        stage_left(wo_s, o, wo_v[:, o * 128:(o + 1) * 128].T.astype(F32),
                   wo_v[:, KH + o * 128:KH + (o + 1) * 128].T.astype(F32))

    def param(k, n, width=D):
        return jnp.concatenate([mod_s[:, k * D:k * D + width]] * (n // 8), axis=0)

    def modulation(col0, n):
        mod_s[:, col0:col0 + n] = _dot(_unpack(vec_s[...]), wmod_v[:, col0:col0 + n])[0:8]

    def first_norm(t, dst, base, normalized=None):
        for r0 in range(0, U, LN_ROWS):
            h = []
            for half in range(2):
                rows = _rows(t * T + half * U + r0, LN_ROWS)
                xn = _normalize(x_v[rows, :].astype(F32)) if normalized is None else normalized[rows, :]
                h.append(xn * param(SCALE_A, LN_ROWS) + param(SHIFT_A, LN_ROWS))
            for i, b in enumerate(_right_terms(h[0][:, :KH], h[1][:, :KH], h[0][:, KH:], h[1][:, KH:])):
                dst[base + i * 64 + r0 // 2:base + i * 64 + (r0 + LN_ROWS) // 2, :] = _pack(b)

    def kv_products(src, base, o, order=ORDER_KV):
        return _Strassen(lambda i: _dot_nt(_unpack(wkv_s[(i * 4 + o) * 128:(i * 4 + o + 1) * 128, :]),
                                           _unpack(src[base + i * 64:base + (i + 1) * 64, :])), order)

    def kv_pairs(block):
        return [(block[j * 128 + 64:(j + 1) * 128].astype(BF), _hedgehog(block[j * 128:j * 128 + 64]).astype(BF))
                for j in range(2)]

    def kv_operands(r):
        return kv_pairs(r[0]) + kv_pairs(r[1])

    def save_kv_operands(r):
        raw_s[...] = r[0]
        for j, (v, phi) in enumerate(kv_pairs(r[1])):
            carry_s[j * 64:(j + 1) * 64, :] = pltpu.bitcast(phi, U32)
            carry_s[128 + j * 32:128 + (j + 1) * 32, :] = pltpu.bitcast(v, U32)

    def load_kv_operands():
        done = [(_unpack(carry_s[128 + j * 32:128 + (j + 1) * 32, :]), _unpack(carry_s[j * 64:(j + 1) * 64, :]))
                for j in range(2)]
        return kv_pairs(raw_s[...]) + done

    def accumulate_kv(ops, o, last=False):
        ones = jnp.ones((16, T), BF)
        for j, (v, phi) in enumerate(ops):
            acc = _dot_nt(jnp.concatenate([v, ones], axis=0), phi) + kv_s[4 * o + j]
            if last:
                z_s[4 * o + j] = jnp.concatenate([acc[64:72]] * 16, axis=0).T
                row_head = lax.broadcasted_iota(I32, (80, 128), 0) // DH
                lane_head = lax.broadcasted_iota(I32, (80, 128), 1) % 2
                acc = jnp.where(row_head == lane_head, acc, 0.0)
            kv_s[4 * o + j] = acc

    start(cp_phi, cp_c, *kv_copies(0), x_copy(0))
    lax.fori_loop(0, 4, lambda j, _: mod_copy(j).start(), None)
    cp_c.wait()
    cv = c_v[...].astype(F32)
    vec_s[...] = _pack(jnp.broadcast_to(cv * jax.nn.sigmoid(cv), (16, D)))
    cp_phi.wait()
    repeat = ((lax.broadcasted_iota(I32, (128, DH), 0) % 64) // 2
              == lax.broadcasted_iota(I32, (128, DH), 1)).astype(BF)
    block_row = lax.broadcasted_iota(I32, (128, 128), 0)
    same_head = 2 * (block_row // 64) + block_row % 2 == lax.broadcasted_iota(I32, (128, 128), 1) // DH
    for g in range(8):
        full = _dot_nt(repeat, wphi_v[g * 128:(g + 1) * 128, :])
        fmap_s[g * 64:(g + 1) * 64, :] = _pack(jnp.where(same_head, full, 0.0))
    kv_s[...] = jnp.zeros(kv_s.shape, F32)
    wait(*kv_copies(0))
    stage_kv_weights(0)
    x_copy(0).wait()
    xn_s[...] = _normalize(x_v[0:T, :].astype(F32))
    for j in range(4):
        mod_copy(j).wait()
        if j == 2:
            start(*kv_copies(1), *kv_copies(2))
        elif j == 3:
            start(*kv_copies(3))
        col0 = (j % 2) * D + (j // 2) * KH
        modulation(col0, KH)
        if j % 2:
            mod_s[:, col0:col0 + KH] += 1.0
        if j == 1:
            left = [xn_s[k * U:(k + 1) * U, 0:KH] * param(SCALE_A, U, KH) + param(SHIFT_A, U, KH)
                    for k in range(2)]
            h_s[64:128, :] = _pack(left[0])
            h_s[320:384, :] = _pack(left[0] + left[1])
            first_products = kv_products(h_s, 0, 0, ORDER_FIRST)
            first_products.step()
            first_products.step()
    first_norm(0, h_s, 0, normalized=xn_s)

    ops = None
    for o, plan in enumerate(PLAN_FIRST):
        products = kv_products(h_s, (o // 4) * HROWS, o % 4) if o else first_products
        for item in plan.split():
            if item == "p":
                products.step()
            elif item == "W":
                wait(*kv_copies(o + 1))
                if o == 0:
                    x_copy(1).start()
                elif o == 1:
                    start(x_copy(2), x_copy(3))
            elif item == "X":
                wait(x_copy(1), x_copy(2))
                start(*(x_copy(t) for t in range(4, NT)), cp_wr, cp_wq, cp_wo)
                x_copy(3).wait()
            elif item == "s":
                stage_kv_weights(o + 1)
            elif item == "L":
                for t in range(1, 4):
                    first_norm(t, h_s, t * HROWS)
            else:
                accumulate_kv(ops, (o - 1) % 4)
        if o + 1 < len(PLAN_FIRST):
            ops = kv_operands(products.result())
    save_kv_operands(products.result())

    def kv_steps(ops, steps, plans, last_from):
        staged_q = staged_out = 0
        for o, (products, plan) in enumerate(zip(steps, plans)):
            for item in plan.split():
                if item == "p":
                    products.step()
                elif item == "s":
                    stage_q_weights(staged_q)
                    staged_q += 1
                elif item == "o":
                    stage_out_weights(staged_out)
                    staged_out += 1
                elif item == "B":
                    cp_wr.wait()
                else:
                    accumulate_kv(ops, (o - 1) % 4, last=o >= last_from)
            if o + 1 < len(plans):
                ops = kv_operands(products.result())
        return products.result()

    def pass1(i, remaining):
        t = 2 * i + 2
        pl.when(i == 0)(cp_mb.start)
        pl.when(i == 1)(cp_mc.start)
        wait(x_copy(t + 2), x_copy(t + 3))
        view = h_s.at[_rows(t * HROWS, 4 * HROWS)]
        first_norm(t + 2, view, 2 * HROWS)
        first_norm(t + 3, view, 3 * HROWS)
        steps = [kv_products(view, k * HROWS, o) for k in range(2) for o in range(4)]
        save_kv_operands(kv_steps(load_kv_operands(), steps, PLAN_KV, last_from=len(steps)))
        return remaining - 1

    first_tile = lax.fori_loop(0, 2, pass1, 2)

    def q_products(t, o):
        return _Strassen(lambda i: _dot_nt(_unpack(wq_s[(i * 4 + o) * 64:(i * 4 + o + 1) * 64, :]),
                                           _unpack(h_s[_rows(t * HROWS + i * 64, 64), :])), ORDER_Q)

    def derived_params():
        wr8 = wr_v[...].astype(F32)
        wr = jnp.broadcast_to(jnp.concatenate([wr8[j:j + 1, :] for j in range(8)], axis=1), (8, D))
        scale = 1.0 + param(SCALE_B, 8)
        mod_s[:, SCALE_B * D:(SCALE_B + 1) * D] = scale
        router = scale * wr
        tables = (param(GATE_A, 8), router, scale * param(GATE_B, 8), param(SHIFT_B, 8) * param(GATE_B, 8))
        for k, row in enumerate(tables):
            for g in range(8):
                tile = jnp.concatenate([row[:, g * 128:(g + 1) * 128]] * 16, axis=0)
                col_s[k * D + g * 128:k * D + (g + 1) * 128, :] = tile.T
        base = ROUTER_SUMS * D
        mod_s[:, base:base + T] = jnp.broadcast_to(jnp.sum(router, axis=-1, keepdims=True), (8, T))
        mod_s[:, base + T:base + 2 * T] = jnp.broadcast_to(
            jnp.sum(param(SHIFT_B, 8) * wr, axis=-1, keepdims=True), (8, T))

    def column(k, ch):
        v = col_s[k * D + ch:k * D + ch + 128, :]
        return jnp.concatenate([v, v], axis=1)

    def feature_pairs(block, p0):
        out = []
        for j in range(2):
            phi = _hedgehog(block[j * 64:(j + 1) * 64])
            z = z_s[p0 + j]
            inv = _recip(_per_head(phi * jnp.concatenate([z, z], axis=1), jnp.add) + 1e-6)
            out.append((phi.astype(BF), inv))
        return out

    def features(r, o):
        return feature_pairs(r[0], 2 * o) + feature_pairs(r[1], 2 * o + 8)

    def save_features(r):
        raw_s[0:128, :] = r[0]
        for j, (phi, inv) in enumerate(feature_pairs(r[1], 8)):
            carry_s[j * 64:(j + 1) * 64, :] = pltpu.bitcast(phi, U32)
            raw_s[128 + 8 * j:136 + 8 * j, :] = inv

    def load_features():
        done = [(_unpack(carry_s[j * 64:(j + 1) * 64, :]), raw_s[128 + 8 * j:136 + 8 * j, :]) for j in range(2)]
        return feature_pairs(raw_s[0:128, :], 0) + done

    def attend(phis, o):
        heads = {}
        for j in (0, 2, 1, 3):
            phi, inv = phis[j]
            num = _dot(kv_s[2 * o + 8 * (j // 2) + j % 2, 0:64, :].astype(BF), phi)
            heads[j] = jnp.concatenate([num[k * DH:(k + 1) * DH] * inv[k:k + 1] for k in range(2)], axis=0)
        return heads

    def stage_heads(dst, o, j, lo, hi):
        base = o * 64 + j * 32
        terms = _right_terms(lo[:, :U], lo[:, U:], hi[:, :U], hi[:, U:])
        dst[base:base + 32, 0:6 * U] = _pack(jnp.concatenate(terms[:6], axis=1))
        dst[base:base + 16, 6 * U:8 * U] = _pack(jnp.concatenate([terms[6][:32], terms[6][32:]], axis=1))

    def out_products(src, o):
        def product(i):
            if i < 6:
                b = src[:, i * U:(i + 1) * U]
            else:
                b = jnp.concatenate([src[k * 32:k * 32 + 16, (6 + c) * U:(7 + c) * U]
                                     for k in range(8) for c in range(2)], axis=0)
            return _dot(_unpack(wo_s[(i * 4 + o) * 64:(i * 4 + o + 1) * 64, :]), _unpack(b))
        return _Strassen(product, ORDER_OUT)

    def residual(t, o, attn, sums):
        ys = []
        for half, a in enumerate(attn):
            ch = half * KH + o * 128
            ys.append(x_v[_rows(t * T, T), ch:ch + 128].T.astype(F32) + column(COL_GATE_A, ch) * a)
        if sums is None:
            shift = jnp.sum(_fold8(ys[0]) + _fold8(ys[1]), axis=0, keepdims=True) * (1.0 / 256)
            sums = (shift, 0.0, 0.0, 0.0)
        shift, s1, s2, s3 = sums
        for half, y in enumerate(ys):
            ch = half * KH + o * 128
            d = y - shift
            for k in range(2):
                x1_s[_rows((2 * t + k) * D + ch, 128), :] = y[:, k * U:(k + 1) * U]
            s1, s2, s3 = s1 + _fold8(d), s2 + _fold8(d * d), s3 + _fold8(d * column(COL_ROUTER, ch))
        return shift, s1, s2, s3

    def route(t, sums, top):
        m1, i1, m2, i2 = top
        shift = sums[0]
        s1, s2, s3 = (jnp.sum(s, axis=0, keepdims=True) for s in sums[1:])
        delta = s1 * (1.0 / D)
        rstd = lax.rsqrt(jnp.maximum(s2 * (1.0 / D) - delta * delta, 0.0) + 1e-5)
        score = (s3 - delta * mod_s[0:1, ROUTER_SUMS * D:ROUTER_SUMS * D + T]) * rstd
        for k, v in enumerate((shift + delta, rstd)):
            for half in range(2):
                stat_s[_rows(((2 * t + half) * 2 + k) * 8, 8), :] = jnp.broadcast_to(
                    v[:, half * U:(half + 1) * U], (8, U))
        idx = lax.broadcasted_iota(I32, (1, T), 1) + t * T
        g1, g2 = score > m1, score > m2
        return (jnp.where(g1, score, m1), jnp.where(g1, idx, i1),
                jnp.where(g1, m1, jnp.where(g2, score, m2)), jnp.where(g1, i1, jnp.where(g2, idx, i2)))

    def stat(block, k, n):
        return jnp.concatenate([stat_s[_rows((block * 2 + k) * 8, 8), :]] * (n // 8), axis=0)

    def emit(t, ch):
        n = 256
        for half in range(2):
            mean, rstd = (stat(2 * t + half, k, n) for k in range(2))
            x1 = x1_s[_rows((2 * t + half) * D + ch, n), :]
            gain = rstd * col_s[COL_GAIN * D + ch:COL_GAIN * D + ch + n, :]
            res = (x1 + col_s[COL_BIAS * D + ch:COL_BIAS * D + ch + n, :]) + (x1 - mean) * gain
            out_s[_rows(t * T + half * U, U), ch:ch + n] = res.T.astype(BF)

    def q_tile(t, phis, top, plans, current, previous, more=True):
        sums, emitted = None, 0
        for o, plan in enumerate(plans):
            qs = None
            if phis is not None and (o < 3 or more):
                qs = q_products(t, o + 1) if o < 3 else q_products(t + 1, 0)
            ws = out_products(previous, o)
            heads, staged = None, 0
            for item in plan.split():
                if item == "q":
                    qs.step()
                elif item == "w":
                    ws.step()
                    if ws.done:
                        sums = residual(t - 1, o, ws.result(), sums)
                elif item == "N":
                    heads = attend(phis, o)
                elif item == "c":
                    stage_heads(current, o, staged, heads[staged], heads[staged + 2])
                    staged += 1
                elif item == "E":
                    emit(t - 2, emitted * 256)
                    emitted += 1
                elif item == "M":
                    modulation((GATE_A + o) * D, D)
            if qs is not None:
                phis = features(qs.result(), o + 1) if o < 3 else qs.result()
        if sums is not None:
            top = route(t - 1, sums, top)
        if emitted:
            out_copy(t - 2).start()
        return phis, top

    wait(cp_wq, cp_wo, cp_mb, cp_mc)
    start(cp_wg, cp_wu)
    steps = [kv_products(h_s, t * HROWS, o) for t in (NT - 2, NT - 1) for o in range(4)]
    r = kv_steps(load_kv_operands(), steps + [q_products(first_tile, 0)], PLAN_KV_LAST, last_from=5)
    lowest = jnp.full((1, T), -jnp.inf, F32)
    zero = jnp.zeros((1, T), I32)
    top = (lowest, zero, lowest, zero)
    r, top = q_tile(first_tile, features(r, 0), top, PLAN_Q_FIRST, oa_s, ob_s)
    derived_params()
    r, top = q_tile(first_tile + 1, features(r, 0), top, PLAN_Q_SECOND, ob_s, oa_s)
    save_features(r)

    def pass2(i, carry):
        top, tile = carry
        pl.when(i == 2)(cp_wd.start)
        r, top = q_tile(2 * i - 2, load_features(), top, PLAN_Q, oa_s, ob_s)
        r, top = q_tile(2 * i - 1, features(r, 0), top, PLAN_Q, ob_s, oa_s)
        save_features(r)
        return top, tile + 2

    top, tile = lax.fori_loop(2, 4, pass2, (top, 2))
    wait(cp_wg, cp_wu, cp_wd)
    r, top = q_tile(tile, load_features(), top, PLAN_Q_LATE, oa_s, ob_s)
    _, top = q_tile(tile + 1, features(r, 0), top, PLAN_Q_LAST, ob_s, oa_s, more=False)
    _, top = q_tile(tile + 2, None, top, PLAN_DRAIN, oa_s, ob_s)

    m1, i1, m2, i2 = top
    best = jnp.max(m1, axis=1, keepdims=True)
    ia = jnp.min(jnp.where(m1 == best, i1, S - 1), axis=1, keepdims=True)
    taken = i1 == ia
    rest, rest_idx = jnp.where(taken, m2, m1), jnp.where(taken, i2, i1)
    second = jnp.max(rest, axis=1, keepdims=True)
    ib = jnp.min(jnp.where(rest == second, rest_idx, S - 1), axis=1, keepdims=True)
    idx = (jnp.clip(ia[0, 0], 0, S - 1), jnp.clip(ib[0, 0], 0, S - 1))

    for g in range(4):
        emit(NT - 1, g * 256)
    out_copy(NT - 1).start()
    out_copy(0).wait()

    row16 = lax.broadcasted_iota(I32, (16, U), 0)
    lane16 = lax.broadcasted_iota(I32, (16, U), 1)
    xn_sel = 0.0
    for k in range(2):
        block = idx[k] // U
        xn = (x1_s[_rows(block * D, D), :] - stat(block, 0, D)) * stat(block, 1, D)
        pick = jnp.where((row16 == k) & (lane16 == idx[k] % U), 1.0, 0.0).astype(BF)
        xn_sel = xn_sel + _dot_nt(pick, xn.astype(BF))
    hs = (xn_sel * param(SCALE_B, 16) + param(SHIFT_B, 16)).astype(BF)
    score = jnp.where(row16[:, 0:1] == 0, best, second) + mod_s[0:1, ROUTER_SUMS * D + T:ROUTER_SUMS * D + T + 1]
    gate = jax.nn.sigmoid(score)

    y = jnp.zeros((16, D), F32)
    for j in range(F // FC):
        gj = _dot(hs, wg_v[:, j * FC:(j + 1) * FC])
        uj = _dot(hs, wu_v[:, j * FC:(j + 1) * FC])
        y = y + _dot((gj * jax.nn.sigmoid(gj) * uj).astype(BF), wd_v[j * FC:(j + 1) * FC, 0:D])
    update = param(GATE_B, 16) * (y * gate)

    wait(*(out_copy(t) for t in range(1, NT)))
    row = lax.broadcasted_iota(I32, (16, D), 0)

    def patch(k):
        base = pl.multiple_of((idx[k] // 16) * 16, 16)
        block = out_s[pl.ds(base, 16), :].astype(F32)
        out_s[pl.ds(base, 16), :] = jnp.where(row == idx[k] - base, block + update[k:k + 1, :], block).astype(BF)
        return pltpu.make_async_copy(out_s.at[pl.ds(base, 16)], out_hbm.at[pl.ds(base, 16)], sem_p.at[k])

    patch_a, patch_b = patch(0), patch(1)
    patch_a.start()

    @pl.when(idx[0] // 16 != idx[1] // 16)
    def _():
        patch_b.start()
        patch_b.wait()

    patch_a.wait()


@jax.jit
def pallas_adaLN_cond__linear_kernel_hedgehog__moe_arch_mod__prompt_kernel(
        A_x, A_wqkv, A_w_phi, A_wo, B_x, B_w_r, B_w_gate, B_w_up, B_w_down, c, w_mod):
    del B_x
    hbm = pl.BlockSpec(memory_space=pl.ANY)
    out = pl.pallas_call(
        _kernel,
        out_shape=jax.ShapeDtypeStruct((S, D), BF),
        in_specs=[hbm] * 10,
        out_specs=hbm,
        scratch_shapes=[
            pltpu.VMEM((S, D), BF),
            pltpu.VMEM((D, 3 * D + PAD), BF),
            pltpu.VMEM((H * DH, DH), BF),
            pltpu.VMEM((D, D + PAD), BF),
            pltpu.VMEM((8, 128), BF),
            pltpu.VMEM((D, F + PAD), BF),
            pltpu.VMEM((D, F + PAD), BF),
            pltpu.VMEM((F, D + PAD), BF),
            pltpu.VMEM((1, D), BF),
            pltpu.VMEM((D, 6 * D + PAD), BF),
            pltpu.VMEM((7 * 512, KH), U32),
            pltpu.VMEM((7 * 256, KH), U32),
            pltpu.VMEM((7 * 256, KH), U32),
            pltpu.VMEM((NT * HROWS, KH), U32),
            pltpu.VMEM((NPAIR, 80, 128), F32),
            pltpu.VMEM((8, 6 * D + 2 * T), F32),
            pltpu.VMEM((4 * D, 128), F32),
            pltpu.VMEM((2 * NT * D, U), F32),
            pltpu.VMEM((2 * NT * 2 * 8, U), F32),
            pltpu.VMEM((S, D), BF),
            pltpu.VMEM((8 * 64, 128), U32),
            pltpu.VMEM((KH // 2, 8 * U), U32),
            pltpu.VMEM((KH // 2, 8 * U), U32),
            pltpu.VMEM((8, D), U32),
            pltpu.VMEM((T, D), F32),
            pltpu.VMEM((192, T), U32),
            pltpu.VMEM((256, T), F32),
            pltpu.VMEM((NPAIR, 128, U), F32),
            pltpu.SemaphoreType.DMA((10,)),
            pltpu.SemaphoreType.DMA((4,)),
            pltpu.SemaphoreType.DMA((4,)),
            pltpu.SemaphoreType.DMA((4,)),
            pltpu.SemaphoreType.DMA((NT,)),
            pltpu.SemaphoreType.DMA((NT,)),
            pltpu.SemaphoreType.DMA((2,)),
        ],
        compiler_params=pltpu.CompilerParams(
            vmem_limit_bytes=110 * 2**20,
            flags={"XLA_TPU_EVENLY_DISTRIBUTE_CRITICAL_NODES": True}),
        name="fused_block",
    )(A_x.reshape(S, D), A_wqkv, A_w_phi.reshape(H * DH, DH), A_wo, B_w_r.reshape(8, 128),
      B_w_gate, B_w_up, B_w_down, c, w_mod)
    return out.reshape(1, S, D)
```

```python
import math

import jax
import jax.numpy as jnp
from jax import lax
import jax.experimental.pallas as pl
import jax.experimental.pallas.tpu as pltpu

S, D, H, DH, F = 2048, 1024, 32, 32, 3584
U = 128
T = 2 * U
NT = S // T
KH = D // 2
NPAIR = H // 2
HROWS = 7 * U // 2
PAD = 128
FC = F // 2
LN_ROWS = 32
LOG2E = math.log2(math.e)
BF, F32, U32, I32 = jnp.bfloat16, jnp.float32, jnp.uint32, jnp.int32

SHIFT_A, SCALE_A, GATE_A, SHIFT_B, SCALE_B, GATE_B, ROUTER_SUMS = range(7)
COL_GATE_A, COL_ROUTER, COL_GAIN, COL_BIAS = range(4)

PLAN_FIRST = (
    "p p p p W s p", "p p N p p W s p p p",
    "p N p p W s p p p p", "p p X L N p p p p p",
    "p p p N p p p p", "p p p p N p p p",
    "p p p p p N p p", "p p N p p p p p")
PLAN_KV = (
    "p p N p p p p p", "p N p p p p p p",
    "p p N p p p p p", "p p p p p N p p",
    "p p p N p p p p", "p N p p p p p p",
    "p p p N p p p p", "p p p p p N p p")
PLAN_KV_LAST = (
    "p p p N p p p p o", "p p p N p p p p o",
    "p p p N p p p p o", "p p N p p p p p o",
    "B p p p N s p p p p", "p N p s p p p p p",
    "p p s p p p N p p", "s p p p p p N p p",
    "p p p N p p p p")
PLAN_Q_FIRST = (
    "q q q M q N c c q q q", "q q M N c c q q q q q",
    "q q M N c c q q q q q", "q M N c c q q q q q q")
PLAN_Q_SECOND = (
    "w w w w w w w q q q N c c q q q q", "w w w w w w w q N c c q q q q q q",
    "w w w w w N c c w w q q q q q q q", "w w w w w w w q q N c c q q q q q")
PLAN_Q = (
    "w w w w w w N c c w q q q q q q q E", "w w w w w N c c w w q q q q q q E q",
    "w w w w w N c c w w q q q q q q q E", "w w w w w w w q N c c q q q q q q E")
PLAN_Q_LATE = (
    "w N c c w w w w w w q q q q q q q E", "w w w w w w w q N c c q q q q q q E",
    "w w w w N c c w w w q q q q q q q E", "w w w w w w w q q q q q q N c c q E")
PLAN_Q_LAST = (
    "w w w w w w w q q q q N c c q q q E", "w w w w w w w q q q N c c q q q E q",
    "w w w w w w w q q N c c q q q q q E", "w w w w w w N c c w E")
PLAN_DRAIN = (
    "w w w w E w w w E", "w w w w w E w w",
    "w w w w w w w E", "w w w w w w w")
ORDER_FIRST = (6, 2, 1, 3, 4, 5, 7)
ORDER_KV = (1, 2, 3, 6, 4, 5, 7)
ORDER_Q = (4, 3, 2, 5, 1, 6, 7)
ORDER_OUT = (4, 7, 3, 1, 5, 2, 6)


def _dot(a, b):
    return jnp.dot(a, b, preferred_element_type=F32)


def _dot_nt(a, b):
    return lax.dot_general(a, b, (((1,), (1,)), ((), ())), preferred_element_type=F32)


def _pack(v):
    return pltpu.bitcast(v.astype(BF), U32)


def _unpack(v):
    return pltpu.bitcast(v, BF)


def _recip(v):
    return pl.reciprocal(v, approx=False, full_range=False)


def _rows(start, size):
    return pl.ds(start if isinstance(start, int) else pl.multiple_of(start, 8), size)


def _normalize(v):
    centered = v - jnp.mean(v, axis=-1, keepdims=True)
    var = jnp.mean(centered * centered, axis=-1, keepdims=True)
    return centered * lax.rsqrt(var + 1e-5)


def _fold8(v, op=jnp.add):
    parts = [v[i:i + 8] for i in range(0, v.shape[0], 8)]
    while len(parts) > 1:
        parts = [op(parts[i], parts[i + 1]) for i in range(0, len(parts), 2)]
    return parts[0]


def _per_head(v, op):
    r = _fold8(v, op)
    r = op(r, pltpu.roll(r, 4, 0))
    return op(r, pltpu.roll(r, 2, 0))


def _hedgehog(p):
    def spread(v):
        return jnp.concatenate([v] * 8, axis=0)

    pos = jnp.exp2(p - spread(_per_head(p, jnp.maximum)))
    neg = jnp.exp2(spread(_per_head(p, jnp.minimum)) - p)
    pos = pos * spread(_recip(_per_head(pos, jnp.add)))
    neg = neg * spread(_recip(_per_head(neg, jnp.add)))
    return jnp.concatenate([pos, neg], axis=0)


def _left_terms(a11, a12, a21, a22):
    return a11 + a22, a21 + a22, a11, a22, a11 + a12, a21 - a11, a12 - a22


def _right_terms(b11, b12, b21, b22):
    return b11 + b22, b11, b12 - b22, b21 - b11, b22, b11 + b12, b21 + b22


class _Strassen:
    _USES = {1: ((0, 1), (3, 1)), 2: ((2, 1), (3, -1)), 3: ((1, 1), (3, 1)), 4: ((0, 1), (2, 1)),
             5: ((0, -1), (1, 1)), 6: ((3, 1),), 7: ((0, 1),)}

    def __init__(self, product, order):
        self._product = product
        self._todo = list(order)
        self._c = [None] * 4

    @property
    def done(self):
        return not self._todo

    def step(self):
        i = self._todo.pop(0)
        m = self._product(i - 1)
        for k, sign in self._USES[i]:
            if self._c[k] is None:
                assert sign > 0
                self._c[k] = m
            else:
                self._c[k] = self._c[k] + m if sign > 0 else self._c[k] - m

    def result(self):
        assert self.done
        return jnp.concatenate(self._c[:2], axis=1), jnp.concatenate(self._c[2:], axis=1)


def _kernel(x_hbm, wqkv_hbm, wphi_hbm, wo_hbm, wr_hbm, wg_hbm, wu_hbm, wd_hbm, c_hbm, wmod_hbm,
            out_hbm,
            x_v, wqkv_v, wphi_v, wo_v, wr_v, wg_v, wu_v, wd_v, c_v, wmod_v,
            wkv_s, wq_s, wo_s, h_s, kv_s, mod_s, col_s, x1_s, stat_s, out_s, fmap_s,
            oa_s, ob_s, vec_s, xn_s, carry_s, raw_s, z_s,
            sem_w, sem_m, sem_k, sem_v, sem_x, sem_o, sem_p):
    def wcopy(i, src, dst):
        return pltpu.make_async_copy(src, dst, sem_w.at[i])

    cp_c = wcopy(0, c_hbm, c_v)
    cp_phi = wcopy(1, wphi_hbm, wphi_v)
    cp_wr = wcopy(2, wr_hbm, wr_v)
    cp_wq = wcopy(3, wqkv_hbm.at[:, 0:D], wqkv_v.at[:, 0:D])
    cp_mb = wcopy(4, wmod_hbm.at[:, 2 * D:4 * D], wmod_v.at[:, 2 * D:4 * D])
    cp_mc = wcopy(5, wmod_hbm.at[:, 4 * D:6 * D], wmod_v.at[:, 4 * D:6 * D])
    cp_wo = wcopy(6, wo_hbm, wo_v.at[:, 0:D])
    cp_wg = wcopy(7, wg_hbm, wg_v.at[:, 0:F])
    cp_wu = wcopy(8, wu_hbm, wu_v.at[:, 0:F])
    cp_wd = wcopy(9, wd_hbm, wd_v.at[:, 0:D])

    def mod_copy(j):
        col0 = (j % 2) * D + (j // 2) * KH
        cols = pl.ds(col0 if isinstance(j, int) else pl.multiple_of(col0, KH), KH)
        return pltpu.make_async_copy(wmod_hbm.at[:, cols], wmod_v.at[:, cols], sem_m.at[j])

    def kv_copies(o):
        ck, cv = pl.ds(D + o * 256, 256), pl.ds(2 * D + o * 256, 256)
        return (pltpu.make_async_copy(wqkv_hbm.at[:, ck], wqkv_v.at[:, ck], sem_k.at[o]),
                pltpu.make_async_copy(wqkv_hbm.at[:, cv], wqkv_v.at[:, cv], sem_v.at[o]))

    def x_copy(t):
        rows = _rows(t * T, T)
        return pltpu.make_async_copy(x_hbm.at[rows], x_v.at[rows], sem_x.at[t])

    def out_copy(t):
        rows = _rows(t * T, T)
        return pltpu.make_async_copy(out_s.at[rows], out_hbm.at[rows], sem_o.at[t])

    def start(*copies):
        for cp in copies:
            cp.start()

    def wait(*copies):
        for cp in copies:
            cp.wait()

    def fold(col0, g):
        return _dot_nt(_unpack(fmap_s[g * 64:(g + 1) * 64, :]),
                       wqkv_v[:, col0 + g * 128:col0 + (g + 1) * 128]) * LOG2E

    def stage_left(dst, o, upper, lower):
        n = upper.shape[0] // 2
        for i, a in enumerate(_left_terms(upper[:, :KH], upper[:, KH:], lower[:, :KH], lower[:, KH:])):
            dst[(i * 4 + o) * n:(i * 4 + o + 1) * n, :] = _pack(a)

    def stage_kv_weights(o):
        blocks = []
        for g in (2 * o, 2 * o + 1):
            fk = fold(D, g)
            fv = wqkv_v[:, 2 * D + g * 128:2 * D + (g + 1) * 128].T.astype(F32)
            blocks.append(jnp.concatenate([fk[:64], fv[:64], fk[64:], fv[64:]], axis=0))
        stage_left(wkv_s, o, *blocks)

    def stage_q_weights(o):
        stage_left(wq_s, o, fold(0, o), fold(0, o + 4))

    def stage_out_weights(o):
        stage_left(wo_s, o, wo_v[:, o * 128:(o + 1) * 128].T.astype(F32),
                   wo_v[:, KH + o * 128:KH + (o + 1) * 128].T.astype(F32))

    def param(k, n, width=D):
        return jnp.concatenate([mod_s[:, k * D:k * D + width]] * (n // 8), axis=0)

    def modulation(col0, n):
        mod_s[:, col0:col0 + n] = _dot(_unpack(vec_s[...]), wmod_v[:, col0:col0 + n])[0:8]

    def first_norm(t, dst, base, normalized=None):
        for r0 in range(0, U, LN_ROWS):
            h = []
            for half in range(2):
                rows = _rows(t * T + half * U + r0, LN_ROWS)
                xn = _normalize(x_v[rows, :].astype(F32)) if normalized is None else normalized[rows, :]
                h.append(xn * param(SCALE_A, LN_ROWS) + param(SHIFT_A, LN_ROWS))
            for i, b in enumerate(_right_terms(h[0][:, :KH], h[1][:, :KH], h[0][:, KH:], h[1][:, KH:])):
                dst[base + i * 64 + r0 // 2:base + i * 64 + (r0 + LN_ROWS) // 2, :] = _pack(b)

    def kv_products(src, base, o, order=ORDER_KV):
        return _Strassen(lambda i: _dot_nt(_unpack(wkv_s[(i * 4 + o) * 128:(i * 4 + o + 1) * 128, :]),
                                           _unpack(src[base + i * 64:base + (i + 1) * 64, :])), order)

    def kv_pairs(block):
        return [(block[j * 128 + 64:(j + 1) * 128].astype(BF), _hedgehog(block[j * 128:j * 128 + 64]).astype(BF))
                for j in range(2)]

    def kv_operands(r):
        return kv_pairs(r[0]) + kv_pairs(r[1])

    def save_kv_operands(r):
        raw_s[...] = r[0]
        for j, (v, phi) in enumerate(kv_pairs(r[1])):
            carry_s[j * 64:(j + 1) * 64, :] = pltpu.bitcast(phi, U32)
            carry_s[128 + j * 32:128 + (j + 1) * 32, :] = pltpu.bitcast(v, U32)

    def load_kv_operands():
        done = [(_unpack(carry_s[128 + j * 32:128 + (j + 1) * 32, :]), _unpack(carry_s[j * 64:(j + 1) * 64, :]))
                for j in range(2)]
        return kv_pairs(raw_s[...]) + done

    def accumulate_kv(ops, o, last=False):
        ones = jnp.ones((16, T), BF)
        for j, (v, phi) in enumerate(ops):
            acc = _dot_nt(jnp.concatenate([v, ones], axis=0), phi) + kv_s[4 * o + j]
            if last:
                z_s[4 * o + j] = jnp.concatenate([acc[64:72]] * 16, axis=0).T
                row_head = lax.broadcasted_iota(I32, (80, 128), 0) // DH
                lane_head = lax.broadcasted_iota(I32, (80, 128), 1) % 2
                acc = jnp.where(row_head == lane_head, acc, 0.0)
            kv_s[4 * o + j] = acc

    start(cp_phi, cp_c, *kv_copies(0), x_copy(0))
    lax.fori_loop(0, 4, lambda j, _: mod_copy(j).start(), None)
    cp_c.wait()
    cv = c_v[...].astype(F32)
    vec_s[...] = _pack(jnp.broadcast_to(cv * jax.nn.sigmoid(cv), (16, D)))
    cp_phi.wait()
    repeat = ((lax.broadcasted_iota(I32, (128, DH), 0) % 64) // 2
              == lax.broadcasted_iota(I32, (128, DH), 1)).astype(BF)
    block_row = lax.broadcasted_iota(I32, (128, 128), 0)
    same_head = 2 * (block_row // 64) + block_row % 2 == lax.broadcasted_iota(I32, (128, 128), 1) // DH
    for g in range(8):
        full = _dot_nt(repeat, wphi_v[g * 128:(g + 1) * 128, :])
        fmap_s[g * 64:(g + 1) * 64, :] = _pack(jnp.where(same_head, full, 0.0))
    kv_s[...] = jnp.zeros(kv_s.shape, F32)
    wait(*kv_copies(0))
    stage_kv_weights(0)
    x_copy(0).wait()
    xn_s[...] = _normalize(x_v[0:T, :].astype(F32))
    for j in range(4):
        mod_copy(j).wait()
        if j == 2:
            start(*kv_copies(1), *kv_copies(2))
        elif j == 3:
            start(*kv_copies(3))
        col0 = (j % 2) * D + (j // 2) * KH
        modulation(col0, KH)
        if j % 2:
            mod_s[:, col0:col0 + KH] += 1.0
        if j == 1:
            left = [xn_s[k * U:(k + 1) * U, 0:KH] * param(SCALE_A, U, KH) + param(SHIFT_A, U, KH)
                    for k in range(2)]
            h_s[64:128, :] = _pack(left[0])
            h_s[320:384, :] = _pack(left[0] + left[1])
            first_products = kv_products(h_s, 0, 0, ORDER_FIRST)
            first_products.step()
            first_products.step()
    first_norm(0, h_s, 0, normalized=xn_s)

    ops = None
    for o, plan in enumerate(PLAN_FIRST):
        products = kv_products(h_s, (o // 4) * HROWS, o % 4) if o else first_products
        for item in plan.split():
            if item == "p":
                products.step()
            elif item == "W":
                wait(*kv_copies(o + 1))
                if o == 0:
                    x_copy(1).start()
                elif o == 1:
                    start(x_copy(2), x_copy(3))
            elif item == "X":
                wait(x_copy(1), x_copy(2))
                start(*(x_copy(t) for t in range(4, NT)), cp_wr, cp_wq, cp_wo)
                x_copy(3).wait()
            elif item == "s":
                stage_kv_weights(o + 1)
            elif item == "L":
                for t in range(1, 4):
                    first_norm(t, h_s, t * HROWS)
            else:
                accumulate_kv(ops, (o - 1) % 4)
        if o + 1 < len(PLAN_FIRST):
            ops = kv_operands(products.result())
    save_kv_operands(products.result())

    def kv_steps(ops, steps, plans, last_from):
        staged_q = staged_out = 0
        for o, (products, plan) in enumerate(zip(steps, plans)):
            for item in plan.split():
                if item == "p":
                    products.step()
                elif item == "s":
                    stage_q_weights(staged_q)
                    staged_q += 1
                elif item == "o":
                    stage_out_weights(staged_out)
                    staged_out += 1
                elif item == "B":
                    cp_wr.wait()
                else:
                    accumulate_kv(ops, (o - 1) % 4, last=o >= last_from)
            if o + 1 < len(plans):
                ops = kv_operands(products.result())
        return products.result()

    def pass1(i, remaining):
        t = 2 * i + 2
        pl.when(i == 0)(cp_mb.start)
        pl.when(i == 1)(cp_mc.start)
        wait(x_copy(t + 2), x_copy(t + 3))
        view = h_s.at[_rows(t * HROWS, 4 * HROWS)]
        first_norm(t + 2, view, 2 * HROWS)
        first_norm(t + 3, view, 3 * HROWS)
        steps = [kv_products(view, k * HROWS, o) for k in range(2) for o in range(4)]
        save_kv_operands(kv_steps(load_kv_operands(), steps, PLAN_KV, last_from=len(steps)))
        return remaining - 1

    first_tile = lax.fori_loop(0, 2, pass1, 2)

    def q_products(t, o):
        return _Strassen(lambda i: _dot_nt(_unpack(wq_s[(i * 4 + o) * 64:(i * 4 + o + 1) * 64, :]),
                                           _unpack(h_s[_rows(t * HROWS + i * 64, 64), :])), ORDER_Q)

    def derived_params():
        wr8 = wr_v[...].astype(F32)
        wr = jnp.broadcast_to(jnp.concatenate([wr8[j:j + 1, :] for j in range(8)], axis=1), (8, D))
        scale = 1.0 + param(SCALE_B, 8)
        mod_s[:, SCALE_B * D:(SCALE_B + 1) * D] = scale
        router = scale * wr
        tables = (param(GATE_A, 8), router, scale * param(GATE_B, 8), param(SHIFT_B, 8) * param(GATE_B, 8))
        for k, row in enumerate(tables):
            for g in range(8):
                tile = jnp.concatenate([row[:, g * 128:(g + 1) * 128]] * 16, axis=0)
                col_s[k * D + g * 128:k * D + (g + 1) * 128, :] = tile.T
        base = ROUTER_SUMS * D
        mod_s[:, base:base + T] = jnp.broadcast_to(jnp.sum(router, axis=-1, keepdims=True), (8, T))
        mod_s[:, base + T:base + 2 * T] = jnp.broadcast_to(
            jnp.sum(param(SHIFT_B, 8) * wr, axis=-1, keepdims=True), (8, T))

    def column(k, ch):
        v = col_s[k * D + ch:k * D + ch + 128, :]
        return jnp.concatenate([v, v], axis=1)

    def feature_pairs(block, p0):
        out = []
        for j in range(2):
            phi = _hedgehog(block[j * 64:(j + 1) * 64])
            z = z_s[p0 + j]
            inv = _recip(_per_head(phi * jnp.concatenate([z, z], axis=1), jnp.add) + 1e-6)
            out.append((phi.astype(BF), inv))
        return out

    def features(r, o):
        return feature_pairs(r[0], 2 * o) + feature_pairs(r[1], 2 * o + 8)

    def save_features(r):
        raw_s[0:128, :] = r[0]
        for j, (phi, inv) in enumerate(feature_pairs(r[1], 8)):
            carry_s[j * 64:(j + 1) * 64, :] = pltpu.bitcast(phi, U32)
            raw_s[128 + 8 * j:136 + 8 * j, :] = inv

    def load_features():
        done = [(_unpack(carry_s[j * 64:(j + 1) * 64, :]), raw_s[128 + 8 * j:136 + 8 * j, :]) for j in range(2)]
        return feature_pairs(raw_s[0:128, :], 0) + done

    def attend(phis, o):
        heads = {}
        for j in (0, 2, 1, 3):
            phi, inv = phis[j]
            num = _dot(kv_s[2 * o + 8 * (j // 2) + j % 2, 0:64, :].astype(BF), phi)
            heads[j] = jnp.concatenate([num[k * DH:(k + 1) * DH] * inv[k:k + 1] for k in range(2)], axis=0)
        return heads

    def stage_heads(dst, o, j, lo, hi):
        base = o * 64 + j * 32
        terms = _right_terms(lo[:, :U], lo[:, U:], hi[:, :U], hi[:, U:])
        dst[base:base + 32, 0:6 * U] = _pack(jnp.concatenate(terms[:6], axis=1))
        dst[base:base + 16, 6 * U:8 * U] = _pack(jnp.concatenate([terms[6][:32], terms[6][32:]], axis=1))

    def out_products(src, o):
        def product(i):
            if i < 6:
                b = src[:, i * U:(i + 1) * U]
            else:
                b = jnp.concatenate([src[k * 32:k * 32 + 16, (6 + c) * U:(7 + c) * U]
                                     for k in range(8) for c in range(2)], axis=0)
            return _dot(_unpack(wo_s[(i * 4 + o) * 64:(i * 4 + o + 1) * 64, :]), _unpack(b))
        return _Strassen(product, ORDER_OUT)

    def residual(t, o, attn, sums):
        ys = []
        for half, a in enumerate(attn):
            ch = half * KH + o * 128
            ys.append(x_v[_rows(t * T, T), ch:ch + 128].T.astype(F32) + column(COL_GATE_A, ch) * a)
        if sums is None:
            shift = jnp.sum(_fold8(ys[0]) + _fold8(ys[1]), axis=0, keepdims=True) * (1.0 / 256)
            sums = (shift, 0.0, 0.0, 0.0)
        shift, s1, s2, s3 = sums
        for half, y in enumerate(ys):
            ch = half * KH + o * 128
            d = y - shift
            for k in range(2):
                x1_s[_rows((2 * t + k) * D + ch, 128), :] = y[:, k * U:(k + 1) * U]
            s1, s2, s3 = s1 + _fold8(d), s2 + _fold8(d * d), s3 + _fold8(d * column(COL_ROUTER, ch))
        return shift, s1, s2, s3

    def route(t, sums, top):
        m1, i1, m2, i2 = top
        shift = sums[0]
        s1, s2, s3 = (jnp.sum(s, axis=0, keepdims=True) for s in sums[1:])
        delta = s1 * (1.0 / D)
        rstd = lax.rsqrt(jnp.maximum(s2 * (1.0 / D) - delta * delta, 0.0) + 1e-5)
        score = (s3 - delta * mod_s[0:1, ROUTER_SUMS * D:ROUTER_SUMS * D + T]) * rstd
        for k, v in enumerate((shift + delta, rstd)):
            for half in range(2):
                stat_s[_rows(((2 * t + half) * 2 + k) * 8, 8), :] = jnp.broadcast_to(
                    v[:, half * U:(half + 1) * U], (8, U))
        idx = lax.broadcasted_iota(I32, (1, T), 1) + t * T
        g1, g2 = score > m1, score > m2
        return (jnp.where(g1, score, m1), jnp.where(g1, idx, i1),
                jnp.where(g1, m1, jnp.where(g2, score, m2)), jnp.where(g1, i1, jnp.where(g2, idx, i2)))

    def stat(block, k, n):
        return jnp.concatenate([stat_s[_rows((block * 2 + k) * 8, 8), :]] * (n // 8), axis=0)

    def emit(t, ch):
        n = 256
        for half in range(2):
            mean, rstd = (stat(2 * t + half, k, n) for k in range(2))
            x1 = x1_s[_rows((2 * t + half) * D + ch, n), :]
            gain = rstd * col_s[COL_GAIN * D + ch:COL_GAIN * D + ch + n, :]
            res = (x1 + col_s[COL_BIAS * D + ch:COL_BIAS * D + ch + n, :]) + (x1 - mean) * gain
            out_s[_rows(t * T + half * U, U), ch:ch + n] = res.T.astype(BF)

    def q_tile(t, phis, top, plans, current, previous, more=True):
        sums, emitted = None, 0
        for o, plan in enumerate(plans):
            qs = None
            if phis is not None and (o < 3 or more):
                qs = q_products(t, o + 1) if o < 3 else q_products(t + 1, 0)
            ws = out_products(previous, o)
            heads, staged = None, 0
            for item in plan.split():
                if item == "q":
                    qs.step()
                elif item == "w":
                    ws.step()
                    if ws.done:
                        sums = residual(t - 1, o, ws.result(), sums)
                elif item == "N":
                    heads = attend(phis, o)
                elif item == "c":
                    stage_heads(current, o, staged, heads[staged], heads[staged + 2])
                    staged += 1
                elif item == "E":
                    emit(t - 2, emitted * 256)
                    emitted += 1
                elif item == "M":
                    modulation((GATE_A + o) * D, D)
            if qs is not None:
                phis = features(qs.result(), o + 1) if o < 3 else qs.result()
        if sums is not None:
            top = route(t - 1, sums, top)
        if emitted:
            out_copy(t - 2).start()
        return phis, top

    wait(cp_wq, cp_wo, cp_mb, cp_mc)
    start(cp_wg, cp_wu)
    steps = [kv_products(h_s, t * HROWS, o) for t in (NT - 2, NT - 1) for o in range(4)]
    r = kv_steps(load_kv_operands(), steps + [q_products(first_tile, 0)], PLAN_KV_LAST, last_from=5)
    lowest = jnp.full((1, T), -jnp.inf, F32)
    zero = jnp.zeros((1, T), I32)
    top = (lowest, zero, lowest, zero)
    r, top = q_tile(first_tile, features(r, 0), top, PLAN_Q_FIRST, oa_s, ob_s)
    derived_params()
    r, top = q_tile(first_tile + 1, features(r, 0), top, PLAN_Q_SECOND, ob_s, oa_s)
    save_features(r)

    def pass2(i, carry):
        top, tile = carry
        pl.when(i == 2)(cp_wd.start)
        r, top = q_tile(2 * i - 2, load_features(), top, PLAN_Q, oa_s, ob_s)
        r, top = q_tile(2 * i - 1, features(r, 0), top, PLAN_Q, ob_s, oa_s)
        save_features(r)
        return top, tile + 2

    top, tile = lax.fori_loop(2, 4, pass2, (top, 2))
    wait(cp_wg, cp_wu, cp_wd)
    r, top = q_tile(tile, load_features(), top, PLAN_Q_LATE, oa_s, ob_s)
    _, top = q_tile(tile + 1, features(r, 0), top, PLAN_Q_LAST, ob_s, oa_s, more=False)
    _, top = q_tile(tile + 2, None, top, PLAN_DRAIN, oa_s, ob_s)

    m1, i1, m2, i2 = top
    best = jnp.max(m1, axis=1, keepdims=True)
    ia = jnp.min(jnp.where(m1 == best, i1, S - 1), axis=1, keepdims=True)
    taken = i1 == ia
    rest, rest_idx = jnp.where(taken, m2, m1), jnp.where(taken, i2, i1)
    second = jnp.max(rest, axis=1, keepdims=True)
    ib = jnp.min(jnp.where(rest == second, rest_idx, S - 1), axis=1, keepdims=True)
    idx = (jnp.clip(ia[0, 0], 0, S - 1), jnp.clip(ib[0, 0], 0, S - 1))

    for g in range(4):
        emit(NT - 1, g * 256)
    out_copy(NT - 1).start()
    out_copy(0).wait()

    row16 = lax.broadcasted_iota(I32, (16, U), 0)
    lane16 = lax.broadcasted_iota(I32, (16, U), 1)
    xn_sel = 0.0
    for k in range(2):
        block = idx[k] // U
        xn = (x1_s[_rows(block * D, D), :] - stat(block, 0, D)) * stat(block, 1, D)
        pick = jnp.where((row16 == k) & (lane16 == idx[k] % U), 1.0, 0.0).astype(BF)
        xn_sel = xn_sel + _dot_nt(pick, xn.astype(BF))
    hs = (xn_sel * param(SCALE_B, 16) + param(SHIFT_B, 16)).astype(BF)
    score = jnp.where(row16[:, 0:1] == 0, best, second) + mod_s[0:1, ROUTER_SUMS * D + T:ROUTER_SUMS * D + T + 1]
    gate = jax.nn.sigmoid(score)

    y = jnp.zeros((16, D), F32)
    for j in range(F // FC):
        gj = _dot(hs, wg_v[:, j * FC:(j + 1) * FC])
        uj = _dot(hs, wu_v[:, j * FC:(j + 1) * FC])
        y = y + _dot((gj * jax.nn.sigmoid(gj) * uj).astype(BF), wd_v[j * FC:(j + 1) * FC, 0:D])
    update = param(GATE_B, 16) * (y * gate)

    wait(*(out_copy(t) for t in range(1, NT)))
    row = lax.broadcasted_iota(I32, (16, D), 0)

    def patch(k):
        base = pl.multiple_of((idx[k] // 16) * 16, 16)
        block = out_s[pl.ds(base, 16), :].astype(F32)
        out_s[pl.ds(base, 16), :] = jnp.where(row == idx[k] - base, block + update[k:k + 1, :], block).astype(BF)
        return pltpu.make_async_copy(out_s.at[pl.ds(base, 16)], out_hbm.at[pl.ds(base, 16)], sem_p.at[k])

    patch_a, patch_b = patch(0), patch(1)
    patch_a.start()

    @pl.when(idx[0] // 16 != idx[1] // 16)
    def _():
        patch_b.start()
        patch_b.wait()

    patch_a.wait()


@jax.jit
def pallas_adaLN_cond__linear_kernel_hedgehog__moe_arch_mod__prompt_kernel(
        A_x, A_wqkv, A_w_phi, A_wo, B_x, B_w_r, B_w_gate, B_w_up, B_w_down, c, w_mod):
    del B_x
    hbm = pl.BlockSpec(memory_space=pl.ANY)
    out = pl.pallas_call(
        _kernel,
        out_shape=jax.ShapeDtypeStruct((S, D), BF),
        in_specs=[hbm] * 10,
        out_specs=hbm,
        scratch_shapes=[
            pltpu.VMEM((S, D), BF),
            pltpu.VMEM((D, 3 * D + PAD), BF),
            pltpu.VMEM((H * DH, DH), BF),
            pltpu.VMEM((D, D + PAD), BF),
            pltpu.VMEM((8, 128), BF),
            pltpu.VMEM((D, F + PAD), BF),
            pltpu.VMEM((D, F + PAD), BF),
            pltpu.VMEM((F, D + PAD), BF),
            pltpu.VMEM((1, D), BF),
            pltpu.VMEM((D, 6 * D + PAD), BF),
            pltpu.VMEM((7 * 512, KH), U32),
            pltpu.VMEM((7 * 256, KH), U32),
            pltpu.VMEM((7 * 256, KH), U32),
            pltpu.VMEM((NT * HROWS, KH), U32),
            pltpu.VMEM((NPAIR, 80, 128), F32),
            pltpu.VMEM((8, 6 * D + 2 * T), F32),
            pltpu.VMEM((4 * D, 128), F32),
            pltpu.VMEM((2 * NT * D, U), F32),
            pltpu.VMEM((2 * NT * 2 * 8, U), F32),
            pltpu.VMEM((S, D), BF),
            pltpu.VMEM((8 * 64, 128), U32),
            pltpu.VMEM((KH // 2, 8 * U), U32),
            pltpu.VMEM((KH // 2, 8 * U), U32),
            pltpu.VMEM((8, D), U32),
            pltpu.VMEM((T, D), F32),
            pltpu.VMEM((192, T), U32),
            pltpu.VMEM((256, T), F32),
            pltpu.VMEM((NPAIR, 128, U), F32),
            pltpu.SemaphoreType.DMA((10,)),
            pltpu.SemaphoreType.DMA((4,)),
            pltpu.SemaphoreType.DMA((4,)),
            pltpu.SemaphoreType.DMA((4,)),
            pltpu.SemaphoreType.DMA((NT,)),
            pltpu.SemaphoreType.DMA((NT,)),
            pltpu.SemaphoreType.DMA((2,)),
        ],
        compiler_params=pltpu.CompilerParams(
            vmem_limit_bytes=110 * 2**20,
            flags={"XLA_TPU_EVENLY_DISTRIBUTE_CRITICAL_NODES": True}),
        name="fused_block",
    )(A_x.reshape(S, D), A_wqkv, A_w_phi.reshape(H * DH, DH), A_wo, B_w_r.reshape(8, 128),
      B_w_gate, B_w_up, B_w_down, c, w_mod)
    return out.reshape(1, S, D)
```

```python
import math

import jax
import jax.numpy as jnp
from jax import lax
import jax.experimental.pallas as pl
import jax.experimental.pallas.tpu as pltpu

S, D, H, DH, F = 2048, 1024, 32, 32, 3584
U = 128
T = 2 * U
NT = S // T
KH = D // 2
NPAIR = H // 2
HROWS = 7 * U // 2
PAD = 128
F_VECTOR = 512
LN_ROWS = 32
LOG2E = math.log2(math.e)
BF, F32, U32, I32 = jnp.bfloat16, jnp.float32, jnp.uint32, jnp.int32

SHIFT_A, SCALE_A, GATE_A, SHIFT_B, SCALE_B, GATE_B, ROUTER_SUMS = range(7)
COL_GATE_A, COL_ROUTER, COL_GAIN, COL_BIAS, COL_VEC0, COL_VEC1 = range(6)

PLAN_FIRST = (
    "p p p p W s p", "p p N p p W s p p p",
    "p N p p W s p p p p", "p p X L N p p p p p",
    "p p p N p p p p", "p p p p N p p p",
    "p p p p p N p p", "p p N p p p p p")
PLAN_KV = (
    "p p N p p p p p", "p N p p p p p p",
    "p p N p p p p p", "p p p p p N p p",
    "p p p N p p p p", "p N p p p p p p",
    "p p p N p p p p", "p p p p p N p p")
PLAN_KV_LAST = (
    "p p p p o p p p N V", "p p p N p p p p o V",
    "p p p p p N p p o V", "p p p p N p p p V o",
    "B p p N p s p p p p", "s p N p p p p p p",
    "s p p p N p p p p", "s p p p N p p p p",
    "p p p p p p N p")
PLAN_Q_FIRST = (
    "q q q N c c q q q q", "q q N c c q q q q q",
    "q q q q q q N c c q", "q q q N c c q q q q")
PLAN_Q_SECOND = (
    "w w w w w w N c c w q q q q q q q", "w w w w N c c w w w q q q q q q q",
    "w w w w N c c w w w q q q q q q q", "w w w w w N c c w w q q q q q q q")
PLAN_Q = (
    "w w w w w w N c c w q q q q q q q E", "w w w N c c w w w w q q q q q q q E",
    "w w w w w N c c w w q q q q q q q E", "w w w w w N c c w w q q q q q q q E")
PLAN_Q_LATE = (
    "w N c c w w w w w w q q q q q q q E", "w w w w w N c c w w q q q q q q q E",
    "w w w w N c c w w w q q q q q q q E", "w w w w w w w q q q q q q N c c q E")
PLAN_Q_LAST = (
    "w w w w w w w q q q q N c c q q q E", "w w w w w w w q q q N c c q q q E q",
    "w w w w w w w q q N c c q q q q q E", "w w w w w w N c c w E")
PLAN_DRAIN = (
    "w w w w E w w w E", "w w w w w E w w",
    "w w w w w w w E", "w w w w w w w")
ORDER_FIRST = (6, 2, 1, 3, 4, 5, 7)
ORDER_KV = (1, 2, 3, 6, 4, 5, 7)
ORDER_Q = (4, 3, 2, 5, 1, 6, 7)
ORDER_OUT = (4, 7, 3, 1, 5, 2, 6)


def _dot(a, b):
    return jnp.dot(a, b, preferred_element_type=F32)


def _dot_nt(a, b):
    return lax.dot_general(a, b, (((1,), (1,)), ((), ())), preferred_element_type=F32)


def _pack(v):
    return pltpu.bitcast(v.astype(BF), U32)


def _unpack(v):
    return pltpu.bitcast(v, BF)


def _recip(v):
    return pl.reciprocal(v, approx=False, full_range=False)


def _rows(start, size):
    return pl.ds(start if isinstance(start, int) else pl.multiple_of(start, 8), size)


def _normalize(v):
    centered = v - jnp.mean(v, axis=-1, keepdims=True)
    var = jnp.mean(centered * centered, axis=-1, keepdims=True)
    return centered * lax.rsqrt(var + 1e-5)


def _fold8(v, op=jnp.add):
    parts = [v[i:i + 8] for i in range(0, v.shape[0], 8)]
    while len(parts) > 1:
        parts = [op(parts[i], parts[i + 1]) for i in range(0, len(parts), 2)]
    return parts[0]


def _per_head(v, op):
    r = _fold8(v, op)
    r = op(r, pltpu.roll(r, 4, 0))
    return op(r, pltpu.roll(r, 2, 0))


def _hedgehog(p):
    def spread(v):
        return jnp.concatenate([v] * 8, axis=0)

    pos = jnp.exp2(p - spread(_per_head(p, jnp.maximum)))
    neg = jnp.exp2(spread(_per_head(p, jnp.minimum)) - p)
    pos = pos * spread(_recip(_per_head(pos, jnp.add)))
    neg = neg * spread(_recip(_per_head(neg, jnp.add)))
    return jnp.concatenate([pos, neg], axis=0)


def _rotate(v, shift):
    return jnp.concatenate([pltpu.roll(v[:, i:i + 128], shift, 1) for i in range(0, v.shape[1], 128)], axis=1)


def _left_terms(a11, a12, a21, a22):
    return a11 + a22, a21 + a22, a11, a22, a11 + a12, a21 - a11, a12 - a22


def _right_terms(b11, b12, b21, b22):
    return b11 + b22, b11, b12 - b22, b21 - b11, b22, b11 + b12, b21 + b22


class _Strassen:
    _USES = {1: ((0, 1), (3, 1)), 2: ((2, 1), (3, -1)), 3: ((1, 1), (3, 1)), 4: ((0, 1), (2, 1)),
             5: ((0, -1), (1, 1)), 6: ((3, 1),), 7: ((0, 1),)}

    def __init__(self, product, order):
        self._product = product
        self._todo = list(order)
        self._c = [None] * 4

    @property
    def done(self):
        return not self._todo

    def step(self):
        i = self._todo.pop(0)
        m = self._product(i - 1)
        for k, sign in self._USES[i]:
            if self._c[k] is None:
                assert sign > 0
                self._c[k] = m
            else:
                self._c[k] = self._c[k] + m if sign > 0 else self._c[k] - m

    def result(self):
        assert self.done
        return jnp.concatenate(self._c[:2], axis=1), jnp.concatenate(self._c[2:], axis=1)


def _kernel(x_hbm, wqkv_hbm, wphi_hbm, wo_hbm, wr_hbm, wg_hbm, wu_hbm, wd_hbm, c_hbm, wmod_hbm,
            out_hbm,
            x_v, wqkv_v, wphi_v, wo_v, wr_v, wg_v, wu_v, wd_v, c_v, wmod_v,
            wkv_s, wq_s, wo_s, h_s, kv_s, mod_s, col_s, x1_s, stat_s, out_s, fmap_s,
            oa_s, ob_s, vec_s, xn_s, carry_s, raw_s, z_s,
            sem_w, sem_m, sem_k, sem_v, sem_x, sem_o, sem_p):
    def wcopy(i, src, dst):
        return pltpu.make_async_copy(src, dst, sem_w.at[i])

    cp_c = wcopy(0, c_hbm, c_v)
    cp_phi = wcopy(1, wphi_hbm, wphi_v)
    cp_wr = wcopy(2, wr_hbm, wr_v)
    cp_wq = wcopy(3, wqkv_hbm.at[:, 0:D], wqkv_v.at[:, 0:D])
    cp_mb = wcopy(4, wmod_hbm.at[:, 2 * D:4 * D], wmod_v.at[:, 2 * D:4 * D])
    cp_mc = wcopy(5, wmod_hbm.at[:, 4 * D:6 * D], wmod_v.at[:, 4 * D:6 * D])
    cp_wo = wcopy(6, wo_hbm, wo_v.at[:, 0:D])
    cp_wg = wcopy(7, wg_hbm, wg_v.at[:, 0:F])
    cp_wu = wcopy(8, wu_hbm, wu_v.at[:, 0:F])
    cp_wd = wcopy(9, wd_hbm, wd_v.at[:, 0:D])

    def mod_copy(j):
        col0 = (j % 2) * D + (j // 2) * KH
        cols = pl.ds(col0 if isinstance(j, int) else pl.multiple_of(col0, KH), KH)
        return pltpu.make_async_copy(wmod_hbm.at[:, cols], wmod_v.at[:, cols], sem_m.at[j])

    def kv_copies(o):
        ck, cv = pl.ds(D + o * 256, 256), pl.ds(2 * D + o * 256, 256)
        return (pltpu.make_async_copy(wqkv_hbm.at[:, ck], wqkv_v.at[:, ck], sem_k.at[o]),
                pltpu.make_async_copy(wqkv_hbm.at[:, cv], wqkv_v.at[:, cv], sem_v.at[o]))

    def x_copy(t):
        rows = _rows(t * T, T)
        return pltpu.make_async_copy(x_hbm.at[rows], x_v.at[rows], sem_x.at[t])

    def out_copy(t):
        rows = _rows(t * T, T)
        return pltpu.make_async_copy(out_s.at[rows], out_hbm.at[rows], sem_o.at[t])

    def start(*copies):
        for cp in copies:
            cp.start()

    def wait(*copies):
        for cp in copies:
            cp.wait()

    def fold(col0, g):
        return _dot_nt(_unpack(fmap_s[g * 64:(g + 1) * 64, :]),
                       wqkv_v[:, col0 + g * 128:col0 + (g + 1) * 128]) * LOG2E

    def stage_left(dst, o, upper, lower):
        n = upper.shape[0] // 2
        for i, a in enumerate(_left_terms(upper[:, :KH], upper[:, KH:], lower[:, :KH], lower[:, KH:])):
            dst[(i * 4 + o) * n:(i * 4 + o + 1) * n, :] = _pack(a)

    def stage_kv_weights(o):
        blocks = []
        for g in (2 * o, 2 * o + 1):
            fk = fold(D, g)
            fv = wqkv_v[:, 2 * D + g * 128:2 * D + (g + 1) * 128].T.astype(F32)
            blocks.append(jnp.concatenate([fk[:64], fv[:64], fk[64:], fv[64:]], axis=0))
        stage_left(wkv_s, o, *blocks)

    def stage_q_weights(o):
        stage_left(wq_s, o, fold(0, o), fold(0, o + 4))

    def stage_out_weights(o):
        stage_left(wo_s, o, wo_v[:, o * 128:(o + 1) * 128].T.astype(F32),
                   wo_v[:, KH + o * 128:KH + (o + 1) * 128].T.astype(F32))

    def param(k, n, width=D):
        return jnp.concatenate([mod_s[:, k * D:k * D + width]] * (n // 8), axis=0)

    def modulation(col0, n):
        mod_s[:, col0:col0 + n] = _dot(_unpack(vec_s[...]), wmod_v[:, col0:col0 + n])[0:8]

    def store_column(k, row):
        for g in range(8):
            col_s[k * D + g * 128:k * D + (g + 1) * 128, :] = jnp.broadcast_to(
                row[:, g * 128:(g + 1) * 128], (128, 128)).T

    def vector_product(w_ref, c0, tables, rows):
        accs = [None] * len(tables)
        for k0 in range(0, D, rows):
            w = w_ref[k0:k0 + rows, c0:c0 + 256].astype(F32)
            for k, table in enumerate(tables):
                v = col_s[table * D + k0:table * D + k0 + rows, :]
                part = _rotate(_fold8(w * jnp.concatenate([v, v], axis=1)), 1)
                accs[k] = part if accs[k] is None else accs[k] + part
        return [jnp.sum(_rotate(a, 127), axis=0, keepdims=True) for a in accs]

    def vector_modulation(k):
        for c0 in range(k * D, (k + 1) * D, 256):
            mod_s[:, c0:c0 + 256] = jnp.broadcast_to(vector_product(wmod_v, c0, (COL_VEC0,), 32)[0], (8, 256))

    def first_norm(t, dst, base, normalized=None):
        for r0 in range(0, U, LN_ROWS):
            h = []
            for half in range(2):
                rows = _rows(t * T + half * U + r0, LN_ROWS)
                xn = _normalize(x_v[rows, :].astype(F32)) if normalized is None else normalized[rows, :]
                h.append(xn * param(SCALE_A, LN_ROWS) + param(SHIFT_A, LN_ROWS))
            for i, b in enumerate(_right_terms(h[0][:, :KH], h[1][:, :KH], h[0][:, KH:], h[1][:, KH:])):
                dst[base + i * 64 + r0 // 2:base + i * 64 + (r0 + LN_ROWS) // 2, :] = _pack(b)

    def kv_products(src, base, o, order=ORDER_KV):
        return _Strassen(lambda i: _dot_nt(_unpack(wkv_s[(i * 4 + o) * 128:(i * 4 + o + 1) * 128, :]),
                                           _unpack(src[base + i * 64:base + (i + 1) * 64, :])), order)

    def kv_pairs(block):
        return [(block[j * 128 + 64:(j + 1) * 128].astype(BF), _hedgehog(block[j * 128:j * 128 + 64]).astype(BF))
                for j in range(2)]

    def kv_operands(r):
        return kv_pairs(r[0]) + kv_pairs(r[1])

    def save_kv_operands(r):
        raw_s[...] = r[0]
        for j, (v, phi) in enumerate(kv_pairs(r[1])):
            carry_s[j * 64:(j + 1) * 64, :] = pltpu.bitcast(phi, U32)
            carry_s[128 + j * 32:128 + (j + 1) * 32, :] = pltpu.bitcast(v, U32)

    def load_kv_operands():
        done = [(_unpack(carry_s[128 + j * 32:128 + (j + 1) * 32, :]), _unpack(carry_s[j * 64:(j + 1) * 64, :]))
                for j in range(2)]
        return kv_pairs(raw_s[...]) + done

    def accumulate_kv(ops, o, last=False):
        ones = jnp.ones((16, T), BF)
        for j, (v, phi) in enumerate(ops):
            acc = _dot_nt(jnp.concatenate([v, ones], axis=0), phi) + kv_s[4 * o + j]
            if last:
                z_s[4 * o + j] = jnp.concatenate([acc[64:72]] * 16, axis=0).T
                row_head = lax.broadcasted_iota(I32, (80, 128), 0) // DH
                lane_head = lax.broadcasted_iota(I32, (80, 128), 1) % 2
                acc = jnp.where(row_head == lane_head, acc, 0.0)
            kv_s[4 * o + j] = acc

    start(cp_phi, cp_c, *kv_copies(0), x_copy(0))
    lax.fori_loop(0, 4, lambda j, _: mod_copy(j).start(), None)
    cp_c.wait()
    cv = c_v[...].astype(F32)
    activated = cv * jax.nn.sigmoid(cv)
    vec_s[...] = _pack(jnp.broadcast_to(activated, (16, D)))
    store_column(COL_VEC0, activated)
    cp_phi.wait()
    repeat = ((lax.broadcasted_iota(I32, (128, DH), 0) % 64) // 2
              == lax.broadcasted_iota(I32, (128, DH), 1)).astype(BF)
    block_row = lax.broadcasted_iota(I32, (128, 128), 0)
    same_head = 2 * (block_row // 64) + block_row % 2 == lax.broadcasted_iota(I32, (128, 128), 1) // DH
    for g in range(8):
        full = _dot_nt(repeat, wphi_v[g * 128:(g + 1) * 128, :])
        fmap_s[g * 64:(g + 1) * 64, :] = _pack(jnp.where(same_head, full, 0.0))
    kv_s[...] = jnp.zeros(kv_s.shape, F32)
    wait(*kv_copies(0))
    stage_kv_weights(0)
    x_copy(0).wait()
    xn_s[...] = _normalize(x_v[0:T, :].astype(F32))
    for j in range(4):
        mod_copy(j).wait()
        if j == 2:
            start(*kv_copies(1), *kv_copies(2))
        elif j == 3:
            start(*kv_copies(3))
        col0 = (j % 2) * D + (j // 2) * KH
        modulation(col0, KH)
        if j % 2:
            mod_s[:, col0:col0 + KH] += 1.0
        if j == 1:
            left = [xn_s[k * U:(k + 1) * U, 0:KH] * param(SCALE_A, U, KH) + param(SHIFT_A, U, KH)
                    for k in range(2)]
            h_s[64:128, :] = _pack(left[0])
            h_s[320:384, :] = _pack(left[0] + left[1])
            first_products = kv_products(h_s, 0, 0, ORDER_FIRST)
            first_products.step()
            first_products.step()
    first_norm(0, h_s, 0, normalized=xn_s)

    ops = None
    for o, plan in enumerate(PLAN_FIRST):
        products = kv_products(h_s, (o // 4) * HROWS, o % 4) if o else first_products
        for item in plan.split():
            if item == "p":
                products.step()
            elif item == "W":
                wait(*kv_copies(o + 1))
                if o == 0:
                    x_copy(1).start()
                elif o == 1:
                    start(x_copy(2), x_copy(3))
            elif item == "X":
                wait(x_copy(1), x_copy(2))
                start(*(x_copy(t) for t in range(4, NT)), cp_wr, cp_wq, cp_wo)
                x_copy(3).wait()
            elif item == "s":
                stage_kv_weights(o + 1)
            elif item == "L":
                for t in range(1, 4):
                    first_norm(t, h_s, t * HROWS)
            else:
                accumulate_kv(ops, (o - 1) % 4)
        if o + 1 < len(PLAN_FIRST):
            ops = kv_operands(products.result())
    save_kv_operands(products.result())

    def kv_steps(ops, steps, plans, last_from):
        staged_q = staged_out = modulated = 0
        for o, (products, plan) in enumerate(zip(steps, plans)):
            for item in plan.split():
                if item == "p":
                    products.step()
                elif item == "s":
                    stage_q_weights(staged_q)
                    staged_q += 1
                elif item == "o":
                    stage_out_weights(staged_out)
                    staged_out += 1
                elif item == "V":
                    vector_modulation(GATE_A + modulated)
                    modulated += 1
                elif item == "B":
                    cp_wr.wait()
                else:
                    accumulate_kv(ops, (o - 1) % 4, last=o >= last_from)
            if o + 1 < len(plans):
                ops = kv_operands(products.result())
        return products.result()

    def pass1(i, remaining):
        t = 2 * i + 2
        pl.when(i == 0)(cp_mb.start)
        pl.when(i == 1)(cp_mc.start)
        wait(x_copy(t + 2), x_copy(t + 3))
        view = h_s.at[_rows(t * HROWS, 4 * HROWS)]
        first_norm(t + 2, view, 2 * HROWS)
        first_norm(t + 3, view, 3 * HROWS)
        steps = [kv_products(view, k * HROWS, o) for k in range(2) for o in range(4)]
        save_kv_operands(kv_steps(load_kv_operands(), steps, PLAN_KV, last_from=len(steps)))
        return remaining - 1

    first_tile = lax.fori_loop(0, 2, pass1, 2)

    def q_products(t, o):
        return _Strassen(lambda i: _dot_nt(_unpack(wq_s[(i * 4 + o) * 64:(i * 4 + o + 1) * 64, :]),
                                           _unpack(h_s[_rows(t * HROWS + i * 64, 64), :])), ORDER_Q)

    def derived_params():
        wr8 = wr_v[...].astype(F32)
        wr = jnp.broadcast_to(jnp.concatenate([wr8[j:j + 1, :] for j in range(8)], axis=1), (8, D))
        scale = 1.0 + param(SCALE_B, 8)
        mod_s[:, SCALE_B * D:(SCALE_B + 1) * D] = scale
        router = scale * wr
        tables = (param(GATE_A, 8), router, scale * param(GATE_B, 8), param(SHIFT_B, 8) * param(GATE_B, 8))
        for k, row in enumerate(tables):
            store_column(k, row[0:1])
        base = ROUTER_SUMS * D
        mod_s[:, base:base + T] = jnp.broadcast_to(jnp.sum(router, axis=-1, keepdims=True), (8, T))
        mod_s[:, base + T:base + 2 * T] = jnp.broadcast_to(
            jnp.sum(param(SHIFT_B, 8) * wr, axis=-1, keepdims=True), (8, T))

    def column(k, ch):
        v = col_s[k * D + ch:k * D + ch + 128, :]
        return jnp.concatenate([v, v], axis=1)

    def feature_pairs(block, p0):
        out = []
        for j in range(2):
            phi = _hedgehog(block[j * 64:(j + 1) * 64])
            z = z_s[p0 + j]
            inv = _recip(_per_head(phi * jnp.concatenate([z, z], axis=1), jnp.add) + 1e-6)
            out.append((phi.astype(BF), inv))
        return out

    def features(r, o):
        return feature_pairs(r[0], 2 * o) + feature_pairs(r[1], 2 * o + 8)

    def save_features(r):
        raw_s[0:128, :] = r[0]
        for j, (phi, inv) in enumerate(feature_pairs(r[1], 8)):
            carry_s[j * 64:(j + 1) * 64, :] = pltpu.bitcast(phi, U32)
            raw_s[128 + 8 * j:136 + 8 * j, :] = inv

    def load_features():
        done = [(_unpack(carry_s[j * 64:(j + 1) * 64, :]), raw_s[128 + 8 * j:136 + 8 * j, :]) for j in range(2)]
        return feature_pairs(raw_s[0:128, :], 0) + done

    def attend(phis, o):
        heads = {}
        for j in (0, 2, 1, 3):
            phi, inv = phis[j]
            num = _dot(kv_s[2 * o + 8 * (j // 2) + j % 2, 0:64, :].astype(BF), phi)
            heads[j] = jnp.concatenate([num[k * DH:(k + 1) * DH] * inv[k:k + 1] for k in range(2)], axis=0)
        return heads

    def stage_heads(dst, o, j, lo, hi):
        base = o * 64 + j * 32
        terms = _right_terms(lo[:, :U], lo[:, U:], hi[:, :U], hi[:, U:])
        dst[base:base + 32, 0:6 * U] = _pack(jnp.concatenate(terms[:6], axis=1))
        dst[base:base + 16, 6 * U:8 * U] = _pack(jnp.concatenate([terms[6][:32], terms[6][32:]], axis=1))

    def out_products(src, o):
        def product(i):
            if i < 6:
                b = src[:, i * U:(i + 1) * U]
            else:
                b = jnp.concatenate([src[k * 32:k * 32 + 16, (6 + c) * U:(7 + c) * U]
                                     for k in range(8) for c in range(2)], axis=0)
            return _dot(_unpack(wo_s[(i * 4 + o) * 64:(i * 4 + o + 1) * 64, :]), _unpack(b))
        return _Strassen(product, ORDER_OUT)

    def residual(t, o, attn, sums):
        ys = []
        for half, a in enumerate(attn):
            ch = half * KH + o * 128
            ys.append(x_v[_rows(t * T, T), ch:ch + 128].T.astype(F32) + column(COL_GATE_A, ch) * a)
        if sums is None:
            shift = jnp.sum(_fold8(ys[0]) + _fold8(ys[1]), axis=0, keepdims=True) * (1.0 / 256)
            sums = (shift, 0.0, 0.0, 0.0)
        shift, s1, s2, s3 = sums
        for half, y in enumerate(ys):
            ch = half * KH + o * 128
            d = y - shift
            for k in range(2):
                x1_s[_rows((2 * t + k) * D + ch, 128), :] = y[:, k * U:(k + 1) * U]
            s1, s2, s3 = s1 + _fold8(d), s2 + _fold8(d * d), s3 + _fold8(d * column(COL_ROUTER, ch))
        return shift, s1, s2, s3

    def route(t, sums, top):
        m1, i1, m2, i2 = top
        shift = sums[0]
        s1, s2, s3 = (jnp.sum(s, axis=0, keepdims=True) for s in sums[1:])
        delta = s1 * (1.0 / D)
        rstd = lax.rsqrt(jnp.maximum(s2 * (1.0 / D) - delta * delta, 0.0) + 1e-5)
        score = (s3 - delta * mod_s[0:1, ROUTER_SUMS * D:ROUTER_SUMS * D + T]) * rstd
        for k, v in enumerate((shift + delta, rstd)):
            for half in range(2):
                stat_s[_rows(((2 * t + half) * 2 + k) * 8, 8), :] = jnp.broadcast_to(
                    v[:, half * U:(half + 1) * U], (8, U))
        idx = lax.broadcasted_iota(I32, (1, T), 1) + t * T
        g1, g2 = score > m1, score > m2
        return (jnp.where(g1, score, m1), jnp.where(g1, idx, i1),
                jnp.where(g1, m1, jnp.where(g2, score, m2)), jnp.where(g1, i1, jnp.where(g2, idx, i2)))

    def stat(block, k, n):
        return jnp.concatenate([stat_s[_rows((block * 2 + k) * 8, 8), :]] * (n // 8), axis=0)

    def emit(t, ch):
        n = 256
        for half in range(2):
            mean, rstd = (stat(2 * t + half, k, n) for k in range(2))
            x1 = x1_s[_rows((2 * t + half) * D + ch, n), :]
            gain = rstd * col_s[COL_GAIN * D + ch:COL_GAIN * D + ch + n, :]
            res = (x1 + col_s[COL_BIAS * D + ch:COL_BIAS * D + ch + n, :]) + (x1 - mean) * gain
            out_s[_rows(t * T + half * U, U), ch:ch + n] = res.T.astype(BF)

    def q_tile(t, phis, top, plans, current, previous, more=True):
        sums, emitted = None, 0
        for o, plan in enumerate(plans):
            qs = None
            if phis is not None and (o < 3 or more):
                qs = q_products(t, o + 1) if o < 3 else q_products(t + 1, 0)
            ws = out_products(previous, o)
            heads, staged = None, 0
            for item in plan.split():
                if item == "q":
                    qs.step()
                elif item == "w":
                    ws.step()
                    if ws.done:
                        sums = residual(t - 1, o, ws.result(), sums)
                elif item == "N":
                    heads = attend(phis, o)
                elif item == "c":
                    stage_heads(current, o, staged, heads[staged], heads[staged + 2])
                    staged += 1
                elif item == "E":
                    emit(t - 2, emitted * 256)
                    emitted += 1
            if qs is not None:
                phis = features(qs.result(), o + 1) if o < 3 else qs.result()
        if sums is not None:
            top = route(t - 1, sums, top)
        if emitted:
            out_copy(t - 2).start()
        return phis, top

    wait(cp_wq, cp_wo, cp_mb, cp_mc)
    start(cp_wg, cp_wu)
    steps = [kv_products(h_s, t * HROWS, o) for t in (NT - 2, NT - 1) for o in range(4)]
    r = kv_steps(load_kv_operands(), steps + [q_products(first_tile, 0)], PLAN_KV_LAST, last_from=5)
    lowest = jnp.full((1, T), -jnp.inf, F32)
    zero = jnp.zeros((1, T), I32)
    top = (lowest, zero, lowest, zero)
    r, top = q_tile(first_tile, features(r, 0), top, PLAN_Q_FIRST, oa_s, ob_s)
    derived_params()
    r, top = q_tile(first_tile + 1, features(r, 0), top, PLAN_Q_SECOND, ob_s, oa_s)
    save_features(r)

    def pass2(i, carry):
        top, tile = carry
        pl.when(i == 2)(cp_wd.start)
        r, top = q_tile(2 * i - 2, load_features(), top, PLAN_Q, oa_s, ob_s)
        r, top = q_tile(2 * i - 1, features(r, 0), top, PLAN_Q, ob_s, oa_s)
        save_features(r)
        return top, tile + 2

    top, tile = lax.fori_loop(2, 4, pass2, (top, 2))
    wait(cp_wg, cp_wu, cp_wd)
    r, top = q_tile(tile, load_features(), top, PLAN_Q_LATE, oa_s, ob_s)
    _, top = q_tile(tile + 1, features(r, 0), top, PLAN_Q_LAST, ob_s, oa_s, more=False)
    _, top = q_tile(tile + 2, None, top, PLAN_DRAIN, oa_s, ob_s)

    m1, i1, m2, i2 = top
    best = jnp.max(m1, axis=1, keepdims=True)
    ia = jnp.min(jnp.where(m1 == best, i1, S - 1), axis=1, keepdims=True)
    taken = i1 == ia
    rest, rest_idx = jnp.where(taken, m2, m1), jnp.where(taken, i2, i1)
    second = jnp.max(rest, axis=1, keepdims=True)
    ib = jnp.min(jnp.where(rest == second, rest_idx, S - 1), axis=1, keepdims=True)
    idx = (jnp.clip(ia[0, 0], 0, S - 1), jnp.clip(ib[0, 0], 0, S - 1))

    for g in range(4):
        emit(NT - 1, g * 256)
    out_copy(NT - 1).start()
    out_copy(0).wait()

    row16 = lax.broadcasted_iota(I32, (16, U), 0)
    lane16 = lax.broadcasted_iota(I32, (16, U), 1)
    xn_sel = 0.0
    for k in range(2):
        block = idx[k] // U
        xn = (x1_s[_rows(block * D, D), :] - stat(block, 0, D)) * stat(block, 1, D)
        pick = jnp.where((row16 == k) & (lane16 == idx[k] % U), 1.0, 0.0).astype(BF)
        xn_sel = xn_sel + _dot_nt(pick, xn.astype(BF))
    hs = (xn_sel * param(SCALE_B, 16) + param(SHIFT_B, 16)).astype(BF)
    score = jnp.where(row16[:, 0:1] == 0, best, second) + mod_s[0:1, ROUTER_SUMS * D + T:ROUTER_SUMS * D + T + 1]
    gate = jax.nn.sigmoid(score)

    for k in range(2):
        store_column(COL_VEC0 + k, hs.astype(F32)[k:k + 1])

    def down(g, u, c0, c1):
        return _dot((g * jax.nn.sigmoid(g) * u).astype(BF), wd_v[c0:c1, 0:D])

    fm = F - F_VECTOR
    y = jnp.zeros((16, D), F32)
    for c0, c1 in ((0, fm // 2), (fm // 2, fm)):
        y = y + down(_dot(hs, wg_v[:, c0:c1]), _dot(hs, wu_v[:, c0:c1]), c0, c1)
    first_row = lax.broadcasted_iota(I32, (16, 256), 0) == 0
    for c0 in range(fm, F, 256):
        g, u = (jnp.where(first_row, *vector_product(w, c0, (COL_VEC0, COL_VEC1), 16)) for w in (wg_v, wu_v))
        y = y + down(g, u, c0, c0 + 256)
    update = param(GATE_B, 16) * (y * gate)

    wait(*(out_copy(t) for t in range(1, NT)))
    row = lax.broadcasted_iota(I32, (16, D), 0)

    def patch(k):
        base = pl.multiple_of((idx[k] // 16) * 16, 16)
        block = out_s[pl.ds(base, 16), :].astype(F32)
        out_s[pl.ds(base, 16), :] = jnp.where(row == idx[k] - base, block + update[k:k + 1, :], block).astype(BF)
        return pltpu.make_async_copy(out_s.at[pl.ds(base, 16)], out_hbm.at[pl.ds(base, 16)], sem_p.at[k])

    patch_a, patch_b = patch(0), patch(1)
    patch_a.start()

    @pl.when(idx[0] // 16 != idx[1] // 16)
    def _():
        patch_b.start()
        patch_b.wait()

    patch_a.wait()


@jax.jit
def pallas_adaLN_cond__linear_kernel_hedgehog__moe_arch_mod__prompt_kernel(
        A_x, A_wqkv, A_w_phi, A_wo, B_x, B_w_r, B_w_gate, B_w_up, B_w_down, c, w_mod):
    del B_x
    hbm = pl.BlockSpec(memory_space=pl.ANY)
    out = pl.pallas_call(
        _kernel,
        out_shape=jax.ShapeDtypeStruct((S, D), BF),
        in_specs=[hbm] * 10,
        out_specs=hbm,
        scratch_shapes=[
            pltpu.VMEM((S, D), BF),
            pltpu.VMEM((D, 3 * D + PAD), BF),
            pltpu.VMEM((H * DH, DH), BF),
            pltpu.VMEM((D, D + PAD), BF),
            pltpu.VMEM((8, 128), BF),
            pltpu.VMEM((D, F + PAD), BF),
            pltpu.VMEM((D, F + PAD), BF),
            pltpu.VMEM((F, D + PAD), BF),
            pltpu.VMEM((1, D), BF),
            pltpu.VMEM((D, 6 * D + PAD), BF),
            pltpu.VMEM((7 * 512, KH), U32),
            pltpu.VMEM((7 * 256, KH), U32),
            pltpu.VMEM((7 * 256, KH), U32),
            pltpu.VMEM((NT * HROWS, KH), U32),
            pltpu.VMEM((NPAIR, 80, 128), F32),
            pltpu.VMEM((8, 6 * D + 2 * T), F32),
            pltpu.VMEM((6 * D, 128), F32),
            pltpu.VMEM((2 * NT * D, U), F32),
            pltpu.VMEM((2 * NT * 2 * 8, U), F32),
            pltpu.VMEM((S, D), BF),
            pltpu.VMEM((8 * 64, 128), U32),
            pltpu.VMEM((KH // 2, 8 * U), U32),
            pltpu.VMEM((KH // 2, 8 * U), U32),
            pltpu.VMEM((8, D), U32),
            pltpu.VMEM((T, D), F32),
            pltpu.VMEM((192, T), U32),
            pltpu.VMEM((256, T), F32),
            pltpu.VMEM((NPAIR, 128, U), F32),
            pltpu.SemaphoreType.DMA((10,)),
            pltpu.SemaphoreType.DMA((4,)),
            pltpu.SemaphoreType.DMA((4,)),
            pltpu.SemaphoreType.DMA((4,)),
            pltpu.SemaphoreType.DMA((NT,)),
            pltpu.SemaphoreType.DMA((NT,)),
            pltpu.SemaphoreType.DMA((2,)),
        ],
        compiler_params=pltpu.CompilerParams(
            vmem_limit_bytes=110 * 2**20,
            flags={"XLA_TPU_EVENLY_DISTRIBUTE_CRITICAL_NODES": True}),
        name="fused_block",
    )(A_x.reshape(S, D), A_wqkv, A_w_phi.reshape(H * DH, DH), A_wo, B_w_r.reshape(8, 128),
      B_w_gate, B_w_up, B_w_down, c, w_mod)
    return out.reshape(1, S, D)
```

```python
import math

import jax
import jax.numpy as jnp
from jax import lax
import jax.experimental.pallas as pl
import jax.experimental.pallas.tpu as pltpu

S, D, H, DH, F = 2048, 1024, 32, 32, 3584
U = 128
T = 2 * U
NT = S // T
KH = D // 2
NPAIR = H // 2
HROWS = 7 * U // 2
PAD = 128
F_VECTOR = 512
LN_ROWS = 32
LOG2E = math.log2(math.e)
BF, F32, U32, I32 = jnp.bfloat16, jnp.float32, jnp.uint32, jnp.int32

SHIFT_A, SCALE_A, GATE_A, SHIFT_B, SCALE_B, GATE_B, ROUTER_SUMS = range(7)
COL_GATE_A, COL_ROUTER, COL_GAIN, COL_BIAS, COL_VEC0, COL_VEC1 = range(6)

PLAN_FIRST = (
    "p p p p W s p", "p p N p p W s p p p",
    "p N p p W s p p p p", "p p X L N p p p p p",
    "p p p N p p p p", "p p p p p N p p",
    "p p p p p N p p", "p p N p p p p p")
PLAN_KV = (
    "p p N p p p p p", "p N p p p p p p",
    "p p N p p p p p", "p p p p p N p p",
    "p p p p N p p p", "p N p p p p p p",
    "p p N p p p p p", "p p N p p p p p")
PLAN_KV_LAST = (
    "p p p p o p p p N V", "p p p p p p p N o V",
    "p p p p p p p o V N", "p p p p p p N p V o",
    "B p p N p s p p p p", "s N p p p p p p p",
    "s p p p N p p p p", "s p p p N p p p p",
    "p p p p p N p p")
PLAN_Q_FIRST = (
    "q q q q N c c q q q", "q q N c c q q q q q",
    "q q q q q q N c c q", "q q q N c c q q q q")
PLAN_Q_SECOND = (
    "w w w w w w N c c w q q q q q q q", "w w w w N c c w w w q q q q q q q",
    "w w w w N c c w w w q q q q q q q", "w w w w w w w q N c c q q q q q q")
PLAN_Q = (
    "w w w w w w N c c w q q q q q q q E", "w w w N c c w w w w q q q q q q q E",
    "w w w w w N c c w w q q q q q q q E", "w w w w w N c c w w q q q q q q q E")
PLAN_Q_LATE = (
    "w N c c w w w w w w q q q q q q q E", "w w w w w N c c w w q q q q q q q E",
    "w w w w N c c w w w q q q q q q q E", "w w w w w w w q q q q q q N c c q E")
PLAN_Q_LAST = (
    "w w w w w w w q q q q N c c q q q E", "w w w w w w w q q q N c c q q q E q",
    "w w w w w w w q q N c c q q q q q E", "w w w w w w N c c w E")
PLAN_DRAIN = (
    "w w w w E w w w E", "w w w w w E w w",
    "w w w w w w w E", "w w w w w w w")
ORDER_FIRST = (6, 2, 1, 3, 4, 5, 7)
ORDER_KV = (1, 2, 3, 6, 4, 5, 7)
ORDER_Q = (4, 3, 2, 5, 1, 6, 7)
ORDER_OUT = (4, 7, 3, 1, 5, 2, 6)


def _dot(a, b):
    return jnp.dot(a, b, preferred_element_type=F32)


def _dot_nt(a, b):
    return lax.dot_general(a, b, (((1,), (1,)), ((), ())), preferred_element_type=F32)


def _pack(v):
    return pltpu.bitcast(v.astype(BF), U32)


def _unpack(v):
    return pltpu.bitcast(v, BF)


def _recip(v):
    return pl.reciprocal(v, approx=False, full_range=False)


def _rows(start, size):
    return pl.ds(start if isinstance(start, int) else pl.multiple_of(start, 8), size)


def _normalize(v):
    centered = v - jnp.mean(v, axis=-1, keepdims=True)
    var = jnp.mean(centered * centered, axis=-1, keepdims=True)
    return centered * lax.rsqrt(var + 1e-5)


def _fold8(v, op=jnp.add):
    parts = [v[i:i + 8] for i in range(0, v.shape[0], 8)]
    while len(parts) > 1:
        parts = [op(parts[i], parts[i + 1]) for i in range(0, len(parts), 2)]
    return parts[0]


def _per_head(v, op):
    r = _fold8(v, op)
    r = op(r, pltpu.roll(r, 4, 0))
    return op(r, pltpu.roll(r, 2, 0))


def _hedgehog(p):
    def spread(v):
        return jnp.concatenate([v] * 8, axis=0)

    pos = jnp.exp2(p - spread(_per_head(p, jnp.maximum)))
    neg = jnp.exp2(spread(_per_head(p, jnp.minimum)) - p)
    pos = pos * spread(_recip(_per_head(pos, jnp.add)))
    neg = neg * spread(_recip(_per_head(neg, jnp.add)))
    return jnp.concatenate([pos, neg], axis=0)


def _rotate(v, shift):
    return jnp.concatenate([pltpu.roll(v[:, i:i + 128], shift, 1) for i in range(0, v.shape[1], 128)], axis=1)


def _left_terms(a11, a12, a21, a22):
    return a11 + a22, a21 + a22, a11, a22, a11 + a12, a21 - a11, a12 - a22


def _right_terms(b11, b12, b21, b22):
    return b11 + b22, b11, b12 - b22, b21 - b11, b22, b11 + b12, b21 + b22


class _Strassen:
    _USES = {1: ((0, 1), (3, 1)), 2: ((2, 1), (3, -1)), 3: ((1, 1), (3, 1)), 4: ((0, 1), (2, 1)),
             5: ((0, -1), (1, 1)), 6: ((3, 1),), 7: ((0, 1),)}

    def __init__(self, product, order):
        self._product = product
        self._todo = list(order)
        self._c = [None] * 4

    @property
    def done(self):
        return not self._todo

    def step(self):
        i = self._todo.pop(0)
        m = self._product(i - 1)
        for k, sign in self._USES[i]:
            if self._c[k] is None:
                assert sign > 0
                self._c[k] = m
            else:
                self._c[k] = self._c[k] + m if sign > 0 else self._c[k] - m

    def result(self):
        assert self.done
        return jnp.concatenate(self._c[:2], axis=1), jnp.concatenate(self._c[2:], axis=1)


def _kernel(x_hbm, wqkv_hbm, wphi_hbm, wo_hbm, wr_hbm, wg_hbm, wu_hbm, wd_hbm, c_hbm, wmod_hbm,
            out_hbm,
            x_v, wqkv_v, wphi_v, wo_v, wr_v, wg_v, wu_v, wd_v, c_v, wmod_v,
            wkv_s, wq_s, wo_s, h_s, kv_s, mod_s, col_s, x1_s, stat_s, out_s, fmap_s,
            oa_s, ob_s, vec_s, xn_s, carry_s, raw_s, z_s,
            sem_w, sem_m, sem_k, sem_v, sem_x, sem_o, sem_p):
    def wcopy(i, src, dst):
        return pltpu.make_async_copy(src, dst, sem_w.at[i])

    cp_c = wcopy(0, c_hbm, c_v)
    cp_phi = wcopy(1, wphi_hbm, wphi_v)
    cp_wr = wcopy(2, wr_hbm, wr_v)
    cp_wq = wcopy(3, wqkv_hbm.at[:, 0:D], wqkv_v.at[:, 0:D])
    cp_mb = wcopy(4, wmod_hbm.at[:, 2 * D:4 * D], wmod_v.at[:, 2 * D:4 * D])
    cp_mc = wcopy(5, wmod_hbm.at[:, 4 * D:6 * D], wmod_v.at[:, 4 * D:6 * D])
    cp_wo = wcopy(6, wo_hbm, wo_v.at[:, 0:D])
    cp_wg = wcopy(7, wg_hbm, wg_v.at[:, 0:F])
    cp_wu = wcopy(8, wu_hbm, wu_v.at[:, 0:F])
    cp_wd = wcopy(9, wd_hbm, wd_v.at[:, 0:D])

    def mod_copy(j):
        col0 = (j % 2) * D + (j // 2) * KH
        cols = pl.ds(col0 if isinstance(j, int) else pl.multiple_of(col0, KH), KH)
        return pltpu.make_async_copy(wmod_hbm.at[:, cols], wmod_v.at[:, cols], sem_m.at[j])

    def kv_copies(o):
        ck, cv = pl.ds(D + o * 256, 256), pl.ds(2 * D + o * 256, 256)
        return (pltpu.make_async_copy(wqkv_hbm.at[:, ck], wqkv_v.at[:, ck], sem_k.at[o]),
                pltpu.make_async_copy(wqkv_hbm.at[:, cv], wqkv_v.at[:, cv], sem_v.at[o]))

    def x_copy(t):
        rows = _rows(t * T, T)
        return pltpu.make_async_copy(x_hbm.at[rows], x_v.at[rows], sem_x.at[t])

    def out_copy(t):
        rows = _rows(t * T, T)
        return pltpu.make_async_copy(out_s.at[rows], out_hbm.at[rows], sem_o.at[t])

    def start(*copies):
        for cp in copies:
            cp.start()

    def wait(*copies):
        for cp in copies:
            cp.wait()

    def fold(col0, g):
        return _dot_nt(_unpack(fmap_s[g * 64:(g + 1) * 64, :]),
                       wqkv_v[:, col0 + g * 128:col0 + (g + 1) * 128]) * LOG2E

    def stage_left(dst, o, upper, lower):
        n = upper.shape[0] // 2
        for i, a in enumerate(_left_terms(upper[:, :KH], upper[:, KH:], lower[:, :KH], lower[:, KH:])):
            dst[(i * 4 + o) * n:(i * 4 + o + 1) * n, :] = _pack(a)

    def stage_kv_weights(o):
        blocks = []
        for g in (2 * o, 2 * o + 1):
            fk = fold(D, g)
            fv = wqkv_v[:, 2 * D + g * 128:2 * D + (g + 1) * 128].T.astype(F32)
            blocks.append(jnp.concatenate([fk[:64], fv[:64], fk[64:], fv[64:]], axis=0))
        stage_left(wkv_s, o, *blocks)

    def stage_q_weights(o):
        stage_left(wq_s, o, fold(0, o), fold(0, o + 4))

    def stage_out_weights(o):
        stage_left(wo_s, o, wo_v[:, o * 128:(o + 1) * 128].T.astype(F32),
                   wo_v[:, KH + o * 128:KH + (o + 1) * 128].T.astype(F32))

    def param(k, n, width=D):
        return jnp.concatenate([mod_s[:, k * D:k * D + width]] * (n // 8), axis=0)

    def modulation(col0, n):
        mod_s[:, col0:col0 + n] = _dot(_unpack(vec_s[...]), wmod_v[:, col0:col0 + n])[0:8]

    def store_column(k, row):
        for g in range(8):
            col_s[k * D + g * 128:k * D + (g + 1) * 128, :] = jnp.broadcast_to(
                row[:, g * 128:(g + 1) * 128], (128, 128)).T

    def vector_product(w_ref, c0, tables, rows):
        accs = [None] * len(tables)
        for k0 in range(0, D, rows):
            w = w_ref[k0:k0 + rows, c0:c0 + 256].astype(F32)
            for k, table in enumerate(tables):
                v = col_s[table * D + k0:table * D + k0 + rows, :]
                part = _rotate(_fold8(w * jnp.concatenate([v, v], axis=1)), 1)
                accs[k] = part if accs[k] is None else accs[k] + part
        return [jnp.sum(_rotate(a, 127), axis=0, keepdims=True) for a in accs]

    def vector_modulation(k):
        for c0 in range(k * D, (k + 1) * D, 256):
            mod_s[:, c0:c0 + 256] = jnp.broadcast_to(vector_product(wmod_v, c0, (COL_VEC0,), 32)[0], (8, 256))

    def first_norm(t, dst, base, normalized=None):
        for r0 in range(0, U, LN_ROWS):
            h = []
            for half in range(2):
                rows = _rows(t * T + half * U + r0, LN_ROWS)
                xn = _normalize(x_v[rows, :].astype(F32)) if normalized is None else normalized[rows, :]
                h.append(xn * param(SCALE_A, LN_ROWS) + param(SHIFT_A, LN_ROWS))
            for i, b in enumerate(_right_terms(h[0][:, :KH], h[1][:, :KH], h[0][:, KH:], h[1][:, KH:])):
                dst[base + i * 64 + r0 // 2:base + i * 64 + (r0 + LN_ROWS) // 2, :] = _pack(b)

    def kv_products(src, base, o, order=ORDER_KV):
        return _Strassen(lambda i: _dot_nt(_unpack(wkv_s[(i * 4 + o) * 128:(i * 4 + o + 1) * 128, :]),
                                           _unpack(src[base + i * 64:base + (i + 1) * 64, :])), order)

    def kv_pairs(block, p0, last=False):
        ops = []
        for j in range(2):
            phi = _hedgehog(block[j * 128:j * 128 + 64])
            z = (phi[:, :U] + phi[:, U:]) + z_s[p0 + j]
            z_s[p0 + j] = jnp.broadcast_to(jnp.sum(z, axis=1, keepdims=True), (128, U)) if last else z
            ops.append((block[j * 128 + 64:(j + 1) * 128].astype(BF), phi.astype(BF)))
        return ops

    def kv_operands(r, o, last=False):
        return kv_pairs(r[0], 4 * o, last) + kv_pairs(r[1], 4 * o + 2, last)

    def save_kv_operands(r):
        raw_s[...] = r[0]
        for j, (v, phi) in enumerate(kv_pairs(r[1], NPAIR - 2)):
            carry_s[j * 64:(j + 1) * 64, :] = pltpu.bitcast(phi, U32)
            carry_s[128 + j * 32:128 + (j + 1) * 32, :] = pltpu.bitcast(v, U32)

    def load_kv_operands():
        done = [(_unpack(carry_s[128 + j * 32:128 + (j + 1) * 32, :]), _unpack(carry_s[j * 64:(j + 1) * 64, :]))
                for j in range(2)]
        return kv_pairs(raw_s[...], NPAIR - 4) + done

    def accumulate_kv(ops, o, last=False):
        for j, (v, phi) in enumerate(ops):
            acc = _dot_nt(v, phi) + kv_s[4 * o + j]
            if last:
                row_head = lax.broadcasted_iota(I32, (64, 128), 0) // DH
                lane_head = lax.broadcasted_iota(I32, (64, 128), 1) % 2
                acc = jnp.where(row_head == lane_head, acc, 0.0)
            kv_s[4 * o + j] = acc

    start(cp_phi, cp_c, *kv_copies(0), x_copy(0))
    lax.fori_loop(0, 4, lambda j, _: mod_copy(j).start(), None)
    cp_c.wait()
    cv = c_v[...].astype(F32)
    activated = cv * jax.nn.sigmoid(cv)
    vec_s[...] = _pack(jnp.broadcast_to(activated, (16, D)))
    store_column(COL_VEC0, activated)
    cp_phi.wait()
    repeat = ((lax.broadcasted_iota(I32, (128, DH), 0) % 64) // 2
              == lax.broadcasted_iota(I32, (128, DH), 1)).astype(BF)
    block_row = lax.broadcasted_iota(I32, (128, 128), 0)
    same_head = 2 * (block_row // 64) + block_row % 2 == lax.broadcasted_iota(I32, (128, 128), 1) // DH
    for g in range(8):
        full = _dot_nt(repeat, wphi_v[g * 128:(g + 1) * 128, :])
        fmap_s[g * 64:(g + 1) * 64, :] = _pack(jnp.where(same_head, full, 0.0))
    kv_s[...] = jnp.zeros(kv_s.shape, F32)
    z_s[...] = jnp.zeros(z_s.shape, F32)
    wait(*kv_copies(0))
    stage_kv_weights(0)
    x_copy(0).wait()
    xn_s[...] = _normalize(x_v[0:T, :].astype(F32))
    for j in range(4):
        mod_copy(j).wait()
        if j == 2:
            start(*kv_copies(1), *kv_copies(2))
        elif j == 3:
            start(*kv_copies(3))
        col0 = (j % 2) * D + (j // 2) * KH
        modulation(col0, KH)
        if j % 2:
            mod_s[:, col0:col0 + KH] += 1.0
        if j == 1:
            left = [xn_s[k * U:(k + 1) * U, 0:KH] * param(SCALE_A, U, KH) + param(SHIFT_A, U, KH)
                    for k in range(2)]
            h_s[64:128, :] = _pack(left[0])
            h_s[320:384, :] = _pack(left[0] + left[1])
            first_products = kv_products(h_s, 0, 0, ORDER_FIRST)
            first_products.step()
            first_products.step()
    first_norm(0, h_s, 0, normalized=xn_s)

    ops = None
    for o, plan in enumerate(PLAN_FIRST):
        products = kv_products(h_s, (o // 4) * HROWS, o % 4) if o else first_products
        for item in plan.split():
            if item == "p":
                products.step()
            elif item == "W":
                wait(*kv_copies(o + 1))
                if o == 0:
                    x_copy(1).start()
                elif o == 1:
                    start(x_copy(2), x_copy(3))
            elif item == "X":
                wait(x_copy(1), x_copy(2))
                start(*(x_copy(t) for t in range(4, NT)), cp_wr, cp_wq, cp_wo)
                x_copy(3).wait()
            elif item == "s":
                stage_kv_weights(o + 1)
            elif item == "L":
                for t in range(1, 4):
                    first_norm(t, h_s, t * HROWS)
            else:
                accumulate_kv(ops, (o - 1) % 4)
        if o + 1 < len(PLAN_FIRST):
            ops = kv_operands(products.result(), o % 4)
    save_kv_operands(products.result())

    def kv_steps(ops, steps, plans, last_from):
        staged_q = staged_out = modulated = 0
        for o, (products, plan) in enumerate(zip(steps, plans)):
            for item in plan.split():
                if item == "p":
                    products.step()
                elif item == "s":
                    stage_q_weights(staged_q)
                    staged_q += 1
                elif item == "o":
                    stage_out_weights(staged_out)
                    staged_out += 1
                elif item == "V":
                    vector_modulation(GATE_A + modulated)
                    modulated += 1
                elif item == "B":
                    cp_wr.wait()
                else:
                    accumulate_kv(ops, (o - 1) % 4, last=o >= last_from)
            if o + 1 < len(plans):
                ops = kv_operands(products.result(), o % 4, last=o + 1 >= last_from)
        return products.result()

    def pass1(i, remaining):
        t = 2 * i + 2
        pl.when(i == 0)(cp_mb.start)
        pl.when(i == 1)(cp_mc.start)
        wait(x_copy(t + 2), x_copy(t + 3))
        view = h_s.at[_rows(t * HROWS, 4 * HROWS)]
        first_norm(t + 2, view, 2 * HROWS)
        first_norm(t + 3, view, 3 * HROWS)
        steps = [kv_products(view, k * HROWS, o) for k in range(2) for o in range(4)]
        save_kv_operands(kv_steps(load_kv_operands(), steps, PLAN_KV, last_from=len(steps)))
        return remaining - 1

    first_tile = lax.fori_loop(0, 2, pass1, 2)

    def q_products(t, o):
        return _Strassen(lambda i: _dot_nt(_unpack(wq_s[(i * 4 + o) * 64:(i * 4 + o + 1) * 64, :]),
                                           _unpack(h_s[_rows(t * HROWS + i * 64, 64), :])), ORDER_Q)

    def derived_params():
        wr8 = wr_v[...].astype(F32)
        wr = jnp.broadcast_to(jnp.concatenate([wr8[j:j + 1, :] for j in range(8)], axis=1), (8, D))
        scale = 1.0 + param(SCALE_B, 8)
        mod_s[:, SCALE_B * D:(SCALE_B + 1) * D] = scale
        router = scale * wr
        tables = (param(GATE_A, 8), router, scale * param(GATE_B, 8), param(SHIFT_B, 8) * param(GATE_B, 8))
        for k, row in enumerate(tables):
            store_column(k, row[0:1])
        base = ROUTER_SUMS * D
        mod_s[:, base:base + T] = jnp.broadcast_to(jnp.sum(router, axis=-1, keepdims=True), (8, T))
        mod_s[:, base + T:base + 2 * T] = jnp.broadcast_to(
            jnp.sum(param(SHIFT_B, 8) * wr, axis=-1, keepdims=True), (8, T))

    def column(k, ch):
        v = col_s[k * D + ch:k * D + ch + 128, :]
        return jnp.concatenate([v, v], axis=1)

    def feature_pairs(block, p0):
        out = []
        for j in range(2):
            phi = _hedgehog(block[j * 64:(j + 1) * 64])
            z = z_s[p0 + j]
            inv = _recip(_per_head(phi * jnp.concatenate([z, z], axis=1), jnp.add) + 1e-6)
            out.append((phi.astype(BF), inv))
        return out

    def features(r, o):
        return feature_pairs(r[0], 2 * o) + feature_pairs(r[1], 2 * o + 8)

    def save_features(r):
        raw_s[0:128, :] = r[0]
        for j, (phi, inv) in enumerate(feature_pairs(r[1], 8)):
            carry_s[j * 64:(j + 1) * 64, :] = pltpu.bitcast(phi, U32)
            raw_s[128 + 8 * j:136 + 8 * j, :] = inv

    def load_features():
        done = [(_unpack(carry_s[j * 64:(j + 1) * 64, :]), raw_s[128 + 8 * j:136 + 8 * j, :]) for j in range(2)]
        return feature_pairs(raw_s[0:128, :], 0) + done

    def attend(phis, o):
        heads = {}
        for j in (0, 2, 1, 3):
            phi, inv = phis[j]
            num = _dot(kv_s[2 * o + 8 * (j // 2) + j % 2].astype(BF), phi)
            heads[j] = jnp.concatenate([num[k * DH:(k + 1) * DH] * inv[k:k + 1] for k in range(2)], axis=0)
        return heads

    def stage_heads(dst, o, j, lo, hi):
        base = o * 64 + j * 32
        terms = _right_terms(lo[:, :U], lo[:, U:], hi[:, :U], hi[:, U:])
        dst[base:base + 32, 0:6 * U] = _pack(jnp.concatenate(terms[:6], axis=1))
        dst[base:base + 16, 6 * U:8 * U] = _pack(jnp.concatenate([terms[6][:32], terms[6][32:]], axis=1))

    def out_products(src, o):
        def product(i):
            if i < 6:
                b = src[:, i * U:(i + 1) * U]
            else:
                b = jnp.concatenate([src[k * 32:k * 32 + 16, (6 + c) * U:(7 + c) * U]
                                     for k in range(8) for c in range(2)], axis=0)
            return _dot(_unpack(wo_s[(i * 4 + o) * 64:(i * 4 + o + 1) * 64, :]), _unpack(b))
        return _Strassen(product, ORDER_OUT)

    def residual(t, o, attn, sums):
        ys = []
        for half, a in enumerate(attn):
            ch = half * KH + o * 128
            ys.append(x_v[_rows(t * T, T), ch:ch + 128].T.astype(F32) + column(COL_GATE_A, ch) * a)
        if sums is None:
            shift = jnp.sum(_fold8(ys[0]) + _fold8(ys[1]), axis=0, keepdims=True) * (1.0 / 256)
            sums = (shift, 0.0, 0.0, 0.0)
        shift, s1, s2, s3 = sums
        for half, y in enumerate(ys):
            ch = half * KH + o * 128
            d = y - shift
            for k in range(2):
                x1_s[_rows((2 * t + k) * D + ch, 128), :] = y[:, k * U:(k + 1) * U]
            s1, s2, s3 = s1 + _fold8(d), s2 + _fold8(d * d), s3 + _fold8(d * column(COL_ROUTER, ch))
        return shift, s1, s2, s3

    def route(t, sums, top):
        m1, i1, m2, i2 = top
        shift = sums[0]
        s1, s2, s3 = (jnp.sum(s, axis=0, keepdims=True) for s in sums[1:])
        delta = s1 * (1.0 / D)
        rstd = lax.rsqrt(jnp.maximum(s2 * (1.0 / D) - delta * delta, 0.0) + 1e-5)
        score = (s3 - delta * mod_s[0:1, ROUTER_SUMS * D:ROUTER_SUMS * D + T]) * rstd
        for k, v in enumerate((shift + delta, rstd)):
            for half in range(2):
                stat_s[_rows(((2 * t + half) * 2 + k) * 8, 8), :] = jnp.broadcast_to(
                    v[:, half * U:(half + 1) * U], (8, U))
        idx = lax.broadcasted_iota(I32, (1, T), 1) + t * T
        g1, g2 = score > m1, score > m2
        return (jnp.where(g1, score, m1), jnp.where(g1, idx, i1),
                jnp.where(g1, m1, jnp.where(g2, score, m2)), jnp.where(g1, i1, jnp.where(g2, idx, i2)))

    def stat(block, k, n):
        return jnp.concatenate([stat_s[_rows((block * 2 + k) * 8, 8), :]] * (n // 8), axis=0)

    def emit(t, ch):
        n = 256
        for half in range(2):
            mean, rstd = (stat(2 * t + half, k, n) for k in range(2))
            x1 = x1_s[_rows((2 * t + half) * D + ch, n), :]
            gain = rstd * col_s[COL_GAIN * D + ch:COL_GAIN * D + ch + n, :]
            res = (x1 + col_s[COL_BIAS * D + ch:COL_BIAS * D + ch + n, :]) + (x1 - mean) * gain
            out_s[_rows(t * T + half * U, U), ch:ch + n] = res.T.astype(BF)

    def q_tile(t, phis, top, plans, current, previous, more=True):
        sums, emitted = None, 0
        for o, plan in enumerate(plans):
            qs = None
            if phis is not None and (o < 3 or more):
                qs = q_products(t, o + 1) if o < 3 else q_products(t + 1, 0)
            ws = out_products(previous, o)
            heads, staged = None, 0
            for item in plan.split():
                if item == "q":
                    qs.step()
                elif item == "w":
                    ws.step()
                    if ws.done:
                        sums = residual(t - 1, o, ws.result(), sums)
                elif item == "N":
                    heads = attend(phis, o)
                elif item == "c":
                    stage_heads(current, o, staged, heads[staged], heads[staged + 2])
                    staged += 1
                elif item == "E":
                    emit(t - 2, emitted * 256)
                    emitted += 1
            if qs is not None:
                phis = features(qs.result(), o + 1) if o < 3 else qs.result()
        if sums is not None:
            top = route(t - 1, sums, top)
        if emitted:
            out_copy(t - 2).start()
        return phis, top

    wait(cp_wq, cp_wo, cp_mb, cp_mc)
    start(cp_wg, cp_wu)
    steps = [kv_products(h_s, t * HROWS, o) for t in (NT - 2, NT - 1) for o in range(4)]
    r = kv_steps(load_kv_operands(), steps + [q_products(first_tile, 0)], PLAN_KV_LAST, last_from=5)
    lowest = jnp.full((1, T), -jnp.inf, F32)
    zero = jnp.zeros((1, T), I32)
    top = (lowest, zero, lowest, zero)
    r, top = q_tile(first_tile, features(r, 0), top, PLAN_Q_FIRST, oa_s, ob_s)
    derived_params()
    r, top = q_tile(first_tile + 1, features(r, 0), top, PLAN_Q_SECOND, ob_s, oa_s)
    save_features(r)

    def pass2(i, carry):
        top, tile = carry
        pl.when(i == 2)(cp_wd.start)
        r, top = q_tile(2 * i - 2, load_features(), top, PLAN_Q, oa_s, ob_s)
        r, top = q_tile(2 * i - 1, features(r, 0), top, PLAN_Q, ob_s, oa_s)
        save_features(r)
        return top, tile + 2

    top, tile = lax.fori_loop(2, 4, pass2, (top, 2))
    wait(cp_wg, cp_wu, cp_wd)
    r, top = q_tile(tile, load_features(), top, PLAN_Q_LATE, oa_s, ob_s)
    _, top = q_tile(tile + 1, features(r, 0), top, PLAN_Q_LAST, ob_s, oa_s, more=False)
    _, top = q_tile(tile + 2, None, top, PLAN_DRAIN, oa_s, ob_s)

    m1, i1, m2, i2 = top
    best = jnp.max(m1, axis=1, keepdims=True)
    ia = jnp.min(jnp.where(m1 == best, i1, S - 1), axis=1, keepdims=True)
    taken = i1 == ia
    rest, rest_idx = jnp.where(taken, m2, m1), jnp.where(taken, i2, i1)
    second = jnp.max(rest, axis=1, keepdims=True)
    ib = jnp.min(jnp.where(rest == second, rest_idx, S - 1), axis=1, keepdims=True)
    idx = (jnp.clip(ia[0, 0], 0, S - 1), jnp.clip(ib[0, 0], 0, S - 1))

    for g in range(4):
        emit(NT - 1, g * 256)
    out_copy(NT - 1).start()
    out_copy(0).wait()

    row16 = lax.broadcasted_iota(I32, (16, U), 0)
    lane16 = lax.broadcasted_iota(I32, (16, U), 1)
    xn_sel = 0.0
    for k in range(2):
        block = idx[k] // U
        xn = (x1_s[_rows(block * D, D), :] - stat(block, 0, D)) * stat(block, 1, D)
        pick = jnp.where((row16 == k) & (lane16 == idx[k] % U), 1.0, 0.0).astype(BF)
        xn_sel = xn_sel + _dot_nt(pick, xn.astype(BF))
    hs = (xn_sel * param(SCALE_B, 16) + param(SHIFT_B, 16)).astype(BF)
    score = jnp.where(row16[:, 0:1] == 0, best, second) + mod_s[0:1, ROUTER_SUMS * D + T:ROUTER_SUMS * D + T + 1]
    gate = jax.nn.sigmoid(score)

    for k in range(2):
        store_column(COL_VEC0 + k, hs.astype(F32)[k:k + 1])

    def down(g, u, c0, c1):
        return _dot((g * jax.nn.sigmoid(g) * u).astype(BF), wd_v[c0:c1, 0:D])

    fm = F - F_VECTOR
    y = jnp.zeros((16, D), F32)
    for c0, c1 in ((0, fm // 2), (fm // 2, fm)):
        y = y + down(_dot(hs, wg_v[:, c0:c1]), _dot(hs, wu_v[:, c0:c1]), c0, c1)
    first_row = lax.broadcasted_iota(I32, (16, 256), 0) == 0
    for c0 in range(fm, F, 256):
        g, u = (jnp.where(first_row, *vector_product(w, c0, (COL_VEC0, COL_VEC1), 16)) for w in (wg_v, wu_v))
        y = y + down(g, u, c0, c0 + 256)
    update = param(GATE_B, 16) * (y * gate)

    wait(*(out_copy(t) for t in range(1, NT)))
    row = lax.broadcasted_iota(I32, (16, D), 0)

    def patch(k):
        base = pl.multiple_of((idx[k] // 16) * 16, 16)
        block = out_s[pl.ds(base, 16), :].astype(F32)
        out_s[pl.ds(base, 16), :] = jnp.where(row == idx[k] - base, block + update[k:k + 1, :], block).astype(BF)
        return pltpu.make_async_copy(out_s.at[pl.ds(base, 16)], out_hbm.at[pl.ds(base, 16)], sem_p.at[k])

    patch_a, patch_b = patch(0), patch(1)
    patch_a.start()

    @pl.when(idx[0] // 16 != idx[1] // 16)
    def _():
        patch_b.start()
        patch_b.wait()

    patch_a.wait()


@jax.jit
def pallas_adaLN_cond__linear_kernel_hedgehog__moe_arch_mod__prompt_kernel(
        A_x, A_wqkv, A_w_phi, A_wo, B_x, B_w_r, B_w_gate, B_w_up, B_w_down, c, w_mod):
    del B_x
    hbm = pl.BlockSpec(memory_space=pl.ANY)
    out = pl.pallas_call(
        _kernel,
        out_shape=jax.ShapeDtypeStruct((S, D), BF),
        in_specs=[hbm] * 10,
        out_specs=hbm,
        scratch_shapes=[
            pltpu.VMEM((S, D), BF),
            pltpu.VMEM((D, 3 * D + PAD), BF),
            pltpu.VMEM((H * DH, DH), BF),
            pltpu.VMEM((D, D + PAD), BF),
            pltpu.VMEM((8, 128), BF),
            pltpu.VMEM((D, F + PAD), BF),
            pltpu.VMEM((D, F + PAD), BF),
            pltpu.VMEM((F, D + PAD), BF),
            pltpu.VMEM((1, D), BF),
            pltpu.VMEM((D, 6 * D + PAD), BF),
            pltpu.VMEM((7 * 512, KH), U32),
            pltpu.VMEM((7 * 256, KH), U32),
            pltpu.VMEM((7 * 256, KH), U32),
            pltpu.VMEM((NT * HROWS, KH), U32),
            pltpu.VMEM((NPAIR, 64, 128), F32),
            pltpu.VMEM((8, 6 * D + 2 * T), F32),
            pltpu.VMEM((6 * D, 128), F32),
            pltpu.VMEM((2 * NT * D, U), F32),
            pltpu.VMEM((2 * NT * 2 * 8, U), F32),
            pltpu.VMEM((S, D), BF),
            pltpu.VMEM((8 * 64, 128), U32),
            pltpu.VMEM((KH // 2, 8 * U), U32),
            pltpu.VMEM((KH // 2, 8 * U), U32),
            pltpu.VMEM((8, D), U32),
            pltpu.VMEM((T, D), F32),
            pltpu.VMEM((192, T), U32),
            pltpu.VMEM((256, T), F32),
            pltpu.VMEM((NPAIR, 128, U), F32),
            pltpu.SemaphoreType.DMA((10,)),
            pltpu.SemaphoreType.DMA((4,)),
            pltpu.SemaphoreType.DMA((4,)),
            pltpu.SemaphoreType.DMA((4,)),
            pltpu.SemaphoreType.DMA((NT,)),
            pltpu.SemaphoreType.DMA((NT,)),
            pltpu.SemaphoreType.DMA((2,)),
        ],
        compiler_params=pltpu.CompilerParams(
            vmem_limit_bytes=110 * 2**20,
            flags={"XLA_TPU_EVENLY_DISTRIBUTE_CRITICAL_NODES": True}),
        name="fused_block",
    )(A_x.reshape(S, D), A_wqkv, A_w_phi.reshape(H * DH, DH), A_wo, B_w_r.reshape(8, 128),
      B_w_gate, B_w_up, B_w_down, c, w_mod)
    return out.reshape(1, S, D)
```

```python
import math

import jax
import jax.numpy as jnp
from jax import lax
import jax.experimental.pallas as pl
import jax.experimental.pallas.tpu as pltpu

S, D, H, DH, F = 2048, 1024, 32, 32, 3584
U = 128
T = 2 * U
NT = S // T
KH = D // 2
NPAIR = H // 2
HROWS = 7 * U // 2
PAD = 128
F_VECTOR = 512
LN_ROWS = 32
LOG2E = math.log2(math.e)
BF, F32, U32, I32 = jnp.bfloat16, jnp.float32, jnp.uint32, jnp.int32

SHIFT_A, SCALE_A, GATE_A, SHIFT_B, SCALE_B, GATE_B, ROUTER_SUMS = range(7)
COL_GATE_A, COL_ROUTER, COL_GAIN, COL_BIAS, COL_VEC0, COL_VEC1 = range(6)

PLAN_FIRST = (
    "p p p p", "p N F p W p p s",
    "p p p p N W F s p p p", "p p p p p p p N",
    "p W X s L N L p p p p p p", "p p N p p p p p",
    "p p N p p p p p", "p p N p p p p p")
PLAN_KV = (
    "p p N p p p p p", "p p N p p p p p",
    "p p N p p p p p", "p p N p p p p p",
    "p p p p N p p p", "p N p p p p p p",
    "p p N p p p p p", "p p N p p p p p")
PLAN_KV_LAST = (
    "p p o p p N p V p p V", "p p p p N p p p o",
    "p p p p p p p o N", "p p V p p p p p V N o",
    "B p p N p s p p p p", "s N p p s p p p p p",
    "p p p N p p p p", "s p p p N p p p p",
    "p p p p p N p p")
PLAN_Q_FIRST = (
    "q q N c c q q q q q", "q q N c c q q q q q",
    "q q q q q q N c c q", "q q N c c q q q q q")
PLAN_Q_SECOND = (
    "w w w w w w N c c w q q q q q q q", "w w w w w w N c c w q q q q q q q",
    "w w w w N c c w w w q q q q q q q", "w w w w w w N c c w q q q q q q q")
PLAN_Q = (
    "w w w w w w N c c w q q q q q q q E", "w w w N c c w w w w q q q q q q q E",
    "w w w w w N c c w w q q q q q q q E", "w w w w w N c c w w q q q q q q q E")
PLAN_Q_LATE = (
    "w N c c w w w w w w q q q q q q q E", "w w w w w N c c w w q q q q q q q E",
    "w w w w N c c w w w q q q q q q q E", "w w w w w w w q q q q q q N c c q E")
PLAN_Q_LAST = (
    "w w w w w w w q q q q N c c q q q E", "w w w w w w w q q q N c c q q q E q",
    "w w w w w w w q q N c c q q q q q E", "w w w w w w N c c w E")
PLAN_DRAIN = (
    "w w w w E w w w E", "w w w w w E w w",
    "w w w w w w w E", "w w w w w w w")
ORDER_KV = (1, 2, 3, 6, 4, 5, 7)
ORDER_Q = (4, 3, 2, 5, 1, 6, 7)
ORDER_OUT = (4, 7, 3, 1, 5, 2, 6)


def _dot(a, b):
    return jnp.dot(a, b, preferred_element_type=F32)


def _dot_nt(a, b):
    return lax.dot_general(a, b, (((1,), (1,)), ((), ())), preferred_element_type=F32)


def _pack(v):
    return pltpu.bitcast(v.astype(BF), U32)


def _unpack(v):
    return pltpu.bitcast(v, BF)


def _recip(v):
    return pl.reciprocal(v, approx=False, full_range=False)


def _rows(start, size):
    return pl.ds(start if isinstance(start, int) else pl.multiple_of(start, 8), size)


def _normalize(v):
    centered = v - jnp.mean(v, axis=-1, keepdims=True)
    var = jnp.mean(centered * centered, axis=-1, keepdims=True)
    return centered * lax.rsqrt(var + 1e-5)


def _fold8(v, op=jnp.add):
    parts = [v[i:i + 8] for i in range(0, v.shape[0], 8)]
    while len(parts) > 1:
        parts = [op(parts[i], parts[i + 1]) for i in range(0, len(parts), 2)]
    return parts[0]


def _per_head(v, op):
    r = _fold8(v, op)
    r = op(r, pltpu.roll(r, 4, 0))
    return op(r, pltpu.roll(r, 2, 0))


def _hedgehog(p):
    def spread(v):
        return jnp.concatenate([v] * 8, axis=0)

    pos = jnp.exp2(p - spread(_per_head(p, jnp.maximum)))
    neg = jnp.exp2(spread(_per_head(p, jnp.minimum)) - p)
    pos = pos * spread(_recip(_per_head(pos, jnp.add)))
    neg = neg * spread(_recip(_per_head(neg, jnp.add)))
    return jnp.concatenate([pos, neg], axis=0)


def _rotate(v, shift):
    return jnp.concatenate([pltpu.roll(v[:, i:i + 128], shift, 1) for i in range(0, v.shape[1], 128)], axis=1)


def _left_terms(a11, a12, a21, a22):
    return a11 + a22, a21 + a22, a11, a22, a11 + a12, a21 - a11, a12 - a22


def _right_terms(b11, b12, b21, b22):
    return b11 + b22, b11, b12 - b22, b21 - b11, b22, b11 + b12, b21 + b22


class _Strassen:
    _USES = {1: ((0, 1), (3, 1)), 2: ((2, 1), (3, -1)), 3: ((1, 1), (3, 1)), 4: ((0, 1), (2, 1)),
             5: ((0, -1), (1, 1)), 6: ((3, 1),), 7: ((0, 1),)}

    def __init__(self, product, order):
        self._product = product
        self._todo = list(order)
        self._c = [None] * 4

    @property
    def done(self):
        return not self._todo

    def step(self):
        i = self._todo.pop(0)
        m = self._product(i - 1)
        for k, sign in self._USES[i]:
            if self._c[k] is None:
                assert sign > 0
                self._c[k] = m
            else:
                self._c[k] = self._c[k] + m if sign > 0 else self._c[k] - m

    def result(self):
        assert self.done
        return jnp.concatenate(self._c[:2], axis=1), jnp.concatenate(self._c[2:], axis=1)


class _Blocks:
    def __init__(self, product, partial):
        self._product = product
        self._partial = partial
        self._todo = [(k, c) for k in range(2) for c in (0, 2, 1, 3)]
        self._c = [None] * 4

    def step(self):
        k, c = self._todo.pop(0)
        m = self._product(c // 2, k, c % 2)
        if k == 0:
            self._partial(c)[...] = m
        else:
            self._c[c] = m + self._partial(c)[...]

    def result(self):
        assert not self._todo
        return jnp.concatenate(self._c[:2], axis=1), jnp.concatenate(self._c[2:], axis=1)


def _kernel(x_hbm, wqkv_hbm, wphi_hbm, wo_hbm, wr_hbm, wg_hbm, wu_hbm, wd_hbm, c_hbm, wmod_hbm,
            out_hbm,
            x_v, wqkv_v, wphi_v, wo_v, wr_v, wg_v, wu_v, wd_v, c_v, wmod_v,
            wkv_s, wq_s, wo_s, h_s, kv_s, mod_s, col_s, x1_s, stat_s, out_s, fmap_s,
            oa_s, ob_s, vec_s, xn_s, carry_s, raw_s, z_s,
            sem_w, sem_m, sem_k, sem_v, sem_x, sem_o, sem_p):
    def wcopy(i, src, dst):
        return pltpu.make_async_copy(src, dst, sem_w.at[i])

    cp_c = wcopy(0, c_hbm, c_v)
    cp_phi = wcopy(1, wphi_hbm, wphi_v)
    cp_wr = wcopy(2, wr_hbm, wr_v)
    cp_wq = wcopy(3, wqkv_hbm.at[:, 0:D], wqkv_v.at[:, 0:D])
    cp_mb = wcopy(4, wmod_hbm.at[:, 2 * D:4 * D], wmod_v.at[:, 2 * D:4 * D])
    cp_mc = wcopy(5, wmod_hbm.at[:, 4 * D:6 * D], wmod_v.at[:, 4 * D:6 * D])
    cp_wo = wcopy(6, wo_hbm, wo_v.at[:, 0:D])
    cp_wg = wcopy(7, wg_hbm, wg_v.at[:, 0:F])
    cp_wu = wcopy(8, wu_hbm, wu_v.at[:, 0:F])
    cp_wd = wcopy(9, wd_hbm, wd_v.at[:, 0:D])

    def mod_copy(j):
        col0 = (j % 2) * D + (j // 2) * KH
        cols = pl.ds(col0 if isinstance(j, int) else pl.multiple_of(col0, KH), KH)
        return pltpu.make_async_copy(wmod_hbm.at[:, cols], wmod_v.at[:, cols], sem_m.at[j])

    def scale_copy(k):
        piece = (slice(k * KH, (k + 1) * KH), slice(D + KH, 2 * D))
        return pltpu.make_async_copy(wmod_hbm.at[piece], wmod_v.at[piece], sem_m.at[3 + k])

    def kv_copies(o):
        ck, cv = pl.ds(D + o * 256, 256), pl.ds(2 * D + o * 256, 256)
        return (pltpu.make_async_copy(wqkv_hbm.at[:, ck], wqkv_v.at[:, ck], sem_k.at[o]),
                pltpu.make_async_copy(wqkv_hbm.at[:, cv], wqkv_v.at[:, cv], sem_v.at[o]))

    def x_copy(t):
        rows = _rows(t * T, T)
        return pltpu.make_async_copy(x_hbm.at[rows], x_v.at[rows], sem_x.at[t])

    def out_copy(t):
        rows = _rows(t * T, T)
        return pltpu.make_async_copy(out_s.at[rows], out_hbm.at[rows], sem_o.at[t])

    def start(*copies):
        for cp in copies:
            cp.start()

    def wait(*copies):
        for cp in copies:
            cp.wait()

    def fold(col0, g):
        return _dot_nt(_unpack(fmap_s[g * 64:(g + 1) * 64, :]),
                       wqkv_v[:, col0 + g * 128:col0 + (g + 1) * 128]) * LOG2E

    def stage_left(dst, o, upper, lower):
        n = upper.shape[0] // 2
        for i, a in enumerate(_left_terms(upper[:, :KH], upper[:, KH:], lower[:, :KH], lower[:, KH:])):
            dst[(i * 4 + o) * n:(i * 4 + o + 1) * n, :] = _pack(a)

    def stage_kv_weights(o):
        blocks = []
        for g in (2 * o, 2 * o + 1):
            fk = fold(D, g)
            fv = wqkv_v[:, 2 * D + g * 128:2 * D + (g + 1) * 128].T.astype(F32)
            blocks.append(jnp.concatenate([fk[:64], fv[:64], fk[64:], fv[64:]], axis=0))
        stage_left(wkv_s, o, *blocks)
        return blocks

    def stage_q_weights(o):
        stage_left(wq_s, o, fold(0, o), fold(0, o + 4))

    def stage_out_weights(o):
        stage_left(wo_s, o, wo_v[:, o * 128:(o + 1) * 128].T.astype(F32),
                   wo_v[:, KH + o * 128:KH + (o + 1) * 128].T.astype(F32))

    def param(k, n):
        return jnp.concatenate([mod_s[:, k * D:(k + 1) * D]] * (n // 8), axis=0)

    def modulation(col0, rows=slice(0, D)):
        return _dot(_unpack(vec_s[:, rows]), wmod_v[rows, col0:col0 + KH])[0:8]

    def store_column(k, row):
        for g in range(8):
            col_s[k * D + g * 128:k * D + (g + 1) * 128, :] = jnp.broadcast_to(
                row[:, g * 128:(g + 1) * 128], (128, 128)).T

    def vector_product(w_ref, c0, tables, rows):
        accs = [None] * len(tables)
        for k0 in range(0, D, rows):
            w = w_ref[k0:k0 + rows, c0:c0 + 256].astype(F32)
            for k, table in enumerate(tables):
                v = col_s[table * D + k0:table * D + k0 + rows, :]
                part = _rotate(_fold8(w * jnp.concatenate([v, v], axis=1)), 1)
                accs[k] = part if accs[k] is None else accs[k] + part
        return [jnp.sum(_rotate(a, 127), axis=0, keepdims=True) for a in accs]

    def vector_modulation(k):
        for c0 in range(k * D, (k + 1) * D, 256):
            mod_s[:, c0:c0 + 256] = jnp.broadcast_to(vector_product(wmod_v, c0, (COL_VEC0,), 32)[0], (8, 256))

    def first_norm(t, dst, base):
        for r0 in range(0, U, LN_ROWS):
            h = []
            for half in range(2):
                rows = _rows(t * T + half * U + r0, LN_ROWS)
                xn = _normalize(x_v[rows, :].astype(F32))
                h.append(xn * param(SCALE_A, LN_ROWS) + param(SHIFT_A, LN_ROWS))
            for i, b in enumerate(_right_terms(h[0][:, :KH], h[1][:, :KH], h[0][:, KH:], h[1][:, KH:])):
                dst[base + i * 64 + r0 // 2:base + i * 64 + (r0 + LN_ROWS) // 2, :] = _pack(b)

    def kv_products(src, base, o):
        return _Strassen(lambda i: _dot_nt(_unpack(wkv_s[(i * 4 + o) * 128:(i * 4 + o + 1) * 128, :]),
                                           _unpack(src[base + i * 64:base + (i + 1) * 64, :])), ORDER_KV)

    def kv_pairs(block, p0, last=False):
        ops = []
        for j in range(2):
            phi = _hedgehog(block[j * 128:j * 128 + 64])
            z = (phi[:, :U] + phi[:, U:]) + z_s[p0 + j]
            z_s[p0 + j] = jnp.broadcast_to(jnp.sum(z, axis=1, keepdims=True), (128, U)) if last else z
            ops.append((block[j * 128 + 64:(j + 1) * 128].astype(BF), phi.astype(BF)))
        return ops

    def kv_operands(r, o, last=False):
        return kv_pairs(r[0], 4 * o, last) + kv_pairs(r[1], 4 * o + 2, last)

    def save_kv_operands(r):
        raw_s[...] = r[0]
        for j, (v, phi) in enumerate(kv_pairs(r[1], NPAIR - 2)):
            carry_s[j * 64:(j + 1) * 64, :] = pltpu.bitcast(phi, U32)
            carry_s[128 + j * 32:128 + (j + 1) * 32, :] = pltpu.bitcast(v, U32)

    def load_kv_operands():
        done = [(_unpack(carry_s[128 + j * 32:128 + (j + 1) * 32, :]), _unpack(carry_s[j * 64:(j + 1) * 64, :]))
                for j in range(2)]
        return kv_pairs(raw_s[...], NPAIR - 4) + done

    def accumulate_kv(ops, o, last=False):
        for j, (v, phi) in enumerate(ops):
            acc = _dot_nt(v, phi) + kv_s[4 * o + j]
            if last:
                row_head = lax.broadcasted_iota(I32, (64, 128), 0) // DH
                lane_head = lax.broadcasted_iota(I32, (64, 128), 1) % 2
                acc = jnp.where(row_head == lane_head, acc, 0.0)
            kv_s[4 * o + j] = acc

    start(cp_phi, cp_c, *kv_copies(0), x_copy(0), x_copy(1))
    lax.fori_loop(0, 3, lambda j, _: mod_copy(j).start(), None)
    start(scale_copy(0), scale_copy(1))
    cp_c.wait()
    cv = c_v[...].astype(F32)
    activated = cv * jax.nn.sigmoid(cv)
    vec_s[...] = _pack(jnp.broadcast_to(activated, (16, D)))
    store_column(COL_VEC0, activated)
    cp_phi.wait()
    repeat = ((lax.broadcasted_iota(I32, (128, DH), 0) % 64) // 2
              == lax.broadcasted_iota(I32, (128, DH), 1)).astype(BF)
    block_row = lax.broadcasted_iota(I32, (128, 128), 0)
    same_head = 2 * (block_row // 64) + block_row % 2 == lax.broadcasted_iota(I32, (128, 128), 1) // DH
    for g in range(8):
        full = _dot_nt(repeat, wphi_v[g * 128:(g + 1) * 128, :])
        fmap_s[g * 64:(g + 1) * 64, :] = _pack(jnp.where(same_head, full, 0.0))
    kv_s[...] = jnp.zeros(kv_s.shape, F32)
    z_s[...] = jnp.zeros(z_s.shape, F32)
    wait(*kv_copies(0))
    upper, lower = stage_kv_weights(0)
    wq_s[0:128, :] = _pack(upper[:, KH:])
    wq_s[128:256, :] = _pack(lower[:, :KH])

    def left_block(r, k):
        return wkv_s[(2 + r) * 512:(2 + r) * 512 + 128, :] if r == k else wq_s[r * 128:(r + 1) * 128, :]

    def right_block(t, k, half):
        if k == half:
            return h_s.at[t * HROWS + (1 + 3 * k) * 64:t * HROWS + (2 + 3 * k) * 64]
        return wq_s.at[256 + (2 * t + k) * 64:256 + (2 * t + k + 1) * 64]

    def early_products(t):
        return _Blocks(lambda r, k, half: _dot_nt(_unpack(left_block(r, k)), _unpack(right_block(t, k, half)[...])),
                       lambda c: x1_s.at[(4 * t + c) * 256:(4 * t + c + 1) * 256])

    def early_operands(t, k):
        cols = slice(k * KH, (k + 1) * KH)
        scale, shift = (jnp.concatenate([mod_s[:, p * D + k * KH:p * D + (k + 1) * KH]] * (U // 8), axis=0)
                        for p in (SCALE_A, SHIFT_A))
        for half in range(2):
            rows = slice(t * T + half * U, t * T + (half + 1) * U)
            h = xn_s[rows, cols] * scale + shift
            xn_s[rows, cols] = h
            right_block(t, k, half)[...] = _pack(h)

    def remaining_terms(t):
        for r0 in range(0, U, LN_ROWS):
            h = [xn_s[t * T + half * U + r0:t * T + half * U + r0 + LN_ROWS, :] for half in range(2)]
            for i, b in enumerate(_right_terms(h[0][:, :KH], h[1][:, :KH], h[0][:, KH:], h[1][:, KH:])):
                if i not in (1, 4):
                    row = t * HROWS + i * 64 + r0 // 2
                    h_s[row:row + LN_ROWS // 2, :] = _pack(b)

    for t in range(2):
        x_copy(t).wait()
        xn_s[t * T:(t + 1) * T, :] = _normalize(x_v[t * T:(t + 1) * T, :].astype(F32))
    early = [early_products(t) for t in range(2)]
    mod_copy(0).wait()
    mod_s[:, 0:KH] = modulation(0)
    mod_copy(1).wait()
    mod_s[:, D:D + KH] = modulation(D) + 1.0
    for t in range(2):
        early_operands(t, 0)
        for _ in range(4):
            early[t].step()
    mod_copy(2).wait()
    start(*kv_copies(1), *kv_copies(2))
    mod_s[:, KH:D] = modulation(KH)
    scale_copy(0).wait()
    mod_s[:, D + KH:2 * D] = modulation(D + KH, slice(0, KH)) + 1.0
    scale_copy(1).wait()
    start(*kv_copies(3))
    mod_s[:, D + KH:2 * D] += modulation(D + KH, slice(KH, D))
    for t in range(2):
        early_operands(t, 1)

    ops = None
    waited = staged = 1
    normalized = 0
    for n, plan in enumerate(PLAN_FIRST):
        products = early[n] if n < 2 else kv_products(h_s, (n % 2) * HROWS, n // 2)
        for item in plan.split():
            if item == "p":
                products.step()
            elif item == "W":
                wait(*kv_copies(waited))
                waited += 1
                if waited == 3:
                    start(x_copy(2), x_copy(3))
            elif item == "X":
                x_copy(2).wait()
                start(*(x_copy(t) for t in range(4, NT)), cp_wr, cp_wq, cp_wo)
                x_copy(3).wait()
            elif item == "s":
                stage_kv_weights(staged)
                staged += 1
            elif item == "F":
                remaining_terms(normalized)
                normalized += 1
            elif item == "L":
                first_norm(normalized, h_s, normalized * HROWS)
                normalized += 1
            else:
                accumulate_kv(ops, (n - 1) // 2)
        if n + 1 < len(PLAN_FIRST):
            ops = kv_operands(products.result(), n // 2)
    save_kv_operands(products.result())

    def kv_steps(ops, steps, plans, last_from):
        staged_q = staged_out = modulated = 0
        for o, (products, plan) in enumerate(zip(steps, plans)):
            for item in plan.split():
                if item == "p":
                    products.step()
                elif item == "s":
                    stage_q_weights(staged_q)
                    staged_q += 1
                elif item == "o":
                    stage_out_weights(staged_out)
                    staged_out += 1
                elif item == "V":
                    vector_modulation(GATE_A + modulated)
                    modulated += 1
                elif item == "B":
                    cp_wr.wait()
                else:
                    if o:
                        ops = kv_operands(projected, (o - 1) % 4, last=o >= last_from)
                    accumulate_kv(ops, (o - 1) % 4, last=o >= last_from)
            projected = products.result()
        return projected

    def pass1(i, remaining):
        t = 2 * i + 2
        pl.when(i == 0)(cp_mb.start)
        pl.when(i == 1)(cp_mc.start)
        wait(x_copy(t + 2), x_copy(t + 3))
        view = h_s.at[_rows(t * HROWS, 4 * HROWS)]
        first_norm(t + 2, view, 2 * HROWS)
        first_norm(t + 3, view, 3 * HROWS)
        steps = [kv_products(view, k * HROWS, o) for k in range(2) for o in range(4)]
        save_kv_operands(kv_steps(load_kv_operands(), steps, PLAN_KV, last_from=len(steps)))
        return remaining - 1

    first_tile = lax.fori_loop(0, 2, pass1, 2)

    def q_products(t, o):
        return _Strassen(lambda i: _dot_nt(_unpack(wq_s[(i * 4 + o) * 64:(i * 4 + o + 1) * 64, :]),
                                           _unpack(h_s[_rows(t * HROWS + i * 64, 64), :])), ORDER_Q)

    def derived_params():
        wr8 = wr_v[...].astype(F32)
        wr = jnp.broadcast_to(jnp.concatenate([wr8[j:j + 1, :] for j in range(8)], axis=1), (8, D))
        scale = 1.0 + param(SCALE_B, 8)
        mod_s[:, SCALE_B * D:(SCALE_B + 1) * D] = scale
        router = scale * wr
        tables = (param(GATE_A, 8), router, scale * param(GATE_B, 8), param(SHIFT_B, 8) * param(GATE_B, 8))
        for k, row in enumerate(tables):
            store_column(k, row[0:1])
        base = ROUTER_SUMS * D
        mod_s[:, base:base + T] = jnp.broadcast_to(jnp.sum(router, axis=-1, keepdims=True), (8, T))
        mod_s[:, base + T:base + 2 * T] = jnp.broadcast_to(
            jnp.sum(param(SHIFT_B, 8) * wr, axis=-1, keepdims=True), (8, T))

    def column(k, ch):
        v = col_s[k * D + ch:k * D + ch + 128, :]
        return jnp.concatenate([v, v], axis=1)

    def feature_pairs(block, p0):
        out = []
        for j in range(2):
            phi = _hedgehog(block[j * 64:(j + 1) * 64])
            z = z_s[p0 + j]
            inv = _recip(_per_head(phi * jnp.concatenate([z, z], axis=1), jnp.add) + 1e-6)
            out.append((phi.astype(BF), inv))
        return out

    def features(r, o):
        return feature_pairs(r[0], 2 * o) + feature_pairs(r[1], 2 * o + 8)

    def save_features(r):
        raw_s[0:128, :] = r[0]
        for j, (phi, inv) in enumerate(feature_pairs(r[1], 8)):
            carry_s[j * 64:(j + 1) * 64, :] = pltpu.bitcast(phi, U32)
            raw_s[128 + 8 * j:136 + 8 * j, :] = inv

    def load_features():
        done = [(_unpack(carry_s[j * 64:(j + 1) * 64, :]), raw_s[128 + 8 * j:136 + 8 * j, :]) for j in range(2)]
        return feature_pairs(raw_s[0:128, :], 0) + done

    def attend(phis, o):
        heads = {}
        for j in (0, 2, 1, 3):
            phi, inv = phis[j]
            num = _dot(kv_s[2 * o + 8 * (j // 2) + j % 2].astype(BF), phi)
            heads[j] = jnp.concatenate([num[k * DH:(k + 1) * DH] * inv[k:k + 1] for k in range(2)], axis=0)
        return heads

    def stage_heads(dst, o, j, lo, hi):
        base = o * 64 + j * 32
        terms = _right_terms(lo[:, :U], lo[:, U:], hi[:, :U], hi[:, U:])
        dst[base:base + 32, 0:6 * U] = _pack(jnp.concatenate(terms[:6], axis=1))
        dst[base:base + 16, 6 * U:8 * U] = _pack(jnp.concatenate([terms[6][:32], terms[6][32:]], axis=1))

    def out_products(src, o):
        def product(i):
            if i < 6:
                b = src[:, i * U:(i + 1) * U]
            else:
                b = jnp.concatenate([src[k * 32:k * 32 + 16, (6 + c) * U:(7 + c) * U]
                                     for k in range(8) for c in range(2)], axis=0)
            return _dot(_unpack(wo_s[(i * 4 + o) * 64:(i * 4 + o + 1) * 64, :]), _unpack(b))
        return _Strassen(product, ORDER_OUT)

    def residual(t, o, attn, sums):
        ys = []
        for half, a in enumerate(attn):
            ch = half * KH + o * 128
            ys.append(x_v[_rows(t * T, T), ch:ch + 128].T.astype(F32) + column(COL_GATE_A, ch) * a)
        if sums is None:
            shift = jnp.sum(_fold8(ys[0]) + _fold8(ys[1]), axis=0, keepdims=True) * (1.0 / 256)
            sums = (shift, 0.0, 0.0, 0.0)
        shift, s1, s2, s3 = sums
        for half, y in enumerate(ys):
            ch = half * KH + o * 128
            d = y - shift
            for k in range(2):
                x1_s[_rows((2 * t + k) * D + ch, 128), :] = y[:, k * U:(k + 1) * U]
            s1, s2, s3 = s1 + _fold8(d), s2 + _fold8(d * d), s3 + _fold8(d * column(COL_ROUTER, ch))
        return shift, s1, s2, s3

    def route(t, sums, top):
        m1, i1, m2, i2 = top
        shift = sums[0]
        s1, s2, s3 = (jnp.sum(s, axis=0, keepdims=True) for s in sums[1:])
        delta = s1 * (1.0 / D)
        rstd = lax.rsqrt(jnp.maximum(s2 * (1.0 / D) - delta * delta, 0.0) + 1e-5)
        score = (s3 - delta * mod_s[0:1, ROUTER_SUMS * D:ROUTER_SUMS * D + T]) * rstd
        for k, v in enumerate((shift + delta, rstd)):
            for half in range(2):
                stat_s[_rows(((2 * t + half) * 2 + k) * 8, 8), :] = jnp.broadcast_to(
                    v[:, half * U:(half + 1) * U], (8, U))
        idx = lax.broadcasted_iota(I32, (1, T), 1) + t * T
        g1, g2 = score > m1, score > m2
        return (jnp.where(g1, score, m1), jnp.where(g1, idx, i1),
                jnp.where(g1, m1, jnp.where(g2, score, m2)), jnp.where(g1, i1, jnp.where(g2, idx, i2)))

    def stat(block, k, n):
        return jnp.concatenate([stat_s[_rows((block * 2 + k) * 8, 8), :]] * (n // 8), axis=0)

    def emit(t, ch):
        n = 256
        for half in range(2):
            mean, rstd = (stat(2 * t + half, k, n) for k in range(2))
            x1 = x1_s[_rows((2 * t + half) * D + ch, n), :]
            gain = rstd * col_s[COL_GAIN * D + ch:COL_GAIN * D + ch + n, :]
            res = (x1 + col_s[COL_BIAS * D + ch:COL_BIAS * D + ch + n, :]) + (x1 - mean) * gain
            out_s[_rows(t * T + half * U, U), ch:ch + n] = res.T.astype(BF)

    def q_tile(t, phis, top, plans, current, previous, more=True):
        sums, emitted = None, 0
        for o, plan in enumerate(plans):
            qs = None
            if phis is not None and (o < 3 or more):
                qs = q_products(t, o + 1) if o < 3 else q_products(t + 1, 0)
            ws = out_products(previous, o)
            heads, staged = None, 0
            for item in plan.split():
                if item == "q":
                    qs.step()
                elif item == "w":
                    ws.step()
                    if ws.done:
                        sums = residual(t - 1, o, ws.result(), sums)
                elif item == "N":
                    heads = attend(phis, o)
                elif item == "c":
                    stage_heads(current, o, staged, heads[staged], heads[staged + 2])
                    staged += 1
                elif item == "E":
                    emit(t - 2, emitted * 256)
                    emitted += 1
            if qs is not None:
                phis = features(qs.result(), o + 1) if o < 3 else qs.result()
        if sums is not None:
            top = route(t - 1, sums, top)
        if emitted:
            out_copy(t - 2).start()
        return phis, top

    wait(cp_wq, cp_wo, cp_mb, cp_mc)
    start(cp_wg, cp_wu)
    steps = [kv_products(h_s, t * HROWS, o) for t in (NT - 2, NT - 1) for o in range(4)]
    r = kv_steps(load_kv_operands(), steps + [q_products(first_tile, 0)], PLAN_KV_LAST, last_from=5)
    lowest = jnp.full((1, T), -jnp.inf, F32)
    zero = jnp.zeros((1, T), I32)
    top = (lowest, zero, lowest, zero)
    r, top = q_tile(first_tile, features(r, 0), top, PLAN_Q_FIRST, oa_s, ob_s)
    derived_params()
    r, top = q_tile(first_tile + 1, features(r, 0), top, PLAN_Q_SECOND, ob_s, oa_s)
    save_features(r)

    def pass2(i, carry):
        top, tile = carry
        pl.when(i == 2)(cp_wd.start)
        r, top = q_tile(2 * i - 2, load_features(), top, PLAN_Q, oa_s, ob_s)
        r, top = q_tile(2 * i - 1, features(r, 0), top, PLAN_Q, ob_s, oa_s)
        save_features(r)
        return top, tile + 2

    top, tile = lax.fori_loop(2, 4, pass2, (top, 2))
    wait(cp_wg, cp_wu, cp_wd)
    r, top = q_tile(tile, load_features(), top, PLAN_Q_LATE, oa_s, ob_s)
    _, top = q_tile(tile + 1, features(r, 0), top, PLAN_Q_LAST, ob_s, oa_s, more=False)
    _, top = q_tile(tile + 2, None, top, PLAN_DRAIN, oa_s, ob_s)

    m1, i1, m2, i2 = top
    best = jnp.max(m1, axis=1, keepdims=True)
    ia = jnp.min(jnp.where(m1 == best, i1, S - 1), axis=1, keepdims=True)
    taken = i1 == ia
    rest, rest_idx = jnp.where(taken, m2, m1), jnp.where(taken, i2, i1)
    second = jnp.max(rest, axis=1, keepdims=True)
    ib = jnp.min(jnp.where(rest == second, rest_idx, S - 1), axis=1, keepdims=True)
    idx = (jnp.clip(ia[0, 0], 0, S - 1), jnp.clip(ib[0, 0], 0, S - 1))

    for g in range(4):
        emit(NT - 1, g * 256)
    out_copy(NT - 1).start()
    out_copy(0).wait()

    row16 = lax.broadcasted_iota(I32, (16, U), 0)
    lane16 = lax.broadcasted_iota(I32, (16, U), 1)
    xn_sel = 0.0
    for k in range(2):
        block = idx[k] // U
        xn = (x1_s[_rows(block * D, D), :] - stat(block, 0, D)) * stat(block, 1, D)
        pick = jnp.where((row16 == k) & (lane16 == idx[k] % U), 1.0, 0.0).astype(BF)
        xn_sel = xn_sel + _dot_nt(pick, xn.astype(BF))
    hs = (xn_sel * param(SCALE_B, 16) + param(SHIFT_B, 16)).astype(BF)
    score = jnp.where(row16[:, 0:1] == 0, best, second) + mod_s[0:1, ROUTER_SUMS * D + T:ROUTER_SUMS * D + T + 1]
    gate = jax.nn.sigmoid(score)

    for k in range(2):
        store_column(COL_VEC0 + k, hs.astype(F32)[k:k + 1])

    def down(g, u, c0, c1):
        return _dot((g * jax.nn.sigmoid(g) * u).astype(BF), wd_v[c0:c1, 0:D])

    fm = F - F_VECTOR
    y = jnp.zeros((16, D), F32)
    for c0, c1 in ((0, fm // 2), (fm // 2, fm)):
        y = y + down(_dot(hs, wg_v[:, c0:c1]), _dot(hs, wu_v[:, c0:c1]), c0, c1)
    first_row = lax.broadcasted_iota(I32, (16, 256), 0) == 0
    for c0 in range(fm, F, 256):
        g, u = (jnp.where(first_row, *vector_product(w, c0, (COL_VEC0, COL_VEC1), 16)) for w in (wg_v, wu_v))
        y = y + down(g, u, c0, c0 + 256)
    update = param(GATE_B, 16) * (y * gate)

    wait(*(out_copy(t) for t in range(1, NT)))
    row = lax.broadcasted_iota(I32, (16, D), 0)

    def patch(k):
        base = pl.multiple_of((idx[k] // 16) * 16, 16)
        block = out_s[pl.ds(base, 16), :].astype(F32)
        out_s[pl.ds(base, 16), :] = jnp.where(row == idx[k] - base, block + update[k:k + 1, :], block).astype(BF)
        return pltpu.make_async_copy(out_s.at[pl.ds(base, 16)], out_hbm.at[pl.ds(base, 16)], sem_p.at[k])

    patch_a, patch_b = patch(0), patch(1)
    patch_a.start()

    @pl.when(idx[0] // 16 != idx[1] // 16)
    def _():
        patch_b.start()
        patch_b.wait()

    patch_a.wait()


@jax.jit
def pallas_adaLN_cond__linear_kernel_hedgehog__moe_arch_mod__prompt_kernel(
        A_x, A_wqkv, A_w_phi, A_wo, B_x, B_w_r, B_w_gate, B_w_up, B_w_down, c, w_mod):
    del B_x
    hbm = pl.BlockSpec(memory_space=pl.ANY)
    out = pl.pallas_call(
        _kernel,
        out_shape=jax.ShapeDtypeStruct((S, D), BF),
        in_specs=[hbm] * 10,
        out_specs=hbm,
        scratch_shapes=[
            pltpu.VMEM((S, D), BF),
            pltpu.VMEM((D, 3 * D + PAD), BF),
            pltpu.VMEM((H * DH, DH), BF),
            pltpu.VMEM((D, D + PAD), BF),
            pltpu.VMEM((8, 128), BF),
            pltpu.VMEM((D, F + PAD), BF),
            pltpu.VMEM((D, F + PAD), BF),
            pltpu.VMEM((F, D + PAD), BF),
            pltpu.VMEM((1, D), BF),
            pltpu.VMEM((D, 6 * D + PAD), BF),
            pltpu.VMEM((7 * 512, KH), U32),
            pltpu.VMEM((7 * 256, KH), U32),
            pltpu.VMEM((7 * 256, KH), U32),
            pltpu.VMEM((NT * HROWS, KH), U32),
            pltpu.VMEM((NPAIR, 64, 128), F32),
            pltpu.VMEM((8, 6 * D + 2 * T), F32),
            pltpu.VMEM((6 * D, 128), F32),
            pltpu.VMEM((2 * NT * D, U), F32),
            pltpu.VMEM((2 * NT * 2 * 8, U), F32),
            pltpu.VMEM((S, D), BF),
            pltpu.VMEM((8 * 64, 128), U32),
            pltpu.VMEM((KH // 2, 8 * U), U32),
            pltpu.VMEM((KH // 2, 8 * U), U32),
            pltpu.VMEM((8, D), U32),
            pltpu.VMEM((2 * T, D), F32),
            pltpu.VMEM((192, T), U32),
            pltpu.VMEM((256, T), F32),
            pltpu.VMEM((NPAIR, 128, U), F32),
            pltpu.SemaphoreType.DMA((10,)),
            pltpu.SemaphoreType.DMA((5,)),
            pltpu.SemaphoreType.DMA((4,)),
            pltpu.SemaphoreType.DMA((4,)),
            pltpu.SemaphoreType.DMA((NT,)),
            pltpu.SemaphoreType.DMA((NT,)),
            pltpu.SemaphoreType.DMA((2,)),
        ],
        compiler_params=pltpu.CompilerParams(
            vmem_limit_bytes=110 * 2**20,
            flags={"XLA_TPU_EVENLY_DISTRIBUTE_CRITICAL_NODES": True}),
        name="fused_block",
    )(A_x.reshape(S, D), A_wqkv, A_w_phi.reshape(H * DH, DH), A_wo, B_w_r.reshape(8, 128),
      B_w_gate, B_w_up, B_w_down, c, w_mod)
    return out.reshape(1, S, D)
```

```python
import math

import jax
import jax.numpy as jnp
from jax import lax
import jax.experimental.pallas as pl
import jax.experimental.pallas.tpu as pltpu

S, D, H, DH, F = 2048, 1024, 32, 32, 3584
U = 128
T = 2 * U
NT = S // T
KH = D // 2
NPAIR = H // 2
HROWS = 7 * U // 2
PAD = 128
F_VECTOR = 512
LN_ROWS = 32
LOG2E = math.log2(math.e)
BF, F32, U32, I32 = jnp.bfloat16, jnp.float32, jnp.uint32, jnp.int32

SHIFT_A, SCALE_A, GATE_A, SHIFT_B, SCALE_B, GATE_B, ROUTER_SUMS = range(7)
COL_GATE_A, COL_ROUTER, COL_GAIN, COL_BIAS, COL_VEC0, COL_VEC1 = range(6)

PLAN_FIRST = (
    "p p p p", "f p N F p W p p s",
    "p p p p f N W F s p p p", "f p p p p p p p N",
    "f p W X N s L L p p p p p p", "f p p N p p p p p",
    "f p p N p p p p p", "f p p N p p p p p")
PLAN_KV = (
    "p p N p p p p p", "p p N p p p p p",
    "p p N p p p p p", "p N p p p p p p",
    "p p p p N p p p", "p N p p p p p p",
    "p p N p p p p p", "p p N p p p p p")
PLAN_KV_LAST = (
    "p p o p p N p V p p V", "p p p p N p p o p",
    "p p p p p p p N o", "p p V p p p p p V o N",
    "B p p N p s p p p p", "s N p p s p p p p p",
    "p p p N p p p p", "p s p p N p p p p",
    "p p p p p N p p")
PLAN_Q_FIRST = (
    "q q N c c q q q q q", "q q N c c q q q q q",
    "q q q q q q N c c q", "q q q N c c q q q q")
PLAN_Q_SECOND = (
    "w w w w w w N c c w q q q q q q q", "w w w w w w N c c w q q q q q q q",
    "w w w w w w w q q N c c q q q q q", "w w w w w w N c c w q q q q q q q")
PLAN_Q = (
    "w w w w w w N c c w q q q q q q q E", "w w w N c c w w w w q q q q q q q E",
    "w w w w w N c c w w q q q q q q q E", "w w w w w N c c w w q q q q q q q E")
PLAN_Q_LATE = (
    "w N c c w w w w w w q q q q q q q E", "w w w w w N c c w w q q q q q q q E",
    "w w w w N c c w w w q q q q q q q E", "w w w w w w w q q q q q q N c c q E")
PLAN_Q_LAST = (
    "w w w w w w w q q q q N c c q q q E", "w w w w w w w q q q N c c q q q E q",
    "w w w w w w w q q N c c q q q q q E", "w w w w w w N c c w E")
PLAN_DRAIN = (
    "w w w w E w w w E", "w w w w w E w w",
    "w w w w w w w E", "w w w w w w w")
ORDER_FIRST = (1, 2, 3, 6, 5, 4, 7)
ORDER_KV = (1, 2, 3, 6, 4, 5, 7)
ORDER_Q = (4, 3, 2, 5, 1, 6, 7)
ORDER_OUT = (4, 7, 3, 1, 5, 2, 6)


def _dot(a, b):
    return jnp.dot(a, b, preferred_element_type=F32)


def _dot_nt(a, b):
    return lax.dot_general(a, b, (((1,), (1,)), ((), ())), preferred_element_type=F32)


def _pack(v):
    return pltpu.bitcast(v.astype(BF), U32)


def _unpack(v):
    return pltpu.bitcast(v, BF)


def _recip(v):
    return pl.reciprocal(v, approx=False, full_range=False)


def _rows(start, size):
    return pl.ds(start if isinstance(start, int) else pl.multiple_of(start, 8), size)


def _normalize(v):
    centered = v - jnp.mean(v, axis=-1, keepdims=True)
    var = jnp.mean(centered * centered, axis=-1, keepdims=True)
    return centered * lax.rsqrt(var + 1e-5)


def _fold8(v, op=jnp.add):
    parts = [v[i:i + 8] for i in range(0, v.shape[0], 8)]
    while len(parts) > 1:
        parts = [op(parts[i], parts[i + 1]) for i in range(0, len(parts), 2)]
    return parts[0]


def _per_head(v, op):
    r = _fold8(v, op)
    r = op(r, pltpu.roll(r, 4, 0))
    return op(r, pltpu.roll(r, 2, 0))


def _hedgehog(p):
    def spread(v):
        return jnp.concatenate([v] * 8, axis=0)

    pos = jnp.exp2(p - spread(_per_head(p, jnp.maximum)))
    neg = jnp.exp2(spread(_per_head(p, jnp.minimum)) - p)
    pos = pos * spread(_recip(_per_head(pos, jnp.add)))
    neg = neg * spread(_recip(_per_head(neg, jnp.add)))
    return jnp.concatenate([pos, neg], axis=0)


def _rotate(v, shift):
    return jnp.concatenate([pltpu.roll(v[:, i:i + 128], shift, 1) for i in range(0, v.shape[1], 128)], axis=1)


def _left_terms(a11, a12, a21, a22):
    return a11 + a22, a21 + a22, a11, a22, a11 + a12, a21 - a11, a12 - a22


def _right_terms(b11, b12, b21, b22):
    return b11 + b22, b11, b12 - b22, b21 - b11, b22, b11 + b12, b21 + b22


class _Strassen:
    _USES = {1: ((0, 1), (3, 1)), 2: ((2, 1), (3, -1)), 3: ((1, 1), (3, 1)), 4: ((0, 1), (2, 1)),
             5: ((0, -1), (1, 1)), 6: ((3, 1),), 7: ((0, 1),)}

    def __init__(self, product, order):
        self._product = product
        self._todo = list(order)
        self._c = [None] * 4

    @property
    def done(self):
        return not self._todo

    def step(self):
        i = self._todo.pop(0)
        m = self._product(i - 1)
        for k, sign in self._USES[i]:
            if self._c[k] is None:
                assert sign > 0
                self._c[k] = m
            else:
                self._c[k] = self._c[k] + m if sign > 0 else self._c[k] - m

    def result(self):
        assert self.done
        return jnp.concatenate(self._c[:2], axis=1), jnp.concatenate(self._c[2:], axis=1)


class _Blocks:
    def __init__(self, product, partial):
        self._product = product
        self._partial = partial
        self._todo = [(k, c) for k in range(2) for c in (0, 2, 1, 3)]
        self._c = [None] * 4

    def step(self):
        k, c = self._todo.pop(0)
        m = self._product(c // 2, k, c % 2)
        if k == 0:
            self._partial(c)[...] = m
        else:
            self._c[c] = m + self._partial(c)[...]

    def result(self):
        assert not self._todo
        return jnp.concatenate(self._c[:2], axis=1), jnp.concatenate(self._c[2:], axis=1)


def _kernel(x_hbm, wqkv_hbm, wphi_hbm, wo_hbm, wr_hbm, wg_hbm, wu_hbm, wd_hbm, c_hbm, wmod_hbm,
            out_hbm,
            x_v, wqkv_v, wphi_v, wo_v, wr_v, wg_v, wu_v, wd_v, c_v, wmod_v,
            wkv_s, wq_s, wo_s, h_s, kv_s, mod_s, col_s, x1_s, stat_s, out_s, fmap_s,
            oa_s, ob_s, vec_s, xn_s, carry_s, raw_s, z_s,
            sem_w, sem_m, sem_k, sem_v, sem_x, sem_o, sem_p):
    def wcopy(i, src, dst):
        return pltpu.make_async_copy(src, dst, sem_w.at[i])

    cp_c = wcopy(0, c_hbm, c_v)
    cp_phi = wcopy(1, wphi_hbm, wphi_v)
    cp_wr = wcopy(2, wr_hbm, wr_v)
    cp_wq = wcopy(3, wqkv_hbm.at[:, 0:D], wqkv_v.at[:, 0:D])
    cp_mb = wcopy(4, wmod_hbm.at[:, 2 * D:4 * D], wmod_v.at[:, 2 * D:4 * D])
    cp_mc = wcopy(5, wmod_hbm.at[:, 4 * D:6 * D], wmod_v.at[:, 4 * D:6 * D])
    cp_wo = wcopy(6, wo_hbm, wo_v.at[:, 0:D])
    cp_wg = wcopy(7, wg_hbm, wg_v.at[:, 0:F])
    cp_wu = wcopy(8, wu_hbm, wu_v.at[:, 0:F])
    cp_wd = wcopy(9, wd_hbm, wd_v.at[:, 0:D])

    def mod_copy(j):
        col0 = (j % 2) * D + (j // 2) * KH
        cols = pl.ds(col0 if isinstance(j, int) else pl.multiple_of(col0, KH), KH)
        return pltpu.make_async_copy(wmod_hbm.at[:, cols], wmod_v.at[:, cols], sem_m.at[j])

    def scale_copy(k):
        piece = (slice(k * KH, (k + 1) * KH), slice(D + KH, 2 * D))
        return pltpu.make_async_copy(wmod_hbm.at[piece], wmod_v.at[piece], sem_m.at[3 + k])

    def kv_copies(o):
        ck, cv = pl.ds(D + o * 256, 256), pl.ds(2 * D + o * 256, 256)
        return (pltpu.make_async_copy(wqkv_hbm.at[:, ck], wqkv_v.at[:, ck], sem_k.at[o]),
                pltpu.make_async_copy(wqkv_hbm.at[:, cv], wqkv_v.at[:, cv], sem_v.at[o]))

    def x_copy(t):
        rows = _rows(t * T, T)
        return pltpu.make_async_copy(x_hbm.at[rows], x_v.at[rows], sem_x.at[t])

    def out_copy(t):
        rows = _rows(t * T, T)
        return pltpu.make_async_copy(out_s.at[rows], out_hbm.at[rows], sem_o.at[t])

    def start(*copies):
        for cp in copies:
            cp.start()

    def wait(*copies):
        for cp in copies:
            cp.wait()

    def fold(col0, g):
        return _dot_nt(_unpack(fmap_s[g * 64:(g + 1) * 64, :]),
                       wqkv_v[:, col0 + g * 128:col0 + (g + 1) * 128]) * LOG2E

    def stage_left(dst, o, upper, lower):
        n = upper.shape[0] // 2
        for i, a in enumerate(_left_terms(upper[:, :KH], upper[:, KH:], lower[:, :KH], lower[:, KH:])):
            dst[(i * 4 + o) * n:(i * 4 + o + 1) * n, :] = _pack(a)

    def stage_kv_weights(o):
        blocks = []
        for g in (2 * o, 2 * o + 1):
            fk = fold(D, g)
            fv = wqkv_v[:, 2 * D + g * 128:2 * D + (g + 1) * 128].T.astype(F32)
            blocks.append(jnp.concatenate([fk[:64], fv[:64], fk[64:], fv[64:]], axis=0))
        stage_left(wkv_s, o, *blocks)
        return blocks

    def stage_q_weights(o):
        stage_left(wq_s, o, fold(0, o), fold(0, o + 4))

    def stage_out_weights(o):
        stage_left(wo_s, o, wo_v[:, o * 128:(o + 1) * 128].T.astype(F32),
                   wo_v[:, KH + o * 128:KH + (o + 1) * 128].T.astype(F32))

    def param(k, n):
        return jnp.concatenate([mod_s[:, k * D:(k + 1) * D]] * (n // 8), axis=0)

    def modulation(col0, rows=slice(0, D)):
        return _dot(_unpack(vec_s[:, rows]), wmod_v[rows, col0:col0 + KH])[0:8]

    def store_column(k, row):
        for g in range(8):
            col_s[k * D + g * 128:k * D + (g + 1) * 128, :] = jnp.broadcast_to(
                row[:, g * 128:(g + 1) * 128], (128, 128)).T

    def vector_product(w_ref, c0, tables, rows):
        accs = [None] * len(tables)
        for k0 in range(0, D, rows):
            w = w_ref[k0:k0 + rows, c0:c0 + 256].astype(F32)
            for k, table in enumerate(tables):
                v = col_s[table * D + k0:table * D + k0 + rows, :]
                part = _rotate(_fold8(w * jnp.concatenate([v, v], axis=1)), 1)
                accs[k] = part if accs[k] is None else accs[k] + part
        return [jnp.sum(_rotate(a, 127), axis=0, keepdims=True) for a in accs]

    def vector_modulation(k):
        for c0 in range(k * D, (k + 1) * D, 256):
            mod_s[:, c0:c0 + 256] = jnp.broadcast_to(vector_product(wmod_v, c0, (COL_VEC0,), 32)[0], (8, 256))

    def first_norm(t, dst, base):
        for r0 in range(0, U, LN_ROWS):
            h = []
            for half in range(2):
                rows = _rows(t * T + half * U + r0, LN_ROWS)
                xn = _normalize(x_v[rows, :].astype(F32))
                h.append(xn * param(SCALE_A, LN_ROWS) + param(SHIFT_A, LN_ROWS))
            for i, b in enumerate(_right_terms(h[0][:, :KH], h[1][:, :KH], h[0][:, KH:], h[1][:, KH:])):
                dst[base + i * 64 + r0 // 2:base + i * 64 + (r0 + LN_ROWS) // 2, :] = _pack(b)

    def kv_products(src, base, o, order=ORDER_KV):
        return _Strassen(lambda i: _dot_nt(_unpack(wkv_s[(i * 4 + o) * 128:(i * 4 + o + 1) * 128, :]),
                                           _unpack(src[base + i * 64:base + (i + 1) * 64, :])), order)

    def kv_pairs(block, p0, last=False):
        ops = []
        for j in range(2):
            phi = _hedgehog(block[j * 128:j * 128 + 64])
            z = (phi[:, :U] + phi[:, U:]) + z_s[p0 + j]
            z_s[p0 + j] = jnp.broadcast_to(jnp.sum(z, axis=1, keepdims=True), (128, U)) if last else z
            ops.append((block[j * 128 + 64:(j + 1) * 128].astype(BF), phi.astype(BF)))
        return ops

    def kv_operands(r, o, last=False):
        return kv_pairs(r[0], 4 * o, last) + kv_pairs(r[1], 4 * o + 2, last)

    def save_kv_operands(r):
        raw_s[...] = r[0]
        for j, (v, phi) in enumerate(kv_pairs(r[1], NPAIR - 2)):
            carry_s[j * 64:(j + 1) * 64, :] = pltpu.bitcast(phi, U32)
            carry_s[128 + j * 32:128 + (j + 1) * 32, :] = pltpu.bitcast(v, U32)

    def load_kv_operands():
        done = [(_unpack(carry_s[128 + j * 32:128 + (j + 1) * 32, :]), _unpack(carry_s[j * 64:(j + 1) * 64, :]))
                for j in range(2)]
        return kv_pairs(raw_s[...], NPAIR - 4) + done

    def accumulate_kv(ops, o, last=False):
        for j, (v, phi) in enumerate(ops):
            acc = _dot_nt(v, phi) + kv_s[4 * o + j]
            if last:
                row_head = lax.broadcasted_iota(I32, (64, 128), 0) // DH
                lane_head = lax.broadcasted_iota(I32, (64, 128), 1) % 2
                acc = jnp.where(row_head == lane_head, acc, 0.0)
            kv_s[4 * o + j] = acc

    start(cp_phi, cp_c, *kv_copies(0), x_copy(0), x_copy(1))
    lax.fori_loop(0, 3, lambda j, _: mod_copy(j).start(), None)
    start(scale_copy(0), scale_copy(1))
    cp_c.wait()
    cv = c_v[...].astype(F32)
    activated = cv * jax.nn.sigmoid(cv)
    vec_s[...] = _pack(jnp.broadcast_to(activated, (16, D)))
    store_column(COL_VEC0, activated)
    cp_phi.wait()
    repeat = ((lax.broadcasted_iota(I32, (128, DH), 0) % 64) // 2
              == lax.broadcasted_iota(I32, (128, DH), 1)).astype(BF)
    block_row = lax.broadcasted_iota(I32, (128, 128), 0)
    same_head = 2 * (block_row // 64) + block_row % 2 == lax.broadcasted_iota(I32, (128, 128), 1) // DH
    for g in range(8):
        full = _dot_nt(repeat, wphi_v[g * 128:(g + 1) * 128, :])
        fmap_s[g * 64:(g + 1) * 64, :] = _pack(jnp.where(same_head, full, 0.0))
    kv_s[...] = jnp.zeros(kv_s.shape, F32)
    z_s[...] = jnp.zeros(z_s.shape, F32)
    wait(*kv_copies(0))
    upper, lower = stage_kv_weights(0)
    wq_s[0:128, :] = _pack(upper[:, KH:])
    wq_s[128:256, :] = _pack(lower[:, :KH])

    def left_block(r, k):
        return wkv_s[(2 + r) * 512:(2 + r) * 512 + 128, :] if r == k else wq_s[r * 128:(r + 1) * 128, :]

    def right_block(t, k, half):
        if k == half:
            return h_s.at[t * HROWS + (1 + 3 * k) * 64:t * HROWS + (2 + 3 * k) * 64]
        return wq_s.at[256 + (2 * t + k) * 64:256 + (2 * t + k + 1) * 64]

    def early_products(t):
        return _Blocks(lambda r, k, half: _dot_nt(_unpack(left_block(r, k)), _unpack(right_block(t, k, half)[...])),
                       lambda c: x1_s.at[(4 * t + c) * 256:(4 * t + c + 1) * 256])

    def early_operands(t, k):
        cols = slice(k * KH, (k + 1) * KH)
        scale, shift = (jnp.concatenate([mod_s[:, p * D + k * KH:p * D + (k + 1) * KH]] * (U // 8), axis=0)
                        for p in (SCALE_A, SHIFT_A))
        for half in range(2):
            rows = slice(t * T + half * U, t * T + (half + 1) * U)
            h = xn_s[rows, cols] * scale + shift
            xn_s[rows, cols] = h
            right_block(t, k, half)[...] = _pack(h)

    def remaining_terms(t):
        for r0 in range(0, U, LN_ROWS):
            h = [xn_s[t * T + half * U + r0:t * T + half * U + r0 + LN_ROWS, :] for half in range(2)]
            for i, b in enumerate(_right_terms(h[0][:, :KH], h[1][:, :KH], h[0][:, KH:], h[1][:, KH:])):
                if i not in (1, 4):
                    row = t * HROWS + i * 64 + r0 // 2
                    h_s[row:row + LN_ROWS // 2, :] = _pack(b)

    for t in range(2):
        x_copy(t).wait()
        xn_s[t * T:(t + 1) * T, :] = _normalize(x_v[t * T:(t + 1) * T, :].astype(F32))
    early = [early_products(t) for t in range(2)]
    mod_copy(0).wait()
    mod_s[:, 0:KH] = modulation(0)
    mod_copy(1).wait()
    mod_s[:, D:D + KH] = modulation(D) + 1.0
    for t in range(2):
        early_operands(t, 0)
        for _ in range(4):
            early[t].step()
    mod_copy(2).wait()
    start(*kv_copies(1), *kv_copies(2))
    mod_s[:, KH:D] = modulation(KH)
    scale_copy(0).wait()
    mod_s[:, D + KH:2 * D] = modulation(D + KH, slice(0, KH)) + 1.0
    scale_copy(1).wait()
    start(*kv_copies(3))
    mod_s[:, D + KH:2 * D] += modulation(D + KH, slice(KH, D))
    for t in range(2):
        early_operands(t, 1)

    waited = staged = 1
    normalized = 0
    for n, plan in enumerate(PLAN_FIRST):
        products = early[n] if n < 2 else kv_products(h_s, (n % 2) * HROWS, n // 2, ORDER_FIRST)
        for item in plan.split():
            if item == "p":
                products.step()
            elif item == "W":
                wait(*kv_copies(waited))
                waited += 1
                if waited == 3:
                    start(x_copy(2), x_copy(3))
            elif item == "X":
                x_copy(2).wait()
                start(*(x_copy(t) for t in range(4, NT)), cp_wr, cp_wq, cp_wo)
                x_copy(3).wait()
            elif item == "s":
                stage_kv_weights(staged)
                staged += 1
            elif item == "F":
                remaining_terms(normalized)
                normalized += 1
            elif item == "L":
                first_norm(normalized, h_s, normalized * HROWS)
                normalized += 1
            elif item == "f":
                ops = kv_operands(projected, (n - 1) // 2)
            else:
                accumulate_kv(ops, (n - 1) // 2)
        projected = products.result()
    save_kv_operands(projected)

    def kv_steps(ops, steps, plans, last_from):
        staged_q = staged_out = modulated = 0
        for o, (products, plan) in enumerate(zip(steps, plans)):
            for item in plan.split():
                if item == "p":
                    products.step()
                elif item == "s":
                    stage_q_weights(staged_q)
                    staged_q += 1
                elif item == "o":
                    stage_out_weights(staged_out)
                    staged_out += 1
                elif item == "V":
                    vector_modulation(GATE_A + modulated)
                    modulated += 1
                elif item == "B":
                    cp_wr.wait()
                else:
                    if o:
                        ops = kv_operands(projected, (o - 1) % 4, last=o >= last_from)
                    accumulate_kv(ops, (o - 1) % 4, last=o >= last_from)
            projected = products.result()
        return projected

    def pass1(i, remaining):
        t = 2 * i + 2
        pl.when(i == 0)(cp_mb.start)
        pl.when(i == 1)(cp_mc.start)
        wait(x_copy(t + 2), x_copy(t + 3))
        view = h_s.at[_rows(t * HROWS, 4 * HROWS)]
        first_norm(t + 2, view, 2 * HROWS)
        first_norm(t + 3, view, 3 * HROWS)
        steps = [kv_products(view, k * HROWS, o) for k in range(2) for o in range(4)]
        save_kv_operands(kv_steps(load_kv_operands(), steps, PLAN_KV, last_from=len(steps)))
        return remaining - 1

    first_tile = lax.fori_loop(0, 2, pass1, 2)

    def q_products(t, o):
        return _Strassen(lambda i: _dot_nt(_unpack(wq_s[(i * 4 + o) * 64:(i * 4 + o + 1) * 64, :]),
                                           _unpack(h_s[_rows(t * HROWS + i * 64, 64), :])), ORDER_Q)

    def derived_params():
        wr8 = wr_v[...].astype(F32)
        wr = jnp.broadcast_to(jnp.concatenate([wr8[j:j + 1, :] for j in range(8)], axis=1), (8, D))
        scale = 1.0 + param(SCALE_B, 8)
        mod_s[:, SCALE_B * D:(SCALE_B + 1) * D] = scale
        router = scale * wr
        tables = (param(GATE_A, 8), router, scale * param(GATE_B, 8), param(SHIFT_B, 8) * param(GATE_B, 8))
        for k, row in enumerate(tables):
            store_column(k, row[0:1])
        base = ROUTER_SUMS * D
        mod_s[:, base:base + T] = jnp.broadcast_to(jnp.sum(router, axis=-1, keepdims=True), (8, T))
        mod_s[:, base + T:base + 2 * T] = jnp.broadcast_to(
            jnp.sum(param(SHIFT_B, 8) * wr, axis=-1, keepdims=True), (8, T))

    def column(k, ch):
        v = col_s[k * D + ch:k * D + ch + 128, :]
        return jnp.concatenate([v, v], axis=1)

    def feature_pairs(block, p0):
        out = []
        for j in range(2):
            phi = _hedgehog(block[j * 64:(j + 1) * 64])
            z = z_s[p0 + j]
            inv = _recip(_per_head(phi * jnp.concatenate([z, z], axis=1), jnp.add) + 1e-6)
            out.append((phi.astype(BF), inv))
        return out

    def features(r, o):
        return feature_pairs(r[0], 2 * o) + feature_pairs(r[1], 2 * o + 8)

    def save_features(r):
        raw_s[0:128, :] = r[0]
        for j, (phi, inv) in enumerate(feature_pairs(r[1], 8)):
            carry_s[j * 64:(j + 1) * 64, :] = pltpu.bitcast(phi, U32)
            raw_s[128 + 8 * j:136 + 8 * j, :] = inv

    def load_features():
        done = [(_unpack(carry_s[j * 64:(j + 1) * 64, :]), raw_s[128 + 8 * j:136 + 8 * j, :]) for j in range(2)]
        return feature_pairs(raw_s[0:128, :], 0) + done

    def attend(phis, o):
        heads = {}
        for j in (0, 2, 1, 3):
            phi, inv = phis[j]
            num = _dot(kv_s[2 * o + 8 * (j // 2) + j % 2].astype(BF), phi)
            heads[j] = jnp.concatenate([num[k * DH:(k + 1) * DH] * inv[k:k + 1] for k in range(2)], axis=0)
        return heads

    def stage_heads(dst, o, j, lo, hi):
        base = o * 64 + j * 32
        terms = _right_terms(lo[:, :U], lo[:, U:], hi[:, :U], hi[:, U:])
        dst[base:base + 32, 0:6 * U] = _pack(jnp.concatenate(terms[:6], axis=1))
        dst[base:base + 16, 6 * U:8 * U] = _pack(jnp.concatenate([terms[6][:32], terms[6][32:]], axis=1))

    def out_products(src, o):
        def product(i):
            if i < 6:
                b = src[:, i * U:(i + 1) * U]
            else:
                b = jnp.concatenate([src[k * 32:k * 32 + 16, (6 + c) * U:(7 + c) * U]
                                     for k in range(8) for c in range(2)], axis=0)
            return _dot(_unpack(wo_s[(i * 4 + o) * 64:(i * 4 + o + 1) * 64, :]), _unpack(b))
        return _Strassen(product, ORDER_OUT)

    def residual(t, o, attn, sums):
        ys = []
        for half, a in enumerate(attn):
            ch = half * KH + o * 128
            ys.append(x_v[_rows(t * T, T), ch:ch + 128].T.astype(F32) + column(COL_GATE_A, ch) * a)
        if sums is None:
            shift = jnp.sum(_fold8(ys[0]) + _fold8(ys[1]), axis=0, keepdims=True) * (1.0 / 256)
            sums = (shift, 0.0, 0.0, 0.0)
        shift, s1, s2, s3 = sums
        for half, y in enumerate(ys):
            ch = half * KH + o * 128
            d = y - shift
            for k in range(2):
                x1_s[_rows((2 * t + k) * D + ch, 128), :] = y[:, k * U:(k + 1) * U]
            s1, s2, s3 = s1 + _fold8(d), s2 + _fold8(d * d), s3 + _fold8(d * column(COL_ROUTER, ch))
        return shift, s1, s2, s3

    def route(t, sums, top):
        m1, i1, m2, i2 = top
        shift = sums[0]
        s1, s2, s3 = (jnp.sum(s, axis=0, keepdims=True) for s in sums[1:])
        delta = s1 * (1.0 / D)
        rstd = lax.rsqrt(jnp.maximum(s2 * (1.0 / D) - delta * delta, 0.0) + 1e-5)
        score = (s3 - delta * mod_s[0:1, ROUTER_SUMS * D:ROUTER_SUMS * D + T]) * rstd
        for k, v in enumerate((shift + delta, rstd)):
            for half in range(2):
                stat_s[_rows(((2 * t + half) * 2 + k) * 8, 8), :] = jnp.broadcast_to(
                    v[:, half * U:(half + 1) * U], (8, U))
        idx = lax.broadcasted_iota(I32, (1, T), 1) + t * T
        g1, g2 = score > m1, score > m2
        return (jnp.where(g1, score, m1), jnp.where(g1, idx, i1),
                jnp.where(g1, m1, jnp.where(g2, score, m2)), jnp.where(g1, i1, jnp.where(g2, idx, i2)))

    def stat(block, k, n):
        return jnp.concatenate([stat_s[_rows((block * 2 + k) * 8, 8), :]] * (n // 8), axis=0)

    def emit(t, ch):
        n = 256
        for half in range(2):
            mean, rstd = (stat(2 * t + half, k, n) for k in range(2))
            x1 = x1_s[_rows((2 * t + half) * D + ch, n), :]
            gain = rstd * col_s[COL_GAIN * D + ch:COL_GAIN * D + ch + n, :]
            res = (x1 + col_s[COL_BIAS * D + ch:COL_BIAS * D + ch + n, :]) + (x1 - mean) * gain
            out_s[_rows(t * T + half * U, U), ch:ch + n] = res.T.astype(BF)

    def q_tile(t, phis, top, plans, current, previous, more=True):
        sums, emitted = None, 0
        for o, plan in enumerate(plans):
            qs = None
            if phis is not None and (o < 3 or more):
                qs = q_products(t, o + 1) if o < 3 else q_products(t + 1, 0)
            ws = out_products(previous, o)
            heads, staged = None, 0
            for item in plan.split():
                if item == "q":
                    qs.step()
                elif item == "w":
                    ws.step()
                    if ws.done:
                        sums = residual(t - 1, o, ws.result(), sums)
                elif item == "N":
                    heads = attend(phis, o)
                elif item == "c":
                    stage_heads(current, o, staged, heads[staged], heads[staged + 2])
                    staged += 1
                elif item == "E":
                    emit(t - 2, emitted * 256)
                    emitted += 1
            if qs is not None:
                phis = features(qs.result(), o + 1) if o < 3 else qs.result()
        if sums is not None:
            top = route(t - 1, sums, top)
        if emitted:
            out_copy(t - 2).start()
        return phis, top

    wait(cp_wq, cp_wo, cp_mb, cp_mc)
    start(cp_wg, cp_wu)
    steps = [kv_products(h_s, t * HROWS, o) for t in (NT - 2, NT - 1) for o in range(4)]
    r = kv_steps(load_kv_operands(), steps + [q_products(first_tile, 0)], PLAN_KV_LAST, last_from=5)
    lowest = jnp.full((1, T), -jnp.inf, F32)
    zero = jnp.zeros((1, T), I32)
    top = (lowest, zero, lowest, zero)
    r, top = q_tile(first_tile, features(r, 0), top, PLAN_Q_FIRST, oa_s, ob_s)
    derived_params()
    r, top = q_tile(first_tile + 1, features(r, 0), top, PLAN_Q_SECOND, ob_s, oa_s)
    save_features(r)

    def pass2(i, carry):
        top, tile = carry
        pl.when(i == 2)(cp_wd.start)
        r, top = q_tile(2 * i - 2, load_features(), top, PLAN_Q, oa_s, ob_s)
        r, top = q_tile(2 * i - 1, features(r, 0), top, PLAN_Q, ob_s, oa_s)
        save_features(r)
        return top, tile + 2

    top, tile = lax.fori_loop(2, 4, pass2, (top, 2))
    wait(cp_wg, cp_wu, cp_wd)
    r, top = q_tile(tile, load_features(), top, PLAN_Q_LATE, oa_s, ob_s)
    _, top = q_tile(tile + 1, features(r, 0), top, PLAN_Q_LAST, ob_s, oa_s, more=False)
    _, top = q_tile(tile + 2, None, top, PLAN_DRAIN, oa_s, ob_s)

    m1, i1, m2, i2 = top
    best = jnp.max(m1, axis=1, keepdims=True)
    ia = jnp.min(jnp.where(m1 == best, i1, S - 1), axis=1, keepdims=True)
    taken = i1 == ia
    rest, rest_idx = jnp.where(taken, m2, m1), jnp.where(taken, i2, i1)
    second = jnp.max(rest, axis=1, keepdims=True)
    ib = jnp.min(jnp.where(rest == second, rest_idx, S - 1), axis=1, keepdims=True)
    idx = (jnp.clip(ia[0, 0], 0, S - 1), jnp.clip(ib[0, 0], 0, S - 1))

    for g in range(4):
        emit(NT - 1, g * 256)
    out_copy(NT - 1).start()
    out_copy(0).wait()

    row16 = lax.broadcasted_iota(I32, (16, U), 0)
    lane16 = lax.broadcasted_iota(I32, (16, U), 1)
    xn_sel = 0.0
    for k in range(2):
        block = idx[k] // U
        xn = (x1_s[_rows(block * D, D), :] - stat(block, 0, D)) * stat(block, 1, D)
        pick = jnp.where((row16 == k) & (lane16 == idx[k] % U), 1.0, 0.0).astype(BF)
        xn_sel = xn_sel + _dot_nt(pick, xn.astype(BF))
    hs = (xn_sel * param(SCALE_B, 16) + param(SHIFT_B, 16)).astype(BF)
    score = jnp.where(row16[:, 0:1] == 0, best, second) + mod_s[0:1, ROUTER_SUMS * D + T:ROUTER_SUMS * D + T + 1]
    gate = jax.nn.sigmoid(score)

    for k in range(2):
        store_column(COL_VEC0 + k, hs.astype(F32)[k:k + 1])

    def down(g, u, c0, c1):
        return _dot((g * jax.nn.sigmoid(g) * u).astype(BF), wd_v[c0:c1, 0:D])

    fm = F - F_VECTOR
    y = jnp.zeros((16, D), F32)
    for c0, c1 in ((0, fm // 2), (fm // 2, fm)):
        y = y + down(_dot(hs, wg_v[:, c0:c1]), _dot(hs, wu_v[:, c0:c1]), c0, c1)
    first_row = lax.broadcasted_iota(I32, (16, 256), 0) == 0
    for c0 in range(fm, F, 256):
        g, u = (jnp.where(first_row, *vector_product(w, c0, (COL_VEC0, COL_VEC1), 16)) for w in (wg_v, wu_v))
        y = y + down(g, u, c0, c0 + 256)
    update = param(GATE_B, 16) * (y * gate)

    wait(*(out_copy(t) for t in range(1, NT)))
    row = lax.broadcasted_iota(I32, (16, D), 0)

    def patch(k):
        base = pl.multiple_of((idx[k] // 16) * 16, 16)
        block = out_s[pl.ds(base, 16), :].astype(F32)
        out_s[pl.ds(base, 16), :] = jnp.where(row == idx[k] - base, block + update[k:k + 1, :], block).astype(BF)
        return pltpu.make_async_copy(out_s.at[pl.ds(base, 16)], out_hbm.at[pl.ds(base, 16)], sem_p.at[k])

    patch_a, patch_b = patch(0), patch(1)
    patch_a.start()

    @pl.when(idx[0] // 16 != idx[1] // 16)
    def _():
        patch_b.start()
        patch_b.wait()

    patch_a.wait()


@jax.jit
def pallas_adaLN_cond__linear_kernel_hedgehog__moe_arch_mod__prompt_kernel(
        A_x, A_wqkv, A_w_phi, A_wo, B_x, B_w_r, B_w_gate, B_w_up, B_w_down, c, w_mod):
    del B_x
    hbm = pl.BlockSpec(memory_space=pl.ANY)
    out = pl.pallas_call(
        _kernel,
        out_shape=jax.ShapeDtypeStruct((S, D), BF),
        in_specs=[hbm] * 10,
        out_specs=hbm,
        scratch_shapes=[
            pltpu.VMEM((S, D), BF),
            pltpu.VMEM((D, 3 * D + PAD), BF),
            pltpu.VMEM((H * DH, DH), BF),
            pltpu.VMEM((D, D + PAD), BF),
            pltpu.VMEM((8, 128), BF),
            pltpu.VMEM((D, F + PAD), BF),
            pltpu.VMEM((D, F + PAD), BF),
            pltpu.VMEM((F, D + PAD), BF),
            pltpu.VMEM((1, D), BF),
            pltpu.VMEM((D, 6 * D + PAD), BF),
            pltpu.VMEM((7 * 512, KH), U32),
            pltpu.VMEM((7 * 256, KH), U32),
            pltpu.VMEM((7 * 256, KH), U32),
            pltpu.VMEM((NT * HROWS, KH), U32),
            pltpu.VMEM((NPAIR, 64, 128), F32),
            pltpu.VMEM((8, 6 * D + 2 * T), F32),
            pltpu.VMEM((6 * D, 128), F32),
            pltpu.VMEM((2 * NT * D, U), F32),
            pltpu.VMEM((2 * NT * 2 * 8, U), F32),
            pltpu.VMEM((S, D), BF),
            pltpu.VMEM((8 * 64, 128), U32),
            pltpu.VMEM((KH // 2, 8 * U), U32),
            pltpu.VMEM((KH // 2, 8 * U), U32),
            pltpu.VMEM((8, D), U32),
            pltpu.VMEM((2 * T, D), F32),
            pltpu.VMEM((192, T), U32),
            pltpu.VMEM((256, T), F32),
            pltpu.VMEM((NPAIR, 128, U), F32),
            pltpu.SemaphoreType.DMA((10,)),
            pltpu.SemaphoreType.DMA((5,)),
            pltpu.SemaphoreType.DMA((4,)),
            pltpu.SemaphoreType.DMA((4,)),
            pltpu.SemaphoreType.DMA((NT,)),
            pltpu.SemaphoreType.DMA((NT,)),
            pltpu.SemaphoreType.DMA((2,)),
        ],
        compiler_params=pltpu.CompilerParams(
            vmem_limit_bytes=110 * 2**20,
            flags={"XLA_TPU_EVENLY_DISTRIBUTE_CRITICAL_NODES": True}),
        name="fused_block",
    )(A_x.reshape(S, D), A_wqkv, A_w_phi.reshape(H * DH, DH), A_wo, B_w_r.reshape(8, 128),
      B_w_gate, B_w_up, B_w_down, c, w_mod)
    return out.reshape(1, S, D)
```

```python
import math

import jax
import jax.numpy as jnp
from jax import lax
import jax.experimental.pallas as pl
import jax.experimental.pallas.tpu as pltpu

S, D, H, DH, F = 2048, 1024, 32, 32, 3584
U = 128
T = 2 * U
NT = S // T
KH = D // 2
NPAIR = H // 2
HROWS = 7 * U // 2
PAD = 128
F_VECTOR = 512
LN_ROWS = 32
LOG2E = math.log2(math.e)
BF, F32, U32, I32 = jnp.bfloat16, jnp.float32, jnp.uint32, jnp.int32

SHIFT_A, SCALE_A, GATE_A, SHIFT_B, SCALE_B, GATE_B, ROUTER_SUMS = range(7)
COL_GATE_A, COL_ROUTER, COL_GAIN, COL_BIAS, COL_VEC0, COL_VEC1 = range(6)

PLAN_FIRST = (
    "p p p p", "f p N F p W p p s",
    "p p p p f N W F s p p p", "f p p p p p p p N",
    "f p N W X s L L p p p p p p", "f p p p N p p p p",
    "f p p N p p p p p", "f p p p p N p p p")
PLAN_KV = (
    "p p N p p p p p", "p p N p p p p p",
    "p p N p p p p p", "p N p p p p p p",
    "p p p p N p p p", "p N p p p p p p",
    "p p N p p p p p", "p p N p p p p p")
PLAN_KV_LAST = (
    "o p p o p V p N p V p p", "p p p p N p p p o",
    "p p p p p p p N", "p p V p p p p V p o N",
    "B p p N s p p p p p", "s N p p s p p p p p",
    "p p p N p p p p", "p s p N p p p p p",
    "p p p p p N p p")
PLAN_Q_FIRST = (
    "q q N c c q q q q q", "q q N c c q q q q q",
    "q q q q q q N c c q", "q q q N c c q q q q")
PLAN_Q_SECOND = (
    "w w w w w w N c c w q q q q q q q", "w w w w w w N c c w q q q q q q q",
    "w w w w w w w q q N c c q q q q q", "w w w w w w w q q N c c q q q q q")
PLAN_Q = (
    "w w w w w w N c c w q q q q q q q E", "w w w N c c w w w w q q q q q q q E",
    "w w w w w N c c w w q q q q q q q E", "w w w w N c c w w w q q q q q q q E")
PLAN_Q_LATE = (
    "w N c c w w w w w w q q q q q q q E", "w w w w N c c w w w q q q q q q q E",
    "w w w w N c c w w w q q q q q q q E", "w w w w w w w q q q q q E q N c c q")
PLAN_Q_LAST = (
    "w w w w w w w q q N c c q q q q q E", "w w w w w w w q q q N c c q q q E q",
    "w w w w w w w q q N c c q q q q q E", "w w w w w w N c c w E")
PLAN_DRAIN = (
    "w w w E w w w w E", "w w w w w w E w",
    "w w w w w w w E", "w w w w w w w")
ORDER_FIRST = (1, 2, 3, 6, 5, 4, 7)
ORDER_KV = (1, 2, 3, 6, 4, 5, 7)
ORDER_Q = (4, 3, 2, 5, 1, 6, 7)
ORDER_OUT = (4, 7, 3, 1, 5, 2, 6)


def _dot(a, b):
    return jnp.dot(a, b, preferred_element_type=F32)


def _dot_nt(a, b):
    return lax.dot_general(a, b, (((1,), (1,)), ((), ())), preferred_element_type=F32)


def _pack(v):
    return pltpu.bitcast(v.astype(BF), U32)


def _unpack(v):
    return pltpu.bitcast(v, BF)


def _recip(v):
    return pl.reciprocal(v, approx=False, full_range=False)


def _rows(start, size):
    return pl.ds(start if isinstance(start, int) else pl.multiple_of(start, 8), size)


def _normalize(v):
    centered = v - jnp.mean(v, axis=-1, keepdims=True)
    var = jnp.mean(centered * centered, axis=-1, keepdims=True)
    return centered * lax.rsqrt(var + 1e-5)


def _fold8(v, op=jnp.add):
    parts = [v[i:i + 8] for i in range(0, v.shape[0], 8)]
    while len(parts) > 1:
        parts = [op(parts[i], parts[i + 1]) for i in range(0, len(parts), 2)]
    return parts[0]


def _per_head(v, op):
    r = _fold8(v, op)
    r = op(r, pltpu.roll(r, 4, 0))
    return op(r, pltpu.roll(r, 2, 0))


def _hedgehog(p):
    def spread(v):
        return jnp.concatenate([v] * 8, axis=0)

    pos = jnp.exp2(p - spread(_per_head(p, jnp.maximum)))
    neg = jnp.exp2(spread(_per_head(p, jnp.minimum)) - p)
    pos = pos * spread(_recip(_per_head(pos, jnp.add)))
    neg = neg * spread(_recip(_per_head(neg, jnp.add)))
    return jnp.concatenate([pos, neg], axis=0)


def _rotate(v, shift):
    return jnp.concatenate([pltpu.roll(v[:, i:i + 128], shift, 1) for i in range(0, v.shape[1], 128)], axis=1)


def _left_terms(a11, a12, a21, a22):
    return a11 + a22, a21 + a22, a11, a22, a11 + a12, a21 - a11, a12 - a22


def _right_terms(b11, b12, b21, b22):
    return b11 + b22, b11, b12 - b22, b21 - b11, b22, b11 + b12, b21 + b22


class _Strassen:
    _USES = {1: ((0, 1), (3, 1)), 2: ((2, 1), (3, -1)), 3: ((1, 1), (3, 1)), 4: ((0, 1), (2, 1)),
             5: ((0, -1), (1, 1)), 6: ((3, 1),), 7: ((0, 1),)}

    def __init__(self, product, order):
        self._product = product
        self._todo = list(order)
        self._c = [None] * 4

    @property
    def done(self):
        return not self._todo

    def step(self):
        i = self._todo.pop(0)
        m = self._product(i - 1)
        for k, sign in self._USES[i]:
            if self._c[k] is None:
                assert sign > 0
                self._c[k] = m
            else:
                self._c[k] = self._c[k] + m if sign > 0 else self._c[k] - m

    def result(self):
        assert self.done
        return jnp.concatenate(self._c[:2], axis=1), jnp.concatenate(self._c[2:], axis=1)


class _Blocks:
    def __init__(self, product, partial):
        self._product = product
        self._partial = partial
        self._todo = [(k, c) for k in range(2) for c in (0, 2, 1, 3)]
        self._c = [None] * 4

    def step(self):
        k, c = self._todo.pop(0)
        m = self._product(c // 2, k, c % 2)
        if k == 0:
            self._partial(c)[...] = m
        else:
            self._c[c] = m + self._partial(c)[...]

    def result(self):
        assert not self._todo
        return jnp.concatenate(self._c[:2], axis=1), jnp.concatenate(self._c[2:], axis=1)


def _kernel(x_hbm, wqkv_hbm, wphi_hbm, wo_hbm, wr_hbm, wg_hbm, wu_hbm, wd_hbm, c_hbm, wmod_hbm,
            out_hbm,
            x_v, wqkv_v, wphi_v, wo_v, wr_v, wg_v, wu_v, wd_v, c_v, wmod_v,
            wkv_s, wq_s, wo_s, h_s, kv_s, mod_s, col_s, x1_s, stat_s, out_s, fmap_s,
            oa_s, ob_s, vec_s, xn_s, carry_s, raw_s, z_s,
            sem_w, sem_m, sem_k, sem_v, sem_x, sem_o, sem_p):
    def wcopy(i, src, dst):
        return pltpu.make_async_copy(src, dst, sem_w.at[i])

    cp_c = wcopy(0, c_hbm, c_v)
    cp_phi = wcopy(1, wphi_hbm, wphi_v)
    cp_wr = wcopy(2, wr_hbm, wr_v)
    cp_wq = wcopy(3, wqkv_hbm.at[:, 0:D], wqkv_v.at[:, 0:D])
    cp_mb = wcopy(4, wmod_hbm.at[:, 2 * D:4 * D], wmod_v.at[:, 2 * D:4 * D])
    cp_mc = wcopy(5, wmod_hbm.at[:, 4 * D:6 * D], wmod_v.at[:, 4 * D:6 * D])
    cp_wo = wcopy(6, wo_hbm, wo_v.at[:, 0:D])
    cp_wg = wcopy(7, wg_hbm, wg_v.at[:, 0:F])
    cp_wu = wcopy(8, wu_hbm, wu_v.at[:, 0:F])
    cp_wd = wcopy(9, wd_hbm, wd_v.at[:, 0:D])

    def mod_copy(j):
        col0 = (j % 2) * D + (j // 2) * KH
        cols = pl.ds(col0 if isinstance(j, int) else pl.multiple_of(col0, KH), KH)
        return pltpu.make_async_copy(wmod_hbm.at[:, cols], wmod_v.at[:, cols], sem_m.at[j])

    def scale_copy(k):
        piece = (slice(k * KH, (k + 1) * KH), slice(D + KH, 2 * D))
        return pltpu.make_async_copy(wmod_hbm.at[piece], wmod_v.at[piece], sem_m.at[3 + k])

    def kv_copies(o):
        ck, cv = pl.ds(D + o * 256, 256), pl.ds(2 * D + o * 256, 256)
        return (pltpu.make_async_copy(wqkv_hbm.at[:, ck], wqkv_v.at[:, ck], sem_k.at[o]),
                pltpu.make_async_copy(wqkv_hbm.at[:, cv], wqkv_v.at[:, cv], sem_v.at[o]))

    def x_copy(t):
        rows = _rows(t * T, T)
        return pltpu.make_async_copy(x_hbm.at[rows], x_v.at[rows], sem_x.at[t])

    def out_copy(t):
        rows = _rows(t * T, T)
        return pltpu.make_async_copy(out_s.at[rows], out_hbm.at[rows], sem_o.at[t])

    def start(*copies):
        for cp in copies:
            cp.start()

    def wait(*copies):
        for cp in copies:
            cp.wait()

    def fold(col0, g):
        return _dot_nt(_unpack(fmap_s[g * 64:(g + 1) * 64, :]),
                       wqkv_v[:, col0 + g * 128:col0 + (g + 1) * 128]) * LOG2E

    def stage_left(dst, o, upper, lower):
        n = upper.shape[0] // 2
        for i, a in enumerate(_left_terms(upper[:, :KH], upper[:, KH:], lower[:, :KH], lower[:, KH:])):
            dst[(i * 4 + o) * n:(i * 4 + o + 1) * n, :] = _pack(a)

    def stage_kv_weights(o):
        blocks = []
        for g in (2 * o, 2 * o + 1):
            fk = fold(D, g)
            fv = wqkv_v[:, 2 * D + g * 128:2 * D + (g + 1) * 128].T.astype(F32)
            blocks.append(jnp.concatenate([fk[:64], fv[:64], fk[64:], fv[64:]], axis=0))
        stage_left(wkv_s, o, *blocks)
        return blocks

    def stage_q_weights(o):
        stage_left(wq_s, o, fold(0, o), fold(0, o + 4))

    def stage_out_weights(o):
        stage_left(wo_s, o, wo_v[:, o * 128:(o + 1) * 128].T.astype(F32),
                   wo_v[:, KH + o * 128:KH + (o + 1) * 128].T.astype(F32))

    def param(k, n):
        return jnp.concatenate([mod_s[:, k * D:(k + 1) * D]] * (n // 8), axis=0)

    def modulation(col0, rows=slice(0, D)):
        return _dot(_unpack(vec_s[:, rows]), wmod_v[rows, col0:col0 + KH])[0:8]

    def store_column(k, row):
        for g in range(8):
            col_s[k * D + g * 128:k * D + (g + 1) * 128, :] = jnp.broadcast_to(
                row[:, g * 128:(g + 1) * 128], (128, 128)).T

    def vector_product(w_ref, c0, tables, rows):
        accs = [None] * len(tables)
        for k0 in range(0, D, rows):
            w = w_ref[k0:k0 + rows, c0:c0 + 256].astype(F32)
            for k, table in enumerate(tables):
                v = col_s[table * D + k0:table * D + k0 + rows, :]
                part = _rotate(_fold8(w * jnp.concatenate([v, v], axis=1)), 1)
                accs[k] = part if accs[k] is None else accs[k] + part
        return [jnp.sum(_rotate(a, 127), axis=0, keepdims=True) for a in accs]

    def vector_modulation(k):
        for c0 in range(k * D, (k + 1) * D, 256):
            mod_s[:, c0:c0 + 256] = jnp.broadcast_to(vector_product(wmod_v, c0, (COL_VEC0,), 32)[0], (8, 256))

    def first_norm(t, dst, base):
        for r0 in range(0, U, LN_ROWS):
            h = []
            for half in range(2):
                rows = _rows(t * T + half * U + r0, LN_ROWS)
                xn = _normalize(x_v[rows, :].astype(F32))
                h.append(xn * param(SCALE_A, LN_ROWS) + param(SHIFT_A, LN_ROWS))
            for i, b in enumerate(_right_terms(h[0][:, :KH], h[1][:, :KH], h[0][:, KH:], h[1][:, KH:])):
                dst[base + i * 64 + r0 // 2:base + i * 64 + (r0 + LN_ROWS) // 2, :] = _pack(b)

    def kv_products(src, base, o, order=ORDER_KV):
        return _Strassen(lambda i: _dot_nt(_unpack(wkv_s[(i * 4 + o) * 128:(i * 4 + o + 1) * 128, :]),
                                           _unpack(src[base + i * 64:base + (i + 1) * 64, :])), order)

    def kv_pairs(block, p0, last=False):
        ops = []
        for j in range(2):
            phi = _hedgehog(block[j * 128:j * 128 + 64])
            z = (phi[:, :U] + phi[:, U:]) + z_s[p0 + j]
            z_s[p0 + j] = jnp.broadcast_to(jnp.sum(z, axis=1, keepdims=True), (128, U)) if last else z
            ops.append((block[j * 128 + 64:(j + 1) * 128].astype(BF), phi.astype(BF)))
        return ops

    def kv_operands(r, o, last=False):
        return kv_pairs(r[0], 4 * o, last) + kv_pairs(r[1], 4 * o + 2, last)

    def save_kv_operands(r):
        raw_s[...] = r[0]
        for j, (v, phi) in enumerate(kv_pairs(r[1], NPAIR - 2)):
            carry_s[j * 64:(j + 1) * 64, :] = pltpu.bitcast(phi, U32)
            carry_s[128 + j * 32:128 + (j + 1) * 32, :] = pltpu.bitcast(v, U32)

    def load_kv_operands():
        done = [(_unpack(carry_s[128 + j * 32:128 + (j + 1) * 32, :]), _unpack(carry_s[j * 64:(j + 1) * 64, :]))
                for j in range(2)]
        return kv_pairs(raw_s[...], NPAIR - 4) + done

    def accumulate_kv(ops, o, last=False):
        for j, (v, phi) in enumerate(ops):
            acc = _dot_nt(v, phi) + kv_s[4 * o + j]
            if last:
                row_head = lax.broadcasted_iota(I32, (64, 128), 0) // DH
                lane_head = lax.broadcasted_iota(I32, (64, 128), 1) % 2
                acc = jnp.where(row_head == lane_head, acc, 0.0)
            kv_s[4 * o + j] = acc

    start(cp_phi, cp_c, *kv_copies(0), x_copy(0), x_copy(1))
    lax.fori_loop(0, 3, lambda j, _: mod_copy(j).start(), None)
    start(scale_copy(0), scale_copy(1))
    cp_c.wait()
    cv = c_v[...].astype(F32)
    activated = cv * jax.nn.sigmoid(cv)
    vec_s[...] = _pack(jnp.broadcast_to(activated, (16, D)))
    store_column(COL_VEC0, activated)
    cp_phi.wait()
    repeat = ((lax.broadcasted_iota(I32, (128, DH), 0) % 64) // 2
              == lax.broadcasted_iota(I32, (128, DH), 1)).astype(BF)
    block_row = lax.broadcasted_iota(I32, (128, 128), 0)
    same_head = 2 * (block_row // 64) + block_row % 2 == lax.broadcasted_iota(I32, (128, 128), 1) // DH
    for g in range(8):
        full = _dot_nt(repeat, wphi_v[g * 128:(g + 1) * 128, :])
        fmap_s[g * 64:(g + 1) * 64, :] = _pack(jnp.where(same_head, full, 0.0))
    kv_s[...] = jnp.zeros(kv_s.shape, F32)
    z_s[...] = jnp.zeros(z_s.shape, F32)
    wait(*kv_copies(0))
    upper, lower = stage_kv_weights(0)
    wq_s[0:128, :] = _pack(upper[:, KH:])
    wq_s[128:256, :] = _pack(lower[:, :KH])

    def left_block(r, k):
        return wkv_s[(2 + r) * 512:(2 + r) * 512 + 128, :] if r == k else wq_s[r * 128:(r + 1) * 128, :]

    def right_block(t, k, half):
        if k == half:
            return h_s.at[t * HROWS + (1 + 3 * k) * 64:t * HROWS + (2 + 3 * k) * 64]
        return wq_s.at[256 + (2 * t + k) * 64:256 + (2 * t + k + 1) * 64]

    def early_products(t):
        return _Blocks(lambda r, k, half: _dot_nt(_unpack(left_block(r, k)), _unpack(right_block(t, k, half)[...])),
                       lambda c: x1_s.at[(4 * t + c) * 256:(4 * t + c + 1) * 256])

    def early_operands(t, k):
        cols = slice(k * KH, (k + 1) * KH)
        scale, shift = (jnp.concatenate([mod_s[:, p * D + k * KH:p * D + (k + 1) * KH]] * (U // 8), axis=0)
                        for p in (SCALE_A, SHIFT_A))
        for half in range(2):
            rows = slice(t * T + half * U, t * T + (half + 1) * U)
            h = xn_s[rows, cols] * scale + shift
            xn_s[rows, cols] = h
            right_block(t, k, half)[...] = _pack(h)

    def remaining_terms(t):
        for r0 in range(0, U, LN_ROWS):
            h = [xn_s[t * T + half * U + r0:t * T + half * U + r0 + LN_ROWS, :] for half in range(2)]
            for i, b in enumerate(_right_terms(h[0][:, :KH], h[1][:, :KH], h[0][:, KH:], h[1][:, KH:])):
                if i not in (1, 4):
                    row = t * HROWS + i * 64 + r0 // 2
                    h_s[row:row + LN_ROWS // 2, :] = _pack(b)

    for t in range(2):
        x_copy(t).wait()
        xn_s[t * T:(t + 1) * T, :] = _normalize(x_v[t * T:(t + 1) * T, :].astype(F32))
    early = [early_products(t) for t in range(2)]
    mod_copy(0).wait()
    mod_s[:, 0:KH] = modulation(0)
    mod_copy(1).wait()
    mod_s[:, D:D + KH] = modulation(D) + 1.0
    for t in range(2):
        early_operands(t, 0)
        for _ in range(4):
            early[t].step()
    mod_copy(2).wait()
    start(*kv_copies(1), *kv_copies(2))
    mod_s[:, KH:D] = modulation(KH)
    scale_copy(0).wait()
    mod_s[:, D + KH:2 * D] = modulation(D + KH, slice(0, KH)) + 1.0
    scale_copy(1).wait()
    start(*kv_copies(3))
    mod_s[:, D + KH:2 * D] += modulation(D + KH, slice(KH, D))
    for t in range(2):
        early_operands(t, 1)

    waited = staged = 1
    normalized = 0
    for n, plan in enumerate(PLAN_FIRST):
        products = early[n] if n < 2 else kv_products(h_s, (n % 2) * HROWS, n // 2, ORDER_FIRST)
        for item in plan.split():
            if item == "p":
                products.step()
            elif item == "W":
                wait(*kv_copies(waited))
                waited += 1
                if waited == 3:
                    start(x_copy(2), x_copy(3))
            elif item == "X":
                x_copy(2).wait()
                start(*(x_copy(t) for t in range(4, NT)), cp_wr, cp_wq, cp_wo)
                x_copy(3).wait()
            elif item == "s":
                stage_kv_weights(staged)
                staged += 1
            elif item == "F":
                remaining_terms(normalized)
                normalized += 1
            elif item == "L":
                first_norm(normalized, h_s, normalized * HROWS)
                normalized += 1
            elif item == "f":
                ops = kv_operands(projected, (n - 1) // 2)
            else:
                accumulate_kv(ops, (n - 1) // 2)
        projected = products.result()
    save_kv_operands(projected)

    def kv_steps(ops, steps, plans, last_from):
        staged_q = staged_out = modulated = 0
        for o, (products, plan) in enumerate(zip(steps, plans)):
            for item in plan.split():
                if item == "p":
                    products.step()
                elif item == "s":
                    stage_q_weights(staged_q)
                    staged_q += 1
                elif item == "o":
                    stage_out_weights(staged_out)
                    staged_out += 1
                elif item == "V":
                    vector_modulation(GATE_A + modulated)
                    modulated += 1
                elif item == "B":
                    cp_wr.wait()
                else:
                    if o:
                        ops = kv_operands(projected, (o - 1) % 4, last=o >= last_from)
                    accumulate_kv(ops, (o - 1) % 4, last=o >= last_from)
            projected = products.result()
        return projected

    def pass1(i, remaining):
        t = 2 * i + 2
        pl.when(i == 0)(cp_mb.start)
        pl.when(i == 1)(cp_mc.start)
        wait(x_copy(t + 2), x_copy(t + 3))
        view = h_s.at[_rows(t * HROWS, 4 * HROWS)]
        first_norm(t + 2, view, 2 * HROWS)
        first_norm(t + 3, view, 3 * HROWS)
        steps = [kv_products(view, k * HROWS, o) for k in range(2) for o in range(4)]
        save_kv_operands(kv_steps(load_kv_operands(), steps, PLAN_KV, last_from=len(steps)))
        return remaining - 1

    first_tile = lax.fori_loop(0, 2, pass1, 2)

    def q_products(t, o):
        return _Strassen(lambda i: _dot_nt(_unpack(wq_s[(i * 4 + o) * 64:(i * 4 + o + 1) * 64, :]),
                                           _unpack(h_s[_rows(t * HROWS + i * 64, 64), :])), ORDER_Q)

    def derived_params():
        wr8 = wr_v[...].astype(F32)
        wr = jnp.broadcast_to(jnp.concatenate([wr8[j:j + 1, :] for j in range(8)], axis=1), (8, D))
        scale = 1.0 + param(SCALE_B, 8)
        mod_s[:, SCALE_B * D:(SCALE_B + 1) * D] = scale
        router = scale * wr
        tables = (param(GATE_A, 8), router, scale * param(GATE_B, 8), param(SHIFT_B, 8) * param(GATE_B, 8))
        for k, row in enumerate(tables):
            store_column(k, row[0:1])
        base = ROUTER_SUMS * D
        mod_s[:, base:base + T] = jnp.broadcast_to(jnp.sum(router, axis=-1, keepdims=True), (8, T))
        mod_s[:, base + T:base + 2 * T] = jnp.broadcast_to(
            jnp.sum(param(SHIFT_B, 8) * wr, axis=-1, keepdims=True), (8, T))

    def column(k, ch):
        v = col_s[k * D + ch:k * D + ch + 128, :]
        return jnp.concatenate([v, v], axis=1)

    def feature_pairs(block, p0):
        out = []
        for j in range(2):
            phi = _hedgehog(block[j * 64:(j + 1) * 64])
            z = z_s[p0 + j]
            inv = _recip(_per_head(phi * jnp.concatenate([z, z], axis=1), jnp.add) + 1e-6)
            out.append((phi.astype(BF), inv))
        return out

    def features(r, o):
        return feature_pairs(r[0], 2 * o) + feature_pairs(r[1], 2 * o + 8)

    def save_features(r):
        raw_s[0:128, :] = r[0]
        for j, (phi, inv) in enumerate(feature_pairs(r[1], 8)):
            carry_s[j * 64:(j + 1) * 64, :] = pltpu.bitcast(phi, U32)
            raw_s[128 + 8 * j:136 + 8 * j, :] = inv

    def load_features():
        done = [(_unpack(carry_s[j * 64:(j + 1) * 64, :]), raw_s[128 + 8 * j:136 + 8 * j, :]) for j in range(2)]
        return feature_pairs(raw_s[0:128, :], 0) + done

    def attend(phis, o):
        heads = {}
        for j in (0, 2, 1, 3):
            phi, inv = phis[j]
            num = _dot(kv_s[2 * o + 8 * (j // 2) + j % 2].astype(BF), phi)
            heads[j] = jnp.concatenate([num[k * DH:(k + 1) * DH] * inv[k:k + 1] for k in range(2)], axis=0)
        return heads

    def stage_heads(dst, o, j, lo, hi):
        base = o * 64 + j * 32
        terms = _right_terms(lo[:, :U], lo[:, U:], hi[:, :U], hi[:, U:])
        dst[base:base + 32, 0:6 * U] = _pack(jnp.concatenate(terms[:6], axis=1))
        dst[base:base + 16, 6 * U:8 * U] = _pack(jnp.concatenate([terms[6][:32], terms[6][32:]], axis=1))

    def out_products(src, o):
        def product(i):
            if i < 6:
                b = src[:, i * U:(i + 1) * U]
            else:
                b = jnp.concatenate([src[k * 32:k * 32 + 16, (6 + c) * U:(7 + c) * U]
                                     for k in range(8) for c in range(2)], axis=0)
            return _dot(_unpack(wo_s[(i * 4 + o) * 64:(i * 4 + o + 1) * 64, :]), _unpack(b))
        return _Strassen(product, ORDER_OUT)

    def residual(t, o, attn, sums):
        ys = []
        for half, a in enumerate(attn):
            ch = half * KH + o * 128
            ys.append(x_v[_rows(t * T, T), ch:ch + 128].T.astype(F32) + column(COL_GATE_A, ch) * a)
        if sums is None:
            shift = jnp.sum(_fold8(ys[0]) + _fold8(ys[1]), axis=0, keepdims=True) * (1.0 / 256)
            sums = (shift, 0.0, 0.0, 0.0)
        shift, s1, s2, s3 = sums
        for half, y in enumerate(ys):
            ch = half * KH + o * 128
            d = y - shift
            for k in range(2):
                x1_s[_rows((2 * t + k) * D + ch, 128), :] = y[:, k * U:(k + 1) * U]
            s1, s2, s3 = s1 + _fold8(d), s2 + _fold8(d * d), s3 + _fold8(d * column(COL_ROUTER, ch))
        return shift, s1, s2, s3

    def route(t, sums, top):
        m1, i1, m2, i2 = top
        shift = sums[0]
        s1, s2, s3 = (jnp.sum(s, axis=0, keepdims=True) for s in sums[1:])
        delta = s1 * (1.0 / D)
        rstd = lax.rsqrt(jnp.maximum(s2 * (1.0 / D) - delta * delta, 0.0) + 1e-5)
        score = (s3 - delta * mod_s[0:1, ROUTER_SUMS * D:ROUTER_SUMS * D + T]) * rstd
        for k, v in enumerate((shift + delta, rstd)):
            for half in range(2):
                stat_s[_rows(((2 * t + half) * 2 + k) * 8, 8), :] = jnp.broadcast_to(
                    v[:, half * U:(half + 1) * U], (8, U))
        idx = lax.broadcasted_iota(I32, (1, T), 1) + t * T
        g1, g2 = score > m1, score > m2
        return (jnp.where(g1, score, m1), jnp.where(g1, idx, i1),
                jnp.where(g1, m1, jnp.where(g2, score, m2)), jnp.where(g1, i1, jnp.where(g2, idx, i2)))

    def stat(block, k, n):
        return jnp.concatenate([stat_s[_rows((block * 2 + k) * 8, 8), :]] * (n // 8), axis=0)

    def emit(t, ch):
        n = 256
        for half in range(2):
            mean, rstd = (stat(2 * t + half, k, n) for k in range(2))
            x1 = x1_s[_rows((2 * t + half) * D + ch, n), :]
            gain = rstd * col_s[COL_GAIN * D + ch:COL_GAIN * D + ch + n, :]
            res = (x1 + col_s[COL_BIAS * D + ch:COL_BIAS * D + ch + n, :]) + (x1 - mean) * gain
            out_s[_rows(t * T + half * U, U), ch:ch + n] = res.T.astype(BF)

    def q_tile(t, phis, top, plans, current, previous, more=True):
        sums, emitted = None, 0
        for o, plan in enumerate(plans):
            qs = None
            if phis is not None and (o < 3 or more):
                qs = q_products(t, o + 1) if o < 3 else q_products(t + 1, 0)
            ws = out_products(previous, o)
            heads, staged = None, 0
            for item in plan.split():
                if item == "q":
                    qs.step()
                elif item == "w":
                    ws.step()
                    if ws.done:
                        sums = residual(t - 1, o, ws.result(), sums)
                elif item == "N":
                    heads = attend(phis, o)
                elif item == "c":
                    stage_heads(current, o, staged, heads[staged], heads[staged + 2])
                    staged += 1
                elif item == "E":
                    emit(t - 2, emitted * 256)
                    emitted += 1
            if qs is not None:
                phis = features(qs.result(), o + 1) if o < 3 else qs.result()
        if sums is not None:
            top = route(t - 1, sums, top)
        if emitted:
            out_copy(t - 2).start()
        return phis, top

    wait(cp_wq, cp_wo, cp_mb, cp_mc)
    start(cp_wg, cp_wu)
    steps = [kv_products(h_s, t * HROWS, o) for t in (NT - 2, NT - 1) for o in range(4)]
    r = kv_steps(load_kv_operands(), steps + [q_products(first_tile, 0)], PLAN_KV_LAST, last_from=5)
    lowest = jnp.full((1, T), -jnp.inf, F32)
    zero = jnp.zeros((1, T), I32)
    top = (lowest, zero, lowest, zero)
    r, top = q_tile(first_tile, features(r, 0), top, PLAN_Q_FIRST, oa_s, ob_s)
    derived_params()
    r, top = q_tile(first_tile + 1, features(r, 0), top, PLAN_Q_SECOND, ob_s, oa_s)
    save_features(r)

    def pass2(i, carry):
        top, tile = carry
        pl.when(i == 2)(cp_wd.start)
        r, top = q_tile(2 * i - 2, load_features(), top, PLAN_Q, oa_s, ob_s)
        r, top = q_tile(2 * i - 1, features(r, 0), top, PLAN_Q, ob_s, oa_s)
        save_features(r)
        return top, tile + 2

    top, tile = lax.fori_loop(2, 4, pass2, (top, 2))
    wait(cp_wg, cp_wu, cp_wd)
    r, top = q_tile(tile, load_features(), top, PLAN_Q_LATE, oa_s, ob_s)
    _, top = q_tile(tile + 1, features(r, 0), top, PLAN_Q_LAST, ob_s, oa_s, more=False)
    _, top = q_tile(tile + 2, None, top, PLAN_DRAIN, oa_s, ob_s)

    m1, i1, m2, i2 = top
    best = jnp.max(m1, axis=1, keepdims=True)
    ia = jnp.min(jnp.where(m1 == best, i1, S - 1), axis=1, keepdims=True)
    taken = i1 == ia
    rest, rest_idx = jnp.where(taken, m2, m1), jnp.where(taken, i2, i1)
    second = jnp.max(rest, axis=1, keepdims=True)
    ib = jnp.min(jnp.where(rest == second, rest_idx, S - 1), axis=1, keepdims=True)
    idx = (jnp.clip(ia[0, 0], 0, S - 1), jnp.clip(ib[0, 0], 0, S - 1))

    for g in range(4):
        emit(NT - 1, g * 256)
    out_copy(NT - 1).start()
    out_copy(0).wait()

    row16 = lax.broadcasted_iota(I32, (16, U), 0)
    lane16 = lax.broadcasted_iota(I32, (16, U), 1)
    xn_sel = 0.0
    for k in range(2):
        block = idx[k] // U
        xn = (x1_s[_rows(block * D, D), :] - stat(block, 0, D)) * stat(block, 1, D)
        pick = jnp.where((row16 == k) & (lane16 == idx[k] % U), 1.0, 0.0).astype(BF)
        xn_sel = xn_sel + _dot_nt(pick, xn.astype(BF))
    hs = (xn_sel * param(SCALE_B, 16) + param(SHIFT_B, 16)).astype(BF)
    score = jnp.where(row16[:, 0:1] == 0, best, second) + mod_s[0:1, ROUTER_SUMS * D + T:ROUTER_SUMS * D + T + 1]
    gate = jax.nn.sigmoid(score)

    for k in range(2):
        store_column(COL_VEC0 + k, hs.astype(F32)[k:k + 1])

    def down(g, u, c0, c1):
        return _dot((g * jax.nn.sigmoid(g) * u).astype(BF), wd_v[c0:c1, 0:D])

    fm = F - F_VECTOR
    y = down(_dot(hs, wg_v[:, 0:fm]), _dot(hs, wu_v[:, 0:fm]), 0, fm)
    first_row = lax.broadcasted_iota(I32, (16, 256), 0) == 0
    for c0 in range(fm, F, 256):
        g, u = (jnp.where(first_row, *vector_product(w, c0, (COL_VEC0, COL_VEC1), 16)) for w in (wg_v, wu_v))
        y = y + down(g, u, c0, c0 + 256)
    update = param(GATE_B, 16) * (y * gate)

    wait(*(out_copy(t) for t in range(1, NT)))
    row = lax.broadcasted_iota(I32, (16, D), 0)

    def patch(k):
        base = pl.multiple_of((idx[k] // 16) * 16, 16)
        block = out_s[pl.ds(base, 16), :].astype(F32)
        out_s[pl.ds(base, 16), :] = jnp.where(row == idx[k] - base, block + update[k:k + 1, :], block).astype(BF)
        return pltpu.make_async_copy(out_s.at[pl.ds(base, 16)], out_hbm.at[pl.ds(base, 16)], sem_p.at[k])

    patch_a, patch_b = patch(0), patch(1)
    patch_a.start()

    @pl.when(idx[0] // 16 != idx[1] // 16)
    def _():
        patch_b.start()
        patch_b.wait()

    patch_a.wait()


@jax.jit
def pallas_adaLN_cond__linear_kernel_hedgehog__moe_arch_mod__prompt_kernel(
        A_x, A_wqkv, A_w_phi, A_wo, B_x, B_w_r, B_w_gate, B_w_up, B_w_down, c, w_mod):
    del B_x
    hbm = pl.BlockSpec(memory_space=pl.ANY)
    out = pl.pallas_call(
        _kernel,
        out_shape=jax.ShapeDtypeStruct((S, D), BF),
        in_specs=[hbm] * 10,
        out_specs=hbm,
        scratch_shapes=[
            pltpu.VMEM((S, D), BF),
            pltpu.VMEM((D, 3 * D + PAD), BF),
            pltpu.VMEM((H * DH, DH), BF),
            pltpu.VMEM((D, D + PAD), BF),
            pltpu.VMEM((8, 128), BF),
            pltpu.VMEM((D, F + PAD), BF),
            pltpu.VMEM((D, F + PAD), BF),
            pltpu.VMEM((F, D + PAD), BF),
            pltpu.VMEM((1, D), BF),
            pltpu.VMEM((D, 6 * D + PAD), BF),
            pltpu.VMEM((7 * 512, KH), U32),
            pltpu.VMEM((7 * 256, KH), U32),
            pltpu.VMEM((7 * 256, KH), U32),
            pltpu.VMEM((NT * HROWS, KH), U32),
            pltpu.VMEM((NPAIR, 64, 128), F32),
            pltpu.VMEM((8, 6 * D + 2 * T), F32),
            pltpu.VMEM((6 * D, 128), F32),
            pltpu.VMEM((2 * NT * D, U), F32),
            pltpu.VMEM((2 * NT * 2 * 8, U), F32),
            pltpu.VMEM((S, D), BF),
            pltpu.VMEM((8 * 64, 128), U32),
            pltpu.VMEM((KH // 2, 8 * U), U32),
            pltpu.VMEM((KH // 2, 8 * U), U32),
            pltpu.VMEM((8, D), U32),
            pltpu.VMEM((2 * T, D), F32),
            pltpu.VMEM((192, T), U32),
            pltpu.VMEM((256, T), F32),
            pltpu.VMEM((NPAIR, 128, U), F32),
            pltpu.SemaphoreType.DMA((10,)),
            pltpu.SemaphoreType.DMA((5,)),
            pltpu.SemaphoreType.DMA((4,)),
            pltpu.SemaphoreType.DMA((4,)),
            pltpu.SemaphoreType.DMA((NT,)),
            pltpu.SemaphoreType.DMA((NT,)),
            pltpu.SemaphoreType.DMA((2,)),
        ],
        compiler_params=pltpu.CompilerParams(
            vmem_limit_bytes=110 * 2**20,
            flags={"XLA_TPU_EVENLY_DISTRIBUTE_CRITICAL_NODES": True}),
        name="fused_block",
    )(A_x.reshape(S, D), A_wqkv, A_w_phi.reshape(H * DH, DH), A_wo, B_w_r.reshape(8, 128),
      B_w_gate, B_w_up, B_w_down, c, w_mod)
    return out.reshape(1, S, D)
```
